```python
import jax
import jax.numpy as jnp

def _softmax(x, axis=-1):
    return jax.nn.softmax(x, axis=axis)
def _gelu(x):
    return jax.nn.gelu(x, approximate=True)
def _silu(x):
    return jax.nn.silu(x)
def _sigmoid(x):
    return jax.nn.sigmoid(x)
def _layernorm(x, axis=-1, eps=1e-5):
    m = jnp.mean(x, axis=axis, keepdims=True)
    v = jnp.var(x, axis=axis, keepdims=True)
    return (x - m) / jnp.sqrt(v + eps)
def _scatter_add(tgt, idx, src, axis=0):
    return tgt.at[idx].add(src)
def _segment_sum(src, seg, n):
    return jax.ops.segment_sum(src, seg, n)
class _Rng:
    def __init__(self, key):
        self._k = key
    def _next(self):
        self._k, sub = jax.random.split(self._k)
        return sub
    def normal(self, shape):
        return jax.random.normal(self._next(), shape, dtype=jnp.bfloat16)
    def randint(self, lo, hi, shape):
        return jax.random.randint(self._next(), shape, lo, hi, dtype=jnp.int32)
    def uniform(self, shape, lo=0.0, hi=1.0):
        return jax.random.uniform(self._next(), shape, jnp.bfloat16, lo, hi)
    def permutation(self, n):
        return jax.random.permutation(self._next(), n)


kernel_name = 'parallel_sum__compressed_kv_cla__moe_arch_mod__prompt'

def setup_inputs():
    _rng = _Rng(jax.random.key(int.from_bytes(__import__("os").urandom(4), "little")))
    _w = (lambda a: (lambda t: t.astype(jnp.bfloat16) if jnp.issubdtype(t.dtype, jnp.floating) else t)(jnp.asarray(a)))
    def _A_setup():
        B, H, Sq, Sk, D, M = 1, 32, 2048, 2048, 128, 640
        Dc = 4 * D
        return {
            "x": _w((lambda *s: _rng.normal(s) * 0.05)(B, Sq, M)),
            "c_kv": _w((lambda *s: _rng.normal(s) * 0.05)(B, Sk, Dc)),
            "w_q": _w((lambda *s: _rng.normal(s) * 0.05)(M, H, D) * (M ** -0.5)),
            "w_uk": _w((lambda *s: _rng.normal(s) * 0.05)(Dc, H, D) * (Dc ** -0.5)),
            "w_uv": _w((lambda *s: _rng.normal(s) * 0.05)(Dc, H, D) * (Dc ** -0.5)),
            "w_o": _w((lambda *s: _rng.normal(s) * 0.05)(H, D, M) * ((H * D) ** -0.5)),
        }
    _A_in = _A_setup()

    def _B_setup():
        B, S, D, F, C = 1, 2048, 640, 1728, 8
        return {
            "x": _w((lambda *s: _rng.normal(s) * 0.05)(B, S, D)),
            "w_r": _w((lambda *s: _rng.normal(s) * 0.05)(D)),
            "w_gate": _w((lambda *s: _rng.normal(s) * 0.05)(D, F)),
            "w_up": _w((lambda *s: _rng.normal(s) * 0.05)(D, F)),
            "w_down": _w((lambda *s: _rng.normal(s) * 0.05)(F, D)),
        }
    _B_in = _B_setup()

    return {
        "A_x": _A_in["x"],
        "A_c_kv": _A_in["c_kv"],
        "A_w_q": _A_in["w_q"],
        "A_w_uk": _A_in["w_uk"],
        "A_w_uv": _A_in["w_uv"],
        "A_w_o": _A_in["w_o"],
        "B_x": _B_in["x"],
        "B_w_r": _B_in["w_r"],
        "B_w_gate": _B_in["w_gate"],
        "B_w_up": _B_in["w_up"],
        "B_w_down": _B_in["w_down"],
    }

def reference(A_x, A_c_kv, A_w_q, A_w_uk, A_w_uv, A_w_o, B_x, B_w_r, B_w_gate, B_w_up, B_w_down):
    def _A_ref(x, c_kv, w_q, w_uk, w_uv, w_o):
        B, Sq, M = x.shape[0], x.shape[1], x.shape[2]
        Sk = c_kv.shape[1]
        H, D = w_q.shape[1], w_q.shape[2]
        q = jnp.einsum("bqm,mhd->bhqd", x, w_q)
        k = jnp.einsum("bkc,chd->bhkd", c_kv, w_uk)
        v = jnp.einsum("bkc,chd->bhkd", c_kv, w_uv)
        scores = jnp.einsum("bhqd,bhkd->bhqk", q, k) * (D ** -0.5)
        off = Sk - Sq
        qi = jnp.arange(Sq)[:, None]
        kj = jnp.arange(Sk)[None, :]
        cmask = kj <= (qi + off)
        scores = jnp.where(cmask[None, None], scores, -1e9)
        p = _softmax(scores, axis=-1)
        ctx = jnp.einsum("bhqk,bhkd->bhqd", p, v)
        return jnp.einsum("bhqd,hdm->bqm", ctx, w_o)

    def _B_ref(x, w_r, w_gate, w_up, w_down):
        B, S, D = x.shape
        C = 8
        r = x @ w_r
        idx = jnp.argsort(-r, axis=-1)[:, :C]
        idx_e = jnp.repeat(idx.reshape(B, C, 1), D, axis=2)
        x_sel = jnp.take_along_axis(x, idx_e, axis=1)
        g = _silu(x_sel @ w_gate)
        u = x_sel @ w_up
        y = (g * u) @ w_down
        r_sel = _sigmoid(jnp.take_along_axis(r, idx, axis=1))
        y = y * r_sel.reshape(B, C, 1)
        b_off = (jnp.arange(B) * S).reshape(B, 1)
        flat_idx = (idx + b_off).reshape(B * C)
        zero = (x * 0.0).reshape(B * S, D)
        upd = _scatter_add(zero, flat_idx, y.reshape(B * C, D), axis=0)
        return x + upd.reshape(B, S, D)

    x = A_x
    xn = _layernorm(x, axis=-1)
    return x + _A_ref(xn, A_c_kv, A_w_q, A_w_uk, A_w_uv, A_w_o) + _B_ref(xn, B_w_r, B_w_gate, B_w_up, B_w_down)
```

```python
import math

import numpy as np
import jax
import jax.numpy as jnp
from jax import lax
import jax.experimental.pallas as pl
import jax.experimental.pallas.tpu as pltpu

BF16 = jnp.bfloat16
F32 = jnp.float32
TOPC = 8
LN_EPS = float(np.float32(np.asarray(1e-5, dtype=jnp.bfloat16)))
NEG = -1e30
BQ = 256


def _rb(v):
    return v.astype(BF16).astype(F32)


def _dot(a, b):
    return jnp.dot(a, b, preferred_element_type=F32)


def _dot_nt(a, b):
    return lax.dot_general(a, b, (((1,), (1,)), ((), ())), preferred_element_type=F32)


def _head_weight(w_ref, h, rows, n_heads):
    w32 = w_ref[pl.ds(h // 2, rows, stride=n_heads // 2), :]
    sh = (16 * (1 - h % 2)).astype(jnp.uint32)
    w32 = (w32 << sh) & jnp.uint32(0xFFFF0000)
    return pltpu.bitcast(w32, F32).astype(BF16)


def _kernel(x_hbm, c_hbm, wq_hbm, wuk_hbm, wuv_hbm, wo_hbm, wr_ref, wg_hbm, wu_hbm, wd_hbm,
            out_hbm,
            x_v, c_v, wq_v, wuk_v, wuv_v, wo_v, wg_v, wu_v, wd_v,
            xn_v, acc_v, q_v, k_v, v_v, o_v, sems):
    S, M = x_v.shape
    DC = c_v.shape[1]
    H, D = wo_v.shape[0], wo_v.shape[1]
    srcs = (x_hbm, c_hbm, wq_hbm.bitcast(jnp.uint32), wuk_hbm.bitcast(jnp.uint32), wuv_hbm.bitcast(jnp.uint32), wo_hbm, wg_hbm, wu_hbm, wd_hbm)
    dsts = (x_v, c_v, wq_v, wuk_v, wuv_v, wo_v, wg_v, wu_v, wd_v)
    cps = [pltpu.make_async_copy(s, d, sems.at[i]) for i, (s, d) in enumerate(zip(srcs, dsts))]
    for cp in cps:
        cp.start()

    cps[0].wait()
    wr = wr_ref[...].astype(F32).reshape(1, M)
    lane = lax.broadcasted_iota(jnp.int32, (8, 128), 1)
    sub = lax.broadcasted_iota(jnp.int32, (8, 128), 0)
    LB = 128
    rds = []
    for half in range(S // 1024):
        def ln_body(i, rd):
            r0 = pl.multiple_of(half * 1024 + i * LB, LB)
            xf = x_v[pl.ds(r0, LB), :].astype(F32)
            mean = jnp.sum(xf, axis=-1, keepdims=True) / M
            cen = xf - mean
            var = jnp.sum(cen * cen, axis=-1, keepdims=True) / M
            den = _rb(jnp.sqrt(_rb(_rb(var) + LN_EPS)))
            xn = _rb(_rb(xf - _rb(mean)) / den)
            xn_v[pl.ds(r0, LB), :] = xn.astype(BF16)
            acc_v[pl.ds(r0, LB), :] = xf + xn
            r = jnp.sum(xn * wr, axis=-1, keepdims=True)
            for g in range(LB // 8):
                rd = jnp.where(lane == i * (LB // 8) + g, r[g * 8:(g + 1) * 8, :], rd)
            return rd
        rds.append(lax.fori_loop(0, 1024 // LB, ln_body, jnp.zeros((8, 128), F32)))

    keys = []
    for half, rd in enumerate(rds):
        bits = pltpu.bitcast(_rb(rd), jnp.int32) >> 16
        mag = bits & 0x7FFF
        order = jnp.where(bits < 0, 0x8000 - mag, 0x8000 + mag)
        order = jnp.where(mag > 0x7F80, 0, order)
        row = half * 1024 + lane * 8 + sub
        keys.append(order * S + (S - 1 - row))
    sel_keys = []
    for _ in range(TOPC):
        mx = keys[0]
        for kk in keys[1:]:
            mx = jnp.maximum(mx, kk)
        top = jnp.max(mx)
        sel_keys.append(top)
        keys = [jnp.where(kk == top, -1, kk) for kk in keys]

    sub16 = lax.broadcasted_iota(jnp.int32, (16, M), 0)
    sub8m = lax.broadcasted_iota(jnp.int32, (TOPC, M), 0)
    xs = jnp.zeros((TOPC, M), F32)
    key_col = jnp.zeros((TOPC, 128), jnp.int32)
    rows = []
    for j, top in enumerate(sel_keys):
        row = S - 1 - (top % S)
        rows.append(row)
        base = pl.multiple_of((row // 16) * 16, 16)
        tile = xn_v[pl.ds(base, 16), :].astype(F32)
        one = jnp.sum(jnp.where(sub16 == row % 16, tile, 0.0), axis=0, keepdims=True)
        xs = jnp.where(sub8m == j, one, xs)
        key_col = jnp.where(sub == j, top, key_col)
    order = key_col // S
    bits = jnp.where(order >= 0x8000, order - 0x8000, (0x8000 - order) | 0x8000)
    bits = jnp.where(order == 0, 0x7FC0, bits)
    r_sel = pltpu.bitcast(bits << 16, F32)[:, 0:1]
    for i in (6, 7, 8):
        cps[i].wait()
    xs = xs.astype(BF16)
    g = _dot_nt(xs, wg_v[...])
    u = _dot_nt(xs, wu_v[...])
    hid = (g * jax.nn.sigmoid(g) * u).astype(BF16)
    y = _dot(hid, wd_v[...]) * jax.nn.sigmoid(r_sel)
    for j, row in enumerate(rows):
        acc_v[pl.ds(row, 1), :] += y[j:j + 1, :]

    for i in (1, 2, 3, 4, 5):
        cps[i].wait()
    qscale = (D ** -0.5) * math.log2(math.e)
    tri = (lax.broadcasted_iota(jnp.int32, (BQ, BQ), 1)
           <= lax.broadcasted_iota(jnp.int32, (BQ, BQ), 0))

    def head_body(h, carry):
        wq = _head_weight(wq_v, h, M, H)
        wk = _head_weight(wuk_v, h, DC, H)
        wv = _head_weight(wuv_v, h, DC, H)
        q_v[...] = (_dot(xn_v[...], wq) * qscale).astype(BF16)
        kv = _dot(c_v[...], jnp.concatenate([wk, wv], axis=1))
        k_v[...] = kv[:, :D].astype(BF16)
        v_v[...] = kv[:, D:].astype(BF16)
        wo = wo_v[h]
        for i in range(S // BQ):
            r0 = i * BQ
            q = q_v[r0:r0 + BQ, :]
            sd = jnp.where(tri, _dot_nt(q, k_v[r0:r0 + BQ, :]), NEG)
            m = jnp.max(sd, axis=-1, keepdims=True)
            if i > 0:
                so = _dot_nt(q, k_v[0:r0, :])
                m = jnp.maximum(m, jnp.max(so, axis=-1, keepdims=True))
            pd = jnp.exp2(sd - m)
            l = jnp.sum(pd, axis=-1, keepdims=True)
            o = _dot(pd.astype(BF16), v_v[r0:r0 + BQ, :])
            if i > 0:
                po = jnp.exp2(so - m)
                l = l + jnp.sum(po, axis=-1, keepdims=True)
                o = o + _dot(po.astype(BF16), v_v[0:r0, :])
            ctx = (o / l).astype(BF16)
            acc_v[r0:r0 + BQ, :] += _dot(ctx, wo)
        return carry

    lax.fori_loop(0, H, head_body, 0)

    o_v[...] = acc_v[...].astype(BF16)
    cp = pltpu.make_async_copy(o_v, out_hbm, sems.at[0])
    cp.start()
    cp.wait()


@jax.jit
def pallas_parallel_sum__compressed_kv_cla__moe_arch_mod__prompt_kernel(
    A_x: jax.Array,
    A_c_kv: jax.Array,
    A_w_q: jax.Array,
    A_w_uk: jax.Array,
    A_w_uv: jax.Array,
    A_w_o: jax.Array,
    B_x: jax.Array,
    B_w_r: jax.Array,
    B_w_gate: jax.Array,
    B_w_up: jax.Array,
    B_w_down: jax.Array,
):
    del B_x
    _, S, M = A_x.shape
    DC = A_c_kv.shape[2]
    H, D = A_w_q.shape[1], A_w_q.shape[2]
    FF = B_w_gate.shape[1]
    any_spec = pl.BlockSpec(memory_space=pltpu.HBM)
    out = pl.pallas_call(
        _kernel,
        out_shape=jax.ShapeDtypeStruct((S, M), A_x.dtype),
        in_specs=[any_spec] * 6 + [pl.BlockSpec(memory_space=pltpu.VMEM)] + [any_spec] * 3,
        out_specs=any_spec,
        scratch_shapes=[
            pltpu.VMEM((S, M), BF16),
            pltpu.VMEM((S, DC), BF16),
            pltpu.VMEM((M * H // 2, D), jnp.uint32),
            pltpu.VMEM((DC * H // 2, D), jnp.uint32),
            pltpu.VMEM((DC * H // 2, D), jnp.uint32),
            pltpu.VMEM((H, D, M), BF16),
            pltpu.VMEM((FF, M), BF16),
            pltpu.VMEM((FF, M), BF16),
            pltpu.VMEM((FF, M), BF16),
            pltpu.VMEM((S, M), BF16),
            pltpu.VMEM((S, M), F32),
            pltpu.VMEM((S, D), BF16),
            pltpu.VMEM((S, D), BF16),
            pltpu.VMEM((S, D), BF16),
            pltpu.VMEM((S, M), BF16),
            pltpu.SemaphoreType.DMA((9,)),
        ],
        compiler_params=pltpu.CompilerParams(vmem_limit_bytes=100 * 1024 * 1024),
    )(
        A_x.reshape(S, M),
        A_c_kv.reshape(S, DC),
        A_w_q.reshape(M * H, D),
        A_w_uk.reshape(DC * H, D),
        A_w_uv.reshape(DC * H, D),
        A_w_o,
        B_w_r,
        B_w_gate.T,
        B_w_up.T,
        B_w_down,
    )
    return out.reshape(1, S, M)
```

```python
import math

import numpy as np
import jax
import jax.numpy as jnp
from jax import lax
import jax.experimental.pallas as pl
import jax.experimental.pallas.tpu as pltpu

BF16 = jnp.bfloat16
F32 = jnp.float32
TOPC = 8
LN_EPS = float(np.float32(np.asarray(1e-5, dtype=jnp.bfloat16)))
NEG = -1e30
T = 128
BQ = 128
CK = 4
PR = 128
AHEAD = 2
OR = 256


def _rb(v):
    return v.astype(BF16).astype(F32)


def _dot(a, b):
    return jnp.dot(a, b, preferred_element_type=F32)


def _dot_nt(a, b):
    return lax.dot_general(a, b, (((1,), (1,)), ((), ())), preferred_element_type=F32)


def _head_weight(w_ref, h, rows, n_heads):
    w32 = w_ref[pl.ds(h // 2, rows, stride=n_heads // 2), :]
    sh = (16 * (1 - h % 2)).astype(jnp.uint32)
    w32 = (w32 << sh) & jnp.uint32(0xFFFF0000)
    return pltpu.bitcast(w32, F32).astype(BF16)


def _interleave(*streams):
    events = []
    for k, (gen, n) in enumerate(streams):
        events += [((j + 0.5) / n, k) for j in range(n)]
    for _, k in sorted(events):
        next(streams[k][0])


def _kernel(x_hbm, c_hbm, wq_hbm, wuk_hbm, wuv_hbm, wo_hbm, wr_ref, wg_hbm, wu_hbm, wd_hbm,
            out_hbm,
            x_v, c_v, wq_v, wuk_v, wuv_v, wo_v, wg_v, wu_v, wd_v,
            xn_v, acc_v, q_v, k_v, v_v, wqh_v, wkvh_v, ctx_v, o_v, sems, osems):
    S, M = x_v.shape
    MT, CT = M // T, c_v.shape[0]
    DC = CT * T
    H, D = ctx_v.shape[0], ctx_v.shape[2]
    srcs = (x_hbm, wq_hbm.bitcast(jnp.uint32), wuk_hbm.bitcast(jnp.uint32),
            wuv_hbm.bitcast(jnp.uint32), wo_hbm, wg_hbm, wu_hbm, wd_hbm)
    dsts = (x_v, wq_v, wuk_v, wuv_v, wo_v, wg_v, wu_v, wd_v)
    cps = [pltpu.make_async_copy(s, d, sems.at[i]) for i, (s, d) in enumerate(zip(srcs, dsts))]
    ccps = [pltpu.make_async_copy(c_hbm.at[:, pl.ds(t * T, T)], c_v.at[t], sems.at[len(cps) + t])
            for t in range(CT)]
    cps[0].start()
    for cp in ccps:
        cp.start()
    for cp in cps[1:]:
        cp.start()

    cps[0].wait()
    wr = wr_ref[...].astype(F32).reshape(1, M)
    lane = lax.broadcasted_iota(jnp.int32, (8, T), 1)
    sub = lax.broadcasted_iota(jnp.int32, (8, T), 0)
    LB = 128
    rds = []
    for half in range(S // 1024):
        def ln_body(i, rd):
            r0 = pl.multiple_of(half * 1024 + i * LB, LB)
            xf = x_v[pl.ds(r0, LB), :].astype(F32)
            mean = jnp.sum(xf, axis=-1, keepdims=True) / M
            cen = xf - mean
            var = jnp.sum(cen * cen, axis=-1, keepdims=True) / M
            den = _rb(jnp.sqrt(_rb(_rb(var) + LN_EPS)))
            xn = _rb(_rb(xf - _rb(mean)) * (1.0 / den))
            for t in range(MT):
                xn_v[t, pl.ds(r0, LB), :] = xn[:, t * T:(t + 1) * T].astype(BF16)
            acc_v[pl.ds(r0, LB), :] = xf + xn
            r = jnp.sum(xn * wr, axis=-1, keepdims=True)
            for g in range(LB // 8):
                rd = jnp.where(lane == i * (LB // 8) + g, r[g * 8:(g + 1) * 8, :], rd)
            return rd
        rds.append(lax.fori_loop(0, 1024 // LB, ln_body, jnp.zeros((8, T), F32)))

    keys = []
    for half, rd in enumerate(rds):
        bits = pltpu.bitcast(_rb(rd), jnp.int32) >> 16
        mag = bits & 0x7FFF
        order = jnp.where(bits < 0, 0x8000 - mag, 0x8000 + mag)
        order = jnp.where(mag > 0x7F80, 0, order)
        row = half * 1024 + lane * 8 + sub
        keys.append(order * S + (S - 1 - row))
    sel_keys = []
    for _ in range(TOPC):
        mx = keys[0]
        for kk in keys[1:]:
            mx = jnp.maximum(mx, kk)
        top = jnp.max(mx)
        sel_keys.append(top)
        keys = [jnp.where(kk == top, -1, kk) for kk in keys]

    for cp in ccps + cps[1:4]:
        cp.wait()
    qscale = (D ** -0.5) * math.log2(math.e)
    NB = S // BQ
    NP = S // PR

    def load_weights(h):
        wqh_v[...] = _head_weight(wq_v, h, M, H)
        wkvh_v[:, 0:D] = _head_weight(wuk_v, h, DC, H)
        wkvh_v[:, D:2 * D] = _head_weight(wuv_v, h, DC, H)

    def project(i):
        rows = slice(i * PR, (i + 1) * PR)
        xn = jnp.concatenate([xn_v[t, rows, :] for t in range(MT)], axis=1)
        q_v[rows, :] = (_dot(xn, wqh_v[...]) * qscale).astype(BF16)
        yield
        c = jnp.concatenate([c_v[t, rows, :] for t in range(CT)], axis=1)
        k_v[rows, :] = _dot(c, wkvh_v[:, 0:D]).astype(BF16)
        yield
        v_v[rows, :] = _dot(c, wkvh_v[:, D:2 * D]).astype(BF16)
        yield

    def chunks(i):
        nk = -(-(i + 1) * BQ // T)
        return [(t, min(CK, nk - t)) for t in range(0, nk, CK)]

    def scores(i, st):
        r0 = i * BQ
        q = q_v[r0:r0 + BQ, :]
        mp = None
        st["s"] = []
        for t, n in chunks(i):
            s = _dot_nt(q, k_v[t * T:(t + n) * T, :])
            for j in range(n):
                sj = s[:, j * T:(j + 1) * T]
                k0 = (t + j) * T
                if k0 + T - 1 > r0:
                    row = lax.broadcasted_iota(jnp.int32, (BQ, T), 0)
                    col = lax.broadcasted_iota(jnp.int32, (BQ, T), 1)
                    sj = jnp.where(col + (k0 - r0) <= row, sj, NEG)
                st["s"].append(sj)
                mp = sj if mp is None else jnp.maximum(mp, sj)
            if t + n == chunks(i)[-1][0] + chunks(i)[-1][1]:
                st["m"] = jnp.max(mp, axis=-1, keepdims=True)
            yield

    def context(i, h, st):
        lp = None
        o = None
        for t, n in chunks(i):
            ps = []
            for j in range(n):
                p = jnp.exp2(st["s"][t + j] - st["m"])
                lp = p if lp is None else lp + p
                ps.append(p.astype(BF16))
            pv = _dot(jnp.concatenate(ps, axis=1) if n > 1 else ps[0], v_v[t * T:(t + n) * T, :])
            o = pv if o is None else o + pv
            if t + n == chunks(i)[-1][0] + chunks(i)[-1][1]:
                l = jnp.sum(lp, axis=-1, keepdims=True)
                inv = pl.reciprocal(l, approx=True)
                inv = inv * (2.0 - l * inv)
                ctx_v[h, i * BQ:(i + 1) * BQ, :] = (o * inv).astype(BF16)
            yield

    def chain(*gens):
        for g in gens:
            yield from g

    load_weights(jnp.int32(0))
    for i in range(AHEAD):
        for _ in project(i):
            pass

    def head_body(h, carry):
        prev = None
        done = AHEAD
        for i in range(NB):
            st = {}
            streams = [(scores(i, st), len(chunks(i)))]
            if prev is not None:
                streams.append((context(i - 1, h, prev), len(chunks(i - 1))))
            want = min(NP, -(-(i + 1) * BQ // PR) + AHEAD)
            if want > done:
                streams.append((chain(*[project(p) for p in range(done, want)]), 3 * (want - done)))
                done = want
            if i == NB - 1:
                load_weights(jnp.minimum(h + 1, H - 1))
            _interleave(*streams)
            prev = st
        last = context(NB - 1, h, prev)
        nlast = len(chunks(NB - 1))
        for _ in range(-(-AHEAD * PR // (CK * T))):
            next(last)
            nlast -= 1
        _interleave((last, nlast), (chain(*[project(p) for p in range(AHEAD)]), 3 * AHEAD))
        return carry

    lax.fori_loop(0, H, head_body, 0)

    sub16 = lax.broadcasted_iota(jnp.int32, (16, M), 0)
    sub8m = lax.broadcasted_iota(jnp.int32, (TOPC, M), 0)
    xs = jnp.zeros((TOPC, M), F32)
    key_col = jnp.zeros((TOPC, T), jnp.int32)
    rows = []
    for j, top in enumerate(sel_keys):
        row = S - 1 - (top % S)
        rows.append(row)
        base = pl.multiple_of((row // 16) * 16, 16)
        tile = jnp.concatenate([xn_v[t, pl.ds(base, 16), :] for t in range(MT)], axis=1).astype(F32)
        one = jnp.sum(jnp.where(sub16 == row % 16, tile, 0.0), axis=0, keepdims=True)
        xs = jnp.where(sub8m == j, one, xs)
        key_col = jnp.where(sub == j, top, key_col)
    order = key_col // S
    bits = jnp.where(order >= 0x8000, order - 0x8000, (0x8000 - order) | 0x8000)
    bits = jnp.where(order == 0, 0x7FC0, bits)
    r_sel = pltpu.bitcast(bits << 16, F32)[:, 0:1]
    for cp in cps[4:]:
        cp.wait()
    xs = xs.astype(BF16)
    g = _dot_nt(xs, wg_v[...])
    u = _dot_nt(xs, wu_v[...])
    hid = (g * jax.nn.sigmoid(g) * u).astype(BF16)
    y = _dot(hid, wd_v[...]) * jax.nn.sigmoid(r_sel)
    for j, row in enumerate(rows):
        acc_v[pl.ds(row, 1), :] += y[j:j + 1, :]

    def out_copy(i):
        r0 = pl.multiple_of(i * OR, OR)
        return pltpu.make_async_copy(o_v.at[pl.ds(r0, OR)], out_hbm.at[pl.ds(r0, OR)], osems.at[i])

    def out_body(i, carry):
        r0 = pl.multiple_of(i * OR, OR)
        ctx = jnp.concatenate([ctx_v[h, pl.ds(r0, OR), :] for h in range(H)], axis=1)
        o_v[pl.ds(r0, OR), :] = (acc_v[pl.ds(r0, OR), :] + _dot(ctx, wo_v[...])).astype(BF16)
        out_copy(i).start()
        return carry

    lax.fori_loop(0, S // OR, out_body, 0)
    for i in range(S // OR):
        out_copy(i).wait()


@jax.jit
def pallas_parallel_sum__compressed_kv_cla__moe_arch_mod__prompt_kernel(
    A_x: jax.Array,
    A_c_kv: jax.Array,
    A_w_q: jax.Array,
    A_w_uk: jax.Array,
    A_w_uv: jax.Array,
    A_w_o: jax.Array,
    B_x: jax.Array,
    B_w_r: jax.Array,
    B_w_gate: jax.Array,
    B_w_up: jax.Array,
    B_w_down: jax.Array,
):
    del B_x
    _, S, M = A_x.shape
    DC = A_c_kv.shape[2]
    H, D = A_w_q.shape[1], A_w_q.shape[2]
    FF = B_w_gate.shape[1]
    hbm = pl.BlockSpec(memory_space=pltpu.HBM)
    out = pl.pallas_call(
        _kernel,
        out_shape=jax.ShapeDtypeStruct((S, M), A_x.dtype),
        in_specs=[hbm] * 6 + [pl.BlockSpec(memory_space=pltpu.VMEM)] + [hbm] * 3,
        out_specs=hbm,
        scratch_shapes=[
            pltpu.VMEM((S, M), BF16),
            pltpu.VMEM((DC // T, S, T), BF16),
            pltpu.VMEM((M * H // 2, D), jnp.uint32),
            pltpu.VMEM((DC * H // 2, D), jnp.uint32),
            pltpu.VMEM((DC * H // 2, D), jnp.uint32),
            pltpu.VMEM((H * D, M), BF16),
            pltpu.VMEM((FF, M), BF16),
            pltpu.VMEM((FF, M), BF16),
            pltpu.VMEM((FF, M), BF16),
            pltpu.VMEM((M // T, S, T), BF16),
            pltpu.VMEM((S, M), F32),
            pltpu.VMEM((S, D), BF16),
            pltpu.VMEM((S, D), BF16),
            pltpu.VMEM((S, D), BF16),
            pltpu.VMEM((M, D), BF16),
            pltpu.VMEM((DC, 2 * D), BF16),
            pltpu.VMEM((H, S, D), BF16),
            pltpu.VMEM((S, M), BF16),
            pltpu.SemaphoreType.DMA((8 + DC // T,)),
            pltpu.SemaphoreType.DMA((S // OR,)),
        ],
        compiler_params=pltpu.CompilerParams(vmem_limit_bytes=110 * 1024 * 1024),
    )(
        A_x.reshape(S, M),
        A_c_kv.reshape(S, DC),
        A_w_q.reshape(M * H, D),
        A_w_uk.reshape(DC * H, D),
        A_w_uv.reshape(DC * H, D),
        A_w_o.reshape(H * D, M),
        B_w_r,
        B_w_gate.T,
        B_w_up.T,
        B_w_down,
    )
    return out.reshape(1, S, M)
```

```python
import math

import numpy as np
import jax
import jax.numpy as jnp
from jax import lax
import jax.experimental.pallas as pl
import jax.experimental.pallas.tpu as pltpu

BF16 = jnp.bfloat16
F32 = jnp.float32
U32 = jnp.uint32
TIE = 0
TOPC = 8
LN_EPS = float(np.float32(np.asarray(1e-5, dtype=jnp.bfloat16)))
NEG = -1e30
T = 128
BQ = 128
CK = 4
PR = 128
WPB = 3
AHEAD = 2
OR = 256


def _rb(v):
    return v.astype(BF16).astype(F32)


def _dot(a, b):
    return jnp.dot(a, b, preferred_element_type=F32)


def _dot_nt(a, b):
    return lax.dot_general(a, b, (((1,), (1,)), ((), ())), preferred_element_type=F32)


def _head_weight(w_ref, h, t, n_heads):
    w32 = w_ref[pl.ds(t * T * (n_heads // 2) + h // 2, T, stride=n_heads // 2), :]
    sh = (16 * (1 - h % 2)).astype(jnp.uint32)
    w32 = (w32 << sh) & jnp.uint32(0xFFFF0000)
    return pltpu.bitcast(w32, F32).astype(BF16)


def _ld(ref, r0, n, *lead):
    return pltpu.bitcast(ref[(*lead, pl.ds(r0 // 2, n // 2), slice(None))], BF16)


def _st(ref, r0, val, *lead):
    n = val.shape[0]
    ref[(*lead, pl.ds(r0 // 2, n // 2), slice(None))] = pltpu.bitcast(val.astype(BF16), U32)


def _tree(op, xs):
    while len(xs) > 1:
        xs = [op(xs[i], xs[i + 1]) if i + 1 < len(xs) else xs[i] for i in range(0, len(xs), 2)]
    return xs[0]


def _interleave(*streams):
    events = []
    for k, (gen, n) in enumerate(streams):
        events += [((j + 0.5) / n, k) for j in range(n)]
    for _, k in sorted(events):
        next(streams[k][0])


def _kernel(x_hbm, c_hbm, wq_hbm, wuk_hbm, wuv_hbm, wo_hbm, wr_ref, wg_hbm, wu_hbm, wd_hbm,
            out_hbm,
            x_v, c_v, wq_v, wuk_v, wuv_v, wo_v, wg_v, wu_v, wd_v,
            xn_v, acc_v, q_v, k_v, v_v, wh_v, ctx_v, o_v, sems, osems):
    S, M = x_v.shape
    MT, CT = M // T, c_v.shape[0]
    DC = CT * T
    H, D = ctx_v.shape[0], ctx_v.shape[2]
    srcs = (x_hbm, wq_hbm.bitcast(jnp.uint32), wuk_hbm.bitcast(jnp.uint32),
            wuv_hbm.bitcast(jnp.uint32), wo_hbm, wg_hbm, wu_hbm, wd_hbm)
    dsts = (x_v, wq_v, wuk_v, wuv_v, wo_v, wg_v, wu_v, wd_v)
    cps = [pltpu.make_async_copy(s, d, sems.at[i]) for i, (s, d) in enumerate(zip(srcs, dsts))]
    ccps = [pltpu.make_async_copy(c_hbm.bitcast(U32).at[:, pl.ds(t * T, T)], c_v.at[t], sems.at[len(cps) + t])
            for t in range(CT)]
    cps[0].start()
    for cp in ccps:
        cp.start()
    for cp in cps[1:]:
        cp.start()

    cps[0].wait()
    wr = wr_ref[...].astype(F32).reshape(1, M)
    lane = lax.broadcasted_iota(jnp.int32, (8, T), 1)
    sub = lax.broadcasted_iota(jnp.int32, (8, T), 0)
    LB = 128
    rds = []
    for half in range(S // 1024):
        def ln_body(i, rd):
            r0 = pl.multiple_of(half * 1024 + i * LB, LB)
            rp = pl.multiple_of(half * 512 + i * (LB // 2), LB // 2)
            xf = x_v[pl.ds(r0, LB), :].astype(F32)
            mean = jnp.sum(xf, axis=-1, keepdims=True) / M
            cen = xf - mean
            var = jnp.sum(cen * cen, axis=-1, keepdims=True) / M
            den = _rb(jnp.sqrt(_rb(_rb(var) + LN_EPS)))
            xn = _rb(_rb(xf - _rb(mean)) * (1.0 / den))
            for t in range(MT):
                xn_v[t, pl.ds(rp, LB // 2), :] = pltpu.bitcast(xn[:, t * T:(t + 1) * T].astype(BF16), U32)
            acc_v[pl.ds(r0, LB), :] = xf + xn
            r = jnp.sum(xn * wr, axis=-1, keepdims=True)
            for g in range(LB // 8):
                rd = jnp.where(lane == i * (LB // 8) + g, r[g * 8:(g + 1) * 8, :], rd)
            return rd
        rds.append(lax.fori_loop(0, 1024 // LB, ln_body, jnp.zeros((8, T), F32)))

    keys = []
    for half, rd in enumerate(rds):
        bits = pltpu.bitcast(_rb(rd), jnp.int32) >> 16
        mag = bits & 0x7FFF
        order = jnp.where(bits < 0, 0x8000 - mag, 0x8000 + mag)
        order = jnp.where(mag > 0x7F80, 0, order)
        row = half * 1024 + lane * 8 + sub
        keys.append(order * S + (S - 1 - row))
    sel_keys = []
    for _ in range(TOPC):
        mx = keys[0]
        for kk in keys[1:]:
            mx = jnp.maximum(mx, kk)
        top = jnp.max(mx)
        sel_keys.append(top)
        keys = [jnp.where(kk == top, -1, kk) for kk in keys]

    for cp in ccps + cps[1:4]:
        cp.wait()
    qscale = (D ** -0.5) * math.log2(math.e)
    NB = S // BQ
    NP = S // PR

    def load_weights(h, slot):
        r = 0
        for w_v, rows in ((wq_v, M), (wuk_v, DC), (wuv_v, DC)):
            for t in range(rows // T):
                _st(wh_v, r, _head_weight(w_v, h, t, H), slot)
                r += T
                yield

    def project(i, slot):
        r0 = i * PR
        xn = jnp.concatenate([_ld(xn_v, r0, PR, t) for t in range(MT)], axis=1)
        _st(q_v, r0, _dot(xn, _ld(wh_v, 0, M, slot)) * qscale)
        yield
        c = jnp.concatenate([_ld(c_v, r0, PR, t) for t in range(CT)], axis=1)
        _st(k_v, r0, _dot(c, _ld(wh_v, M, DC, slot)))
        yield
        c = jnp.concatenate([_ld(c_v, r0, PR, t) for t in range(CT)], axis=1)
        _st(v_v, r0, _dot(c, _ld(wh_v, M + DC, DC, slot)))
        yield

    def chunks(i):
        nk = -(-(i + 1) * BQ // T)
        return [(t, min(CK, nk - t)) for t in range(0, nk, CK)]

    def scores(i, st):
        r0 = i * BQ
        mp = None
        st["s"] = []
        for t, n in chunks(i):
            s = _dot_nt(_ld(q_v, r0, BQ), _ld(k_v, t * T, n * T))
            tiles = []
            for j in range(n):
                sj = s[:, j * T:(j + 1) * T]
                k0 = (t + j) * T
                if k0 + T - 1 > r0:
                    row = lax.broadcasted_iota(jnp.int32, (BQ, T), 0)
                    col = lax.broadcasted_iota(jnp.int32, (BQ, T), 1)
                    sj = jnp.where(col + (k0 - r0) <= row, sj, NEG)
                tiles.append(sj)
            st["s"].append(jnp.concatenate(tiles, axis=1) if n > 1 else tiles[0])
            mp = _tree(jnp.maximum, tiles if mp is None else tiles + [mp])
            if (t, n) == chunks(i)[-1]:
                st["m"] = jnp.max(mp, axis=-1, keepdims=True)
            yield

    link = {}

    def context(i, h, st):
        lp = None
        o = None
        tie = link.get("tie")
        for ci, (t, n) in enumerate(chunks(i)):
            m = st["m"]
            d = st["s"][ci] - m
            if TIE and tie is not None:
                d0 = jnp.minimum(d[:, 0:T], tie)
                d = jnp.concatenate([d0, d[:, T:]], axis=1) if n > 1 else d0
            p = jnp.exp2(d)
            ps = _tree(jnp.add, [p[:, j * T:(j + 1) * T] for j in range(n)])
            lp = ps if lp is None else lp + ps
            pv = _dot(p.astype(BF16), _ld(v_v, t * T, n * T))
            o = pv if o is None else o + pv
            if TIE > 1:
                tie = lp
            else:
                tie = None
            if (t, n) == chunks(i)[-1]:
                l = jnp.sum(lp, axis=-1, keepdims=True)
                inv = pl.reciprocal(l, approx=True)
                inv = inv * (2.0 - l * inv)
                o = o * inv
                link["tie"] = jnp.abs(o)
                _st(ctx_v, i * BQ, o, h)
            yield

    def chain(*gens):
        for g in gens:
            yield from g

    for _ in load_weights(jnp.int32(0), 0):
        pass
    for i in range(AHEAD):
        for _ in project(i, 0):
            pass

    def head_body(h, carry):
        prev = None
        done = AHEAD
        wnext = load_weights(jnp.minimum(h + 1, H - 1), 1 - h % 2)
        wleft = (M + 2 * DC) // T
        for i in range(NB):
            st = {}
            streams = [(scores(i, st), len(chunks(i)))]
            if prev is not None:
                streams.append((context(i - 1, h, prev), len(chunks(i - 1))))
            want = min(NP, -(-(i + 1) * BQ // PR) + AHEAD)
            if want > done:
                streams.append((chain(*[project(p, h % 2) for p in range(done, want)]), 3 * (want - done)))
                done = want
            nw = min(WPB, wleft)
            if nw:
                streams.append((wnext, nw))
                wleft -= nw
            _interleave(*streams)
            prev = st
        last = context(NB - 1, h, prev)
        nlast = len(chunks(NB - 1))
        for _ in range(-(-AHEAD * PR // (CK * T))):
            next(last)
            nlast -= 1
        _interleave((last, nlast), (chain(*[project(p, 1 - h % 2) for p in range(AHEAD)]), 3 * AHEAD))
        return carry

    lax.fori_loop(0, H, head_body, 0)

    sub16 = lax.broadcasted_iota(jnp.int32, (16, M), 0)
    sub8m = lax.broadcasted_iota(jnp.int32, (TOPC, M), 0)
    xs = jnp.zeros((TOPC, M), F32)
    key_col = jnp.zeros((TOPC, T), jnp.int32)
    rows = []
    for j, top in enumerate(sel_keys):
        row = S - 1 - (top % S)
        rows.append(row)
        base = pl.multiple_of((row // 16) * 8, 8)
        tile = jnp.concatenate(
            [pltpu.bitcast(xn_v[t, pl.ds(base, 8), :], BF16) for t in range(MT)], axis=1).astype(F32)
        one = jnp.sum(jnp.where(sub16 == row % 16, tile, 0.0), axis=0, keepdims=True)
        xs = jnp.where(sub8m == j, one, xs)
        key_col = jnp.where(sub == j, top, key_col)
    order = key_col // S
    bits = jnp.where(order >= 0x8000, order - 0x8000, (0x8000 - order) | 0x8000)
    bits = jnp.where(order == 0, 0x7FC0, bits)
    r_sel = pltpu.bitcast(bits << 16, F32)[:, 0:1]
    for cp in cps[4:]:
        cp.wait()
    xs = xs.astype(BF16)
    g = _dot_nt(xs, wg_v[...])
    u = _dot_nt(xs, wu_v[...])
    hid = (g * jax.nn.sigmoid(g) * u).astype(BF16)
    y = _dot(hid, wd_v[...]) * jax.nn.sigmoid(r_sel)
    for j, row in enumerate(rows):
        acc_v[pl.ds(row, 1), :] += y[j:j + 1, :]

    def out_copy(i):
        r0 = pl.multiple_of(i * OR, OR)
        return pltpu.make_async_copy(o_v.at[pl.ds(r0, OR)], out_hbm.at[pl.ds(r0, OR)], osems.at[i])

    def out_body(i, carry):
        r0 = pl.multiple_of(i * OR, OR)
        rp = pl.multiple_of(i * (OR // 2), OR // 2)
        ctx = jnp.concatenate(
            [pltpu.bitcast(ctx_v[h, pl.ds(rp, OR // 2), :], BF16) for h in range(H)], axis=1)
        o_v[pl.ds(r0, OR), :] = (acc_v[pl.ds(r0, OR), :] + _dot(ctx, wo_v[...])).astype(BF16)
        out_copy(i).start()
        return carry

    lax.fori_loop(0, S // OR, out_body, 0)
    for i in range(S // OR):
        out_copy(i).wait()


@jax.jit
def pallas_parallel_sum__compressed_kv_cla__moe_arch_mod__prompt_kernel(
    A_x: jax.Array,
    A_c_kv: jax.Array,
    A_w_q: jax.Array,
    A_w_uk: jax.Array,
    A_w_uv: jax.Array,
    A_w_o: jax.Array,
    B_x: jax.Array,
    B_w_r: jax.Array,
    B_w_gate: jax.Array,
    B_w_up: jax.Array,
    B_w_down: jax.Array,
):
    del B_x
    _, S, M = A_x.shape
    DC = A_c_kv.shape[2]
    H, D = A_w_q.shape[1], A_w_q.shape[2]
    FF = B_w_gate.shape[1]
    hbm = pl.BlockSpec(memory_space=pltpu.HBM)
    out = pl.pallas_call(
        _kernel,
        out_shape=jax.ShapeDtypeStruct((S, M), A_x.dtype),
        in_specs=[hbm] * 6 + [pl.BlockSpec(memory_space=pltpu.VMEM)] + [hbm] * 3,
        out_specs=hbm,
        scratch_shapes=[
            pltpu.VMEM((S, M), BF16),
            pltpu.VMEM((DC // T, S // 2, T), U32),
            pltpu.VMEM((M * H // 2, D), jnp.uint32),
            pltpu.VMEM((DC * H // 2, D), jnp.uint32),
            pltpu.VMEM((DC * H // 2, D), jnp.uint32),
            pltpu.VMEM((H * D, M), BF16),
            pltpu.VMEM((FF, M), BF16),
            pltpu.VMEM((FF, M), BF16),
            pltpu.VMEM((FF, M), BF16),
            pltpu.VMEM((M // T, S // 2, T), U32),
            pltpu.VMEM((S, M), F32),
            pltpu.VMEM((S // 2, D), U32),
            pltpu.VMEM((S // 2, D), U32),
            pltpu.VMEM((S // 2, D), U32),
            pltpu.VMEM((2, (M + 2 * DC) // 2, D), U32),
            pltpu.VMEM((H, S // 2, D), U32),
            pltpu.VMEM((S, M), BF16),
            pltpu.SemaphoreType.DMA((8 + DC // T,)),
            pltpu.SemaphoreType.DMA((S // OR,)),
        ],
        compiler_params=pltpu.CompilerParams(vmem_limit_bytes=110 * 1024 * 1024),
    )(
        A_x.reshape(S, M),
        A_c_kv.reshape(S, DC),
        A_w_q.reshape(M * H, D),
        A_w_uk.reshape(DC * H, D),
        A_w_uv.reshape(DC * H, D),
        A_w_o.reshape(H * D, M),
        B_w_r,
        B_w_gate.T,
        B_w_up.T,
        B_w_down,
    )
    return out.reshape(1, S, M)
```

```python
import math

import numpy as np
import jax
import jax.numpy as jnp
from jax import lax
import jax.experimental.pallas as pl
import jax.experimental.pallas.tpu as pltpu

BF16 = jnp.bfloat16
F32 = jnp.float32
U32 = jnp.uint32
TIE = 0
HG = 2
TOPC = 8
LN_EPS = float(np.float32(np.asarray(1e-5, dtype=jnp.bfloat16)))
NEG = -1e30
T = 128
BQ = 128
CK = 4
PR = 128
WPB = 3
AHEAD = 2
OR = 256


def _rb(v):
    return v.astype(BF16).astype(F32)


def _dot(a, b):
    return jnp.dot(a, b, preferred_element_type=F32)


def _dot_nt(a, b):
    return lax.dot_general(a, b, (((1,), (1,)), ((), ())), preferred_element_type=F32)


def _head_weight(w_ref, h, t, n_heads):
    w32 = w_ref[h // 2, pl.ds(t * T, T), :]
    sh = (16 * (1 - h % 2)).astype(jnp.uint32)
    w32 = (w32 << sh) & jnp.uint32(0xFFFF0000)
    return pltpu.bitcast(w32, F32).astype(BF16)


def _ld(ref, r0, n, *lead):
    return pltpu.bitcast(ref[(*lead, pl.ds(r0 // 2, n // 2), slice(None))], BF16)


def _st(ref, r0, val, *lead):
    n = val.shape[0]
    ref[(*lead, pl.ds(r0 // 2, n // 2), slice(None))] = pltpu.bitcast(val.astype(BF16), U32)


def _tree(op, xs):
    while len(xs) > 1:
        xs = [op(xs[i], xs[i + 1]) if i + 1 < len(xs) else xs[i] for i in range(0, len(xs), 2)]
    return xs[0]


def _interleave(*streams):
    events = []
    for k, (gen, n) in enumerate(streams):
        events += [((j + 0.5) / n, k) for j in range(n)]
    for _, k in sorted(events):
        next(streams[k][0])


def _kernel(x_hbm, c_hbm, wq_hbm, wuk_hbm, wuv_hbm, wo_hbm, wr_ref, wg_hbm, wu_hbm, wd_hbm,
            out_hbm,
            x_v, c_v, wq_v, wuk_v, wuv_v, wo_v, wg_v, wu_v, wd_v,
            xn_v, acc_v, q_v, k_v, v_v, wh_v, ctx_v, o_v, sems, wsems, osems):
    S, M = x_v.shape
    MT, CT = M // T, c_v.shape[0]
    DC = CT * T
    H, D = ctx_v.shape[0], ctx_v.shape[2]
    NG = H // HG
    xcp = pltpu.make_async_copy(x_hbm, x_v, sems.at[0])
    ccps = [pltpu.make_async_copy(c_hbm.bitcast(U32).at[:, pl.ds(t * T, T)], c_v.at[t], sems.at[1 + t])
            for t in range(CT)]
    late = [pltpu.make_async_copy(s, d, sems.at[1 + CT + i]) for i, (s, d) in enumerate(
        ((wg_hbm, wg_v), (wu_hbm, wu_v), (wd_hbm, wd_v), (wo_hbm, wo_v)))]

    def wcps(g):
        return [pltpu.make_async_copy(src.bitcast(U32).at[:, g, :],
                                      dst.at[g], wsems.at[3 * g + i])
                for i, (src, dst) in enumerate(((wq_hbm, wq_v), (wuk_hbm, wuk_v), (wuv_hbm, wuv_v)))]

    xcp.start()
    for cp in ccps + wcps(0):
        cp.start()

    xcp.wait()
    wr = wr_ref[...].astype(F32).reshape(1, M)
    lane = lax.broadcasted_iota(jnp.int32, (8, T), 1)
    sub = lax.broadcasted_iota(jnp.int32, (8, T), 0)
    LB = 128
    rds = []
    for half in range(S // 1024):
        def ln_body(i, rd):
            r0 = pl.multiple_of(half * 1024 + i * LB, LB)
            rp = pl.multiple_of(half * 512 + i * (LB // 2), LB // 2)
            xf = x_v[pl.ds(r0, LB), :].astype(F32)
            mean = jnp.sum(xf, axis=-1, keepdims=True) / M
            cen = xf - mean
            var = jnp.sum(cen * cen, axis=-1, keepdims=True) / M
            den = _rb(jnp.sqrt(_rb(_rb(var) + LN_EPS)))
            xn = _rb(_rb(xf - _rb(mean)) * (1.0 / den))
            for t in range(MT):
                xn_v[t, pl.ds(rp, LB // 2), :] = pltpu.bitcast(xn[:, t * T:(t + 1) * T].astype(BF16), U32)
            acc_v[pl.ds(r0, LB), :] = xf + xn
            r = jnp.sum(xn * wr, axis=-1, keepdims=True)
            for g in range(LB // 8):
                rd = jnp.where(lane == i * (LB // 8) + g, r[g * 8:(g + 1) * 8, :], rd)
            return rd
        rds.append(lax.fori_loop(0, 1024 // LB, ln_body, jnp.zeros((8, T), F32)))

    keys = []
    for half, rd in enumerate(rds):
        bits = pltpu.bitcast(_rb(rd), jnp.int32) >> 16
        mag = bits & 0x7FFF
        order = jnp.where(bits < 0, 0x8000 - mag, 0x8000 + mag)
        order = jnp.where(mag > 0x7F80, 0, order)
        row = half * 1024 + lane * 8 + sub
        keys.append(order * S + (S - 1 - row))
    sel_keys = []
    for _ in range(TOPC):
        mx = keys[0]
        for kk in keys[1:]:
            mx = jnp.maximum(mx, kk)
        top = jnp.max(mx)
        sel_keys.append(top)
        keys = [jnp.where(kk == top, -1, kk) for kk in keys]

    for cp in ccps + wcps(0):
        cp.wait()
    for g in range(1, NG):
        for cp in wcps(g):
            cp.start()
    for cp in late:
        cp.start()
    qscale = (D ** -0.5) * math.log2(math.e)
    NB = S // BQ
    NP = S // PR

    def load_weights(h, slot):
        r = 0
        for w_v, rows in ((wq_v, M), (wuk_v, DC), (wuv_v, DC)):
            for t in range(rows // T):
                _st(wh_v, r, _head_weight(w_v, h, t, H), slot)
                r += T
                yield

    def project(i, slot):
        r0 = i * PR
        xn = jnp.concatenate([_ld(xn_v, r0, PR, t) for t in range(MT)], axis=1)
        _st(q_v, r0, _dot(xn, _ld(wh_v, 0, M, slot)) * qscale)
        yield
        c = jnp.concatenate([_ld(c_v, r0, PR, t) for t in range(CT)], axis=1)
        _st(k_v, r0, _dot(c, _ld(wh_v, M, DC, slot)))
        yield
        c = jnp.concatenate([_ld(c_v, r0, PR, t) for t in range(CT)], axis=1)
        _st(v_v, r0, _dot(c, _ld(wh_v, M + DC, DC, slot)))
        yield

    def chunks(i):
        nk = -(-(i + 1) * BQ // T)
        return [(t, min(CK, nk - t)) for t in range(0, nk, CK)]

    def scores(i, st):
        r0 = i * BQ
        mp = None
        st["s"] = []
        for t, n in chunks(i):
            s = _dot_nt(_ld(q_v, r0, BQ), _ld(k_v, t * T, n * T))
            tiles = []
            for j in range(n):
                sj = s[:, j * T:(j + 1) * T]
                k0 = (t + j) * T
                if k0 + T - 1 > r0:
                    row = lax.broadcasted_iota(jnp.int32, (BQ, T), 0)
                    col = lax.broadcasted_iota(jnp.int32, (BQ, T), 1)
                    sj = jnp.where(col + (k0 - r0) <= row, sj, NEG)
                tiles.append(sj)
            st["s"].append(jnp.concatenate(tiles, axis=1) if n > 1 else tiles[0])
            mp = _tree(jnp.maximum, tiles if mp is None else tiles + [mp])
            if (t, n) == chunks(i)[-1]:
                st["m"] = jnp.max(mp, axis=-1, keepdims=True)
            yield

    link = {}

    def context(i, h, st):
        lp = None
        o = None
        tie = link.get("tie")
        for ci, (t, n) in enumerate(chunks(i)):
            m = st["m"]
            d = st["s"][ci] - m
            if TIE and tie is not None:
                d0 = jnp.minimum(d[:, 0:T], tie)
                d = jnp.concatenate([d0, d[:, T:]], axis=1) if n > 1 else d0
            p = jnp.exp2(d)
            ps = _tree(jnp.add, [p[:, j * T:(j + 1) * T] for j in range(n)])
            lp = ps if lp is None else lp + ps
            pv = _dot(p.astype(BF16), _ld(v_v, t * T, n * T))
            o = pv if o is None else o + pv
            if TIE > 1:
                tie = lp
            else:
                tie = None
            if (t, n) == chunks(i)[-1]:
                l = jnp.sum(lp, axis=-1, keepdims=True)
                inv = pl.reciprocal(l, approx=True)
                inv = inv * (2.0 - l * inv)
                o = o * inv
                link["tie"] = jnp.abs(o)
                _st(ctx_v, i * BQ, o, h)
            yield

    def chain(*gens):
        for g in gens:
            yield from g

    for _ in load_weights(jnp.int32(0), 0):
        pass
    for i in range(AHEAD):
        for _ in project(i, 0):
            pass

    def head_body(h, carry):
        @pl.when(jnp.logical_and(h % 2 == 1, h < H - 1))
        def _():
            for cp in wcps((h + 1) // 2):
                cp.wait()

        prev = None
        done = AHEAD
        wnext = load_weights(jnp.minimum(h + 1, H - 1), 1 - h % 2)
        wleft = (M + 2 * DC) // T
        for i in range(NB):
            st = {}
            streams = [(scores(i, st), len(chunks(i)))]
            if prev is not None:
                streams.append((context(i - 1, h, prev), len(chunks(i - 1))))
            want = min(NP, -(-(i + 1) * BQ // PR) + AHEAD)
            if want > done:
                streams.append((chain(*[project(p, h % 2) for p in range(done, want)]), 3 * (want - done)))
                done = want
            nw = min(WPB, wleft)
            if nw:
                streams.append((wnext, nw))
                wleft -= nw
            _interleave(*streams)
            prev = st
        last = context(NB - 1, h, prev)
        nlast = len(chunks(NB - 1))
        for _ in range(-(-AHEAD * PR // (CK * T))):
            next(last)
            nlast -= 1
        _interleave((last, nlast), (chain(*[project(p, 1 - h % 2) for p in range(AHEAD)]), 3 * AHEAD))
        return carry

    lax.fori_loop(0, H, head_body, 0)

    sub16 = lax.broadcasted_iota(jnp.int32, (16, M), 0)
    sub8m = lax.broadcasted_iota(jnp.int32, (TOPC, M), 0)
    xs = jnp.zeros((TOPC, M), F32)
    key_col = jnp.zeros((TOPC, T), jnp.int32)
    rows = []
    for j, top in enumerate(sel_keys):
        row = S - 1 - (top % S)
        rows.append(row)
        base = pl.multiple_of((row // 16) * 8, 8)
        tile = jnp.concatenate(
            [pltpu.bitcast(xn_v[t, pl.ds(base, 8), :], BF16) for t in range(MT)], axis=1).astype(F32)
        one = jnp.sum(jnp.where(sub16 == row % 16, tile, 0.0), axis=0, keepdims=True)
        xs = jnp.where(sub8m == j, one, xs)
        key_col = jnp.where(sub == j, top, key_col)
    order = key_col // S
    bits = jnp.where(order >= 0x8000, order - 0x8000, (0x8000 - order) | 0x8000)
    bits = jnp.where(order == 0, 0x7FC0, bits)
    r_sel = pltpu.bitcast(bits << 16, F32)[:, 0:1]
    for cp in late:
        cp.wait()
    xs = xs.astype(BF16)
    g = _dot_nt(xs, wg_v[...])
    u = _dot_nt(xs, wu_v[...])
    hid = (g * jax.nn.sigmoid(g) * u).astype(BF16)
    y = _dot(hid, wd_v[...]) * jax.nn.sigmoid(r_sel)
    for j, row in enumerate(rows):
        acc_v[pl.ds(row, 1), :] += y[j:j + 1, :]

    def out_copy(i):
        r0 = pl.multiple_of(i * OR, OR)
        return pltpu.make_async_copy(o_v.at[pl.ds(r0, OR)], out_hbm.at[pl.ds(r0, OR)], osems.at[i])

    def out_body(i, carry):
        r0 = pl.multiple_of(i * OR, OR)
        rp = pl.multiple_of(i * (OR // 2), OR // 2)
        ctx = jnp.concatenate(
            [pltpu.bitcast(ctx_v[h, pl.ds(rp, OR // 2), :], BF16) for h in range(H)], axis=1)
        o_v[pl.ds(r0, OR), :] = (acc_v[pl.ds(r0, OR), :] + _dot(ctx, wo_v[...])).astype(BF16)
        out_copy(i).start()
        return carry

    lax.fori_loop(0, S // OR, out_body, 0)
    for i in range(S // OR):
        out_copy(i).wait()


@jax.jit
def pallas_parallel_sum__compressed_kv_cla__moe_arch_mod__prompt_kernel(
    A_x: jax.Array,
    A_c_kv: jax.Array,
    A_w_q: jax.Array,
    A_w_uk: jax.Array,
    A_w_uv: jax.Array,
    A_w_o: jax.Array,
    B_x: jax.Array,
    B_w_r: jax.Array,
    B_w_gate: jax.Array,
    B_w_up: jax.Array,
    B_w_down: jax.Array,
):
    del B_x
    _, S, M = A_x.shape
    DC = A_c_kv.shape[2]
    H, D = A_w_q.shape[1], A_w_q.shape[2]
    FF = B_w_gate.shape[1]
    hbm = pl.BlockSpec(memory_space=pltpu.HBM)
    out = pl.pallas_call(
        _kernel,
        out_shape=jax.ShapeDtypeStruct((S, M), A_x.dtype),
        in_specs=[hbm] * 6 + [pl.BlockSpec(memory_space=pltpu.VMEM)] + [hbm] * 3,
        out_specs=hbm,
        scratch_shapes=[
            pltpu.VMEM((S, M), BF16),
            pltpu.VMEM((DC // T, S // 2, T), U32),
            pltpu.VMEM((H // HG, M, D), U32),
            pltpu.VMEM((H // HG, DC, D), U32),
            pltpu.VMEM((H // HG, DC, D), U32),
            pltpu.VMEM((H * D, M), BF16),
            pltpu.VMEM((FF, M), BF16),
            pltpu.VMEM((FF, M), BF16),
            pltpu.VMEM((FF, M), BF16),
            pltpu.VMEM((M // T, S // 2, T), U32),
            pltpu.VMEM((S, M), F32),
            pltpu.VMEM((S // 2, D), U32),
            pltpu.VMEM((S // 2, D), U32),
            pltpu.VMEM((S // 2, D), U32),
            pltpu.VMEM((2, (M + 2 * DC) // 2, D), U32),
            pltpu.VMEM((H, S // 2, D), U32),
            pltpu.VMEM((S, M), BF16),
            pltpu.SemaphoreType.DMA((5 + DC // T,)),
            pltpu.SemaphoreType.DMA((3 * H // HG,)),
            pltpu.SemaphoreType.DMA((S // OR,)),
        ],
        compiler_params=pltpu.CompilerParams(vmem_limit_bytes=110 * 1024 * 1024),
    )(
        A_x.reshape(S, M),
        A_c_kv.reshape(S, DC),
        A_w_q,
        A_w_uk,
        A_w_uv,
        A_w_o.reshape(H * D, M),
        B_w_r,
        B_w_gate.T,
        B_w_up.T,
        B_w_down,
    )
    return out.reshape(1, S, M)
```

```python
import math

import numpy as np
import jax
import jax.numpy as jnp
from jax import lax
import jax.experimental.pallas as pl
import jax.experimental.pallas.tpu as pltpu

BF16 = jnp.bfloat16
F32 = jnp.float32
U32 = jnp.uint32
TOPC = 8
LN_EPS = float(np.float32(np.asarray(1e-5, dtype=jnp.bfloat16)))
NEG = -1e30
T = 128
CK = 4
AHEAD = 2
WPB = 1
XC = 256
XF = 3
OR = 512
OS = 128
AC = 1
ANC = 0
TIE = 1
GATE = 0
LAG = 2
DEV = 0
WA = 1
LP = 0
ORD = 3
EV = 0


def _rb(v):
    return v.astype(BF16).astype(F32)


def _dot(a, b):
    return jnp.dot(a, b, preferred_element_type=F32)


def _dot_nt(a, b):
    return lax.dot_general(a, b, (((1,), (1,)), ((), ())), preferred_element_type=F32)


def _recip(v):
    inv = pl.reciprocal(v, approx=True)
    return inv * (2.0 - v * inv)


def _ld(ref, r0, n, *lead):
    return pltpu.bitcast(ref[(*lead, pl.ds(r0 // 2, n // 2), slice(None))], BF16)


def _st(ref, r0, val, *lead):
    n = val.shape[0]
    ref[(*lead, pl.ds(r0 // 2, n // 2), slice(None))] = pltpu.bitcast(val.astype(BF16), U32)


def _tree(op, xs):
    while len(xs) > 1:
        xs = [op(xs[i], xs[i + 1]) if i + 1 < len(xs) else xs[i] for i in range(0, len(xs), 2)]
    return xs[0]


def _tiles(v):
    return [v[:, j * T:(j + 1) * T] for j in range(v.shape[1] // T)]


def _rowsum(v):
    return jnp.sum(_tree(jnp.add, _tiles(v)), axis=-1, keepdims=True)


def _chain(*gens):
    for g in gens:
        yield from g


def _interleave(*streams):
    events = []
    for k, (gen, n) in enumerate(streams):
        events += [((j + 0.5) / n, k) for j in range(n)]
    for _, k in sorted(events):
        next(streams[k][0])


def _kernel(x_hbm, c_hbm, wq_hbm, wuk_hbm, wuv_hbm, wo_hbm, wr_ref, wg_hbm, wu_hbm, wd_hbm,
            out_hbm,
            x_v, c_v, wp_v, wo_v, wg_v, wu_v, wd_v,
            xn_v, acc_v, q_v, k_v, v_v, wh_v, ctx_v, o_v, xsems, wsems, lsems, osems):
    S, M, DC = 2 * x_v.shape[0], x_v.shape[1], c_v.shape[1]
    H, D = ctx_v.shape[0], ctx_v.shape[2]
    NB, NX, NPAIR, WT = S // T, S // XC, H // 2, (M + 2 * DC) // T

    def in_copies(j):
        rows = pl.ds(j * XC // 2, XC // 2)
        return [pltpu.make_async_copy(src.bitcast(U32).at[rows], dst.at[rows], xsems.at[2 * j + i])
                for i, (src, dst) in enumerate(((x_hbm, x_v), (c_hbm, c_v)))]

    def pair_copies(g):
        return [pltpu.make_async_copy(src.bitcast(U32).at[:, g, :],
                                      wp_v.at[g % 2, pl.ds(r0, n)], wsems.at[3 * (g % 2) + i])
                for i, (src, r0, n) in enumerate(
                    ((wq_hbm, 0, M), (wuk_hbm, M, DC), (wuv_hbm, M + DC, DC)))]

    late = [pltpu.make_async_copy(s, d, lsems.at[i]) for i, (s, d) in enumerate(
        ((wg_hbm, wg_v), (wu_hbm, wu_v), (wd_hbm, wd_v), (wo_hbm, wo_v)))]

    def start(cps):
        for cp in cps:
            cp.start()

    def wait(cps):
        for cp in cps:
            cp.wait()

    start(in_copies(0))
    start(pair_copies(0))
    for j in range(1, XF):
        start(in_copies(j))

    lane = lax.broadcasted_iota(jnp.int32, (8, T), 1)
    sub = lax.broadcasted_iota(jnp.int32, (8, T), 0)
    qscale = (D ** -0.5) * math.log2(math.e)

    zero = jnp.min(lane)
    zero8 = pl.multiple_of(zero * 8, 8)
    pending = []

    def anchored(w32):
        top = w32[0:8]
        while pending:
            top = jnp.where(zero > 0, pending.pop()(), top)
        return jnp.concatenate([top, w32[8:]], axis=0)

    def layernorm(i):
        if i * T % XC == 0:
            j = i * T // XC
            wait(in_copies(j))
            if j + XF < NX:
                start(in_copies(j + XF))
            elif j + XF == NX:
                start(pair_copies(1))
        xf = _ld(x_v, i * T, T).astype(F32)
        mean = _rowsum(xf) * (1.0 / M)
        cen = xf - mean
        var = _rowsum(cen * cen) * (1.0 / M)
        den = _rb(jnp.sqrt(_rb(_rb(var) + LN_EPS)))
        _st(xn_v, i * T, _rb(xf - _rb(mean)) * (1.0 / den))
        yield

    scores_r = [jnp.zeros((8, T), F32) for _ in range(S // (8 * T))]
    wr = wr_ref[...].astype(F32).reshape(1, M)

    def residual_and_router(i):
        xn = _ld(xn_v, i * T, T).astype(F32)
        acc_v[i * T:(i + 1) * T, :] = _ld(x_v, i * T, T).astype(F32) + xn
        r = _rowsum(xn * wr)
        for g in range(T // 8):
            k, ln = divmod(i * (T // 8) + g, T)
            scores_r[k] = jnp.where(lane == ln, r[g * 8:(g + 1) * 8, :], scores_r[k])
        pending.append(lambda: pltpu.bitcast(acc_v[pl.ds(zero8, 8), 0:T], U32))
        done = scores_r[k]
        pending.append(lambda: pltpu.bitcast(done, U32))
        yield

    def unpack_weights(g, tiles):
        for t in tiles:
            even = wp_v[g % 2, pl.ds(t * T, T // 2, stride=2), :]
            odd = wp_v[g % 2, pl.ds(t * T + 1, T // 2, stride=2), :]
            rows = pl.ds(t * T // 2, T // 2)
            wh_v[2 * (g % 2), rows, :] = (even & U32(0xFFFF)) | (odd << 16)
            wh_v[2 * (g % 2) + 1, rows, :] = (even >> 16) | (odd & U32(0xFFFF0000))
            if WA:
                pending.append(lambda: wh_v[zero, pl.ds(zero8, 8), :])
            yield

    def project_q(i, slot):
        _st(q_v, i * T, _dot(_ld(xn_v, i * T, T), _ld(wh_v, 0, M, slot)) * qscale)
        yield

    def project_kv(i, slot):
        _st(k_v, i * T, _dot(_ld(c_v, i * T, T), _ld(wh_v, M, DC, slot)))
        yield
        _st(v_v, i * T, _dot(_ld(c_v, i * T, T), _ld(wh_v, M + DC, DC, slot)))
        yield

    def project(i, slot):
        return _chain(project_kv(i, slot), project_q(i, slot))

    def chunks(i):
        return [(t, min(CK, i + 1 - t)) for t in range(0, i + 1, CK)]

    toks = []
    link = {}

    def scores(i, st):
        mp = None
        st["s"] = []
        for ci, (t, n) in enumerate(chunks(i)):
            q = q_v[i * T // 2:(i + 1) * T // 2, :]
            if ci == min(AC, len(chunks(i)) - 1):
                q = anchored(q)
            tiles = _tiles(_dot_nt(pltpu.bitcast(q, BF16), _ld(k_v, t * T, n * T)))
            if t + n == i + 1:
                row = lax.broadcasted_iota(jnp.int32, (T, T), 0)
                col = lax.broadcasted_iota(jnp.int32, (T, T), 1)
                tiles[-1] = jnp.where(col <= row, tiles[-1], NEG)
            toks.append(tiles[-1])
            st["s"].append(jnp.concatenate(tiles, axis=1) if n > 1 else tiles[0])
            mp = _tree(jnp.maximum, tiles if mp is None else tiles + [mp])
            if t + n == i + 1:
                st["m"] = jnp.max(mp, axis=-1, keepdims=True)
            yield

    def context(i, h, st):
        lp = None
        o = None
        for ci, (t, n) in enumerate(chunks(i)):
            m = st["m"]
            if GATE == 1 and len(toks) >= 2:
                m = jnp.where(zero > 0, jnp.concatenate([toks[-2][T - 8:T]] * (T // 8), axis=0), m)
            if GATE == 2 and len(toks) >= 2:
                c = T - 16 * LAG
                m = jnp.where(zero > 0, jnp.concatenate([toks[-2][c:T], toks[-1][0:c]], axis=0), m)
            if m.shape[1] == T and n > 1:
                m = jnp.concatenate([m] * n, axis=1)
            d = st["s"][ci] - m
            if TIE and ci == 0 and "tie" in link:
                d0 = jnp.minimum(d[:, 0:T], link["tie"])
                d = jnp.concatenate([d0, d[:, T:]], axis=1) if n > 1 else d0
            p = jnp.exp2(d)
            ps = _tree(jnp.add, _tiles(p))
            lp = ps if lp is None else lp + ps
            pv = _dot(p.astype(BF16), _ld(v_v, t * T, n * T))
            o = pv if o is None else o + pv
            if GATE == 2:
                toks.append(pv)
            if t + n == i + 1:
                o = o * _recip(jnp.sum(lp, axis=-1, keepdims=True))
                link["tie"] = jnp.abs(o)
                _st(ctx_v, i * T, o, h)
            yield

    def head(h, slot, next_slot, before=None, extra=None):
        prev = None
        for i in range(NB):
            st = {}
            streams = [(scores(i, st), len(chunks(i)))]
            if prev is not None:
                streams.append((context(i - 1, h, prev), len(chunks(i - 1))))
            if i + AHEAD < NB:
                if before is not None:
                    next(before(i + AHEAD))
                streams.append((project(i + AHEAD, slot), 3))
            if extra is not None:
                streams += extra(i)
            if ORD == 1:
                for g_, n_ in streams:
                    for _ in range(n_):
                        next(g_)
            elif ORD == 2:
                next(streams[0][0])
                streams[0] = (streams[0][0], streams[0][1] - 1)
                _interleave(*[s_ for s_ in (streams[1:] + streams[:1]) if s_[1]])
            elif ORD == 3:
                for _ in range(min(2, streams[0][1])):
                    next(streams[0][0])
                streams[0] = (streams[0][0], streams[0][1] - min(2, streams[0][1]))
                _interleave(*[s_ for s_ in (streams[1:] + streams[:1]) if s_[1]])
            else:
                _interleave(*streams)
            if ANC and prev is not None:
                pending.append(lambda: ctx_v[h, pl.ds(zero8, 8), :])
            prev = st
        last = context(NB - 1, h, prev)
        next(last)
        _interleave((last, len(chunks(NB - 1)) - 1),
                    (_chain(*[project(p, next_slot) for p in range(AHEAD)]), 3 * AHEAD))
        if ANC:
            pending.append(lambda: ctx_v[h, pl.ds(zero8, 8), :])

    def unpack_schedule(g, first):
        gen = unpack_weights(g, range(WT))

        def sched(i):
            n = min(WPB, WT - (i - first) * WPB)
            return [(gen, n)] if i >= first and n > 0 else []
        return sched

    next(layernorm(0))
    wait(pair_copies(0))
    for _ in unpack_weights(0, range(WT)):
        pass
    for i in range(AHEAD):
        if i:
            next(layernorm(i))
        for _ in project(i, 0):
            pass
    pending.clear()
    if not DEV:
        head(0, 0, 1, before=layernorm)
    wait(pair_copies(1))
    start(pair_copies(2))
    start(late)
    sched = unpack_schedule(1, 1)
    if not DEV:
        head(1, 1, 2, extra=lambda i: sched(i) + [(residual_and_router(i), 1)])

    def pair_body(g, carry):
        pending.clear()
        toks.clear()
        link.clear()

        @pl.when(g + 1 < NPAIR)
        def _():
            wait(pair_copies(g + 1))

        @pl.when(g + 2 < NPAIR)
        def _():
            start(pair_copies(g + 2))

        s0 = 2 * (g % 2)
        head(2 * g, s0, s0 + 1, extra=unpack_schedule(g + 1, 1))
        head(2 * g + 1, s0 + 1, 2 - s0)
        return carry

    lax.fori_loop(1, NPAIR, pair_body, 0)

    keys = []
    for k, rd in enumerate(scores_r):
        bits = pltpu.bitcast(_rb(rd), jnp.int32) >> 16
        mag = bits & 0x7FFF
        order = jnp.where(bits < 0, 0x8000 - mag, 0x8000 + mag)
        order = jnp.where(mag > 0x7F80, 0, order)
        row = k * 8 * T + lane * 8 + sub
        keys.append(order * S + (S - 1 - row))
    sel_keys = []
    for _ in range(TOPC):
        top = jnp.max(_tree(jnp.maximum, keys))
        sel_keys.append(top)
        keys = [jnp.where(kk == top, -1, kk) for kk in keys]

    sub16 = lax.broadcasted_iota(jnp.int32, (16, M), 0)
    sub8m = lax.broadcasted_iota(jnp.int32, (TOPC, M), 0)
    xs = jnp.zeros((TOPC, M), F32)
    key_col = jnp.zeros((TOPC, T), jnp.int32)
    rows = []
    for j, top in enumerate(sel_keys):
        row = S - 1 - (top % S)
        rows.append(row)
        base = pl.multiple_of((row // 16) * 8, 8)
        tile = pltpu.bitcast(xn_v[pl.ds(base, 8), :], BF16).astype(F32)
        one = jnp.sum(jnp.where(sub16 == row % 16, tile, 0.0), axis=0, keepdims=True)
        xs = jnp.where(sub8m == j, one, xs)
        key_col = jnp.where(sub == j, top, key_col)
    order = key_col // S
    bits = jnp.where(order >= 0x8000, order - 0x8000, (0x8000 - order) | 0x8000)
    bits = jnp.where(order == 0, 0x7FC0, bits)
    r_sel = pltpu.bitcast(bits << 16, F32)[:, 0:1]
    wait(late)
    xs = xs.astype(BF16)
    g = _dot_nt(xs, wg_v[...])
    u = _dot_nt(xs, wu_v[...])
    hid = (g * jax.nn.sigmoid(g) * u).astype(BF16)
    y = _dot(hid, wd_v[...]) * jax.nn.sigmoid(r_sel)
    for j, row in enumerate(rows):
        acc_v[pl.ds(row, 1), :] += y[j:j + 1, :]

    def out_copy(i):
        r0 = pl.multiple_of(i * OS, OS)
        return pltpu.make_async_copy(o_v.at[pl.ds(r0, OS)], out_hbm.at[pl.ds(r0, OS)], osems.at[i])

    def out_body(b, carry):
        for u in range(OR // OS):
            i = b * (OR // OS) + u
            r0 = pl.multiple_of(i * OS, OS)
            rp = pl.multiple_of(i * (OS // 2), OS // 2)
            ctx = jnp.concatenate(
                [pltpu.bitcast(ctx_v[h, pl.ds(rp, OS // 2), :], BF16) for h in range(H)], axis=1)
            o_v[pl.ds(r0, OS), :] = (acc_v[pl.ds(r0, OS), :] + _dot(ctx, wo_v[...])).astype(BF16)
            out_copy(i).start()
        return carry

    lax.fori_loop(0, S // OR, out_body, 0)
    for i in range(S // OS):
        out_copy(i).wait()


@jax.jit
def pallas_parallel_sum__compressed_kv_cla__moe_arch_mod__prompt_kernel(
    A_x: jax.Array,
    A_c_kv: jax.Array,
    A_w_q: jax.Array,
    A_w_uk: jax.Array,
    A_w_uv: jax.Array,
    A_w_o: jax.Array,
    B_x: jax.Array,
    B_w_r: jax.Array,
    B_w_gate: jax.Array,
    B_w_up: jax.Array,
    B_w_down: jax.Array,
):
    del B_x
    _, S, M = A_x.shape
    DC = A_c_kv.shape[2]
    H, D = A_w_q.shape[1], A_w_q.shape[2]
    FF = B_w_gate.shape[1]
    hbm = pl.BlockSpec(memory_space=pltpu.HBM)
    out = pl.pallas_call(
        _kernel,
        out_shape=jax.ShapeDtypeStruct((S, M), A_x.dtype),
        in_specs=[hbm] * 6 + [pl.BlockSpec(memory_space=pltpu.VMEM)] + [hbm] * 3,
        out_specs=hbm,
        scratch_shapes=[
            pltpu.VMEM((S // 2, M), U32),
            pltpu.VMEM((S // 2, DC), U32),
            pltpu.VMEM((2, M + 2 * DC, D), U32),
            pltpu.VMEM((H * D, M), BF16),
            pltpu.VMEM((FF, M), BF16),
            pltpu.VMEM((FF, M), BF16),
            pltpu.VMEM((FF, M), BF16),
            pltpu.VMEM((S // 2, M), U32),
            pltpu.VMEM((S, M), F32),
            pltpu.VMEM((S // 2, D), U32),
            pltpu.VMEM((S // 2, D), U32),
            pltpu.VMEM((S // 2, D), U32),
            pltpu.VMEM((4, (M + 2 * DC) // 2, D), U32),
            pltpu.VMEM((H, S // 2, D), U32),
            pltpu.VMEM((S, M), BF16),
            pltpu.SemaphoreType.DMA((2 * S // XC,)),
            pltpu.SemaphoreType.DMA((6,)),
            pltpu.SemaphoreType.DMA((4,)),
            pltpu.SemaphoreType.DMA((S // OS,)),
        ],
        compiler_params=pltpu.CompilerParams(
            vmem_limit_bytes=100 * 1024 * 1024,
            flags={**({"XLA_TPU_FORCE_LP_LLO_SCHEDULER": True} if LP else {}),
                   **({"XLA_TPU_EVENLY_DISTRIBUTE_CRITICAL_NODES": True} if EV else {})}),
    )(
        A_x.reshape(S, M),
        A_c_kv.reshape(S, DC),
        A_w_q,
        A_w_uk,
        A_w_uv,
        A_w_o.reshape(H * D, M),
        B_w_r,
        B_w_gate.T,
        B_w_up.T,
        B_w_down,
    )
    return out.reshape(1, S, M)
```

```python
import math

import numpy as np
import jax
import jax.numpy as jnp
from jax import lax
import jax.experimental.pallas as pl
import jax.experimental.pallas.tpu as pltpu

BF16 = jnp.bfloat16
F32 = jnp.float32
U32 = jnp.uint32
TOPC = 8
LN_EPS = float(np.float32(np.asarray(1e-5, dtype=jnp.bfloat16)))
NEG = -1e30
T = 128
CK = 4
LAG = 10
ORDER = 1
BIAS = 0
XC = 256
XF = 3
OR = 512
TIE = 1
GATE = 3
GR = 120
H1 = 4
H2 = 2
GB = 2
DEV = 0


def _rb(v):
    return v.astype(BF16).astype(F32)


def _dot(a, b):
    return jnp.dot(a, b, preferred_element_type=F32)


def _dot_nt(a, b):
    return lax.dot_general(a, b, (((1,), (1,)), ((), ())), preferred_element_type=F32)


def _recip(v):
    inv = pl.reciprocal(v, approx=True)
    return inv * (2.0 - v * inv)


def _ld(ref, r0, n, *lead):
    return pltpu.bitcast(ref[(*lead, pl.ds(r0 // 2, n // 2), slice(None))], BF16)


def _st(ref, r0, val, *lead):
    n = val.shape[0]
    ref[(*lead, pl.ds(r0 // 2, n // 2), slice(None))] = pltpu.bitcast(val.astype(BF16), U32)


def _tree(op, xs):
    while len(xs) > 1:
        xs = [op(xs[i], xs[i + 1]) if i + 1 < len(xs) else xs[i] for i in range(0, len(xs), 2)]
    return xs[0]


def _tiles(v):
    return [v[:, j * T:(j + 1) * T] for j in range(v.shape[1] // T)]


def _rowsum(v):
    return jnp.sum(_tree(jnp.add, _tiles(v)), axis=-1, keepdims=True)


def _merge(*lists):
    keyed = []
    for k, items in enumerate(lists):
        keyed += [((j + 0.5) / len(items), k, j) for j in range(len(items))]
    return [lists[k][j] for _, k, j in sorted(keyed)]


def _kernel(x_hbm, c_hbm, wq_hbm, wuk_hbm, wuv_hbm, wo_hbm, wr_ref, wg_hbm, wu_hbm, wd_hbm,
            out_hbm,
            x_v, c_v, wp_v, wo_v, wg_v, wu_v, wd_v,
            xn_v, q_v, k_v, v_v, wh_v, ctx_v, y_v, o_v, xsems, wsems, lsems, osems):
    S, M, DC = 2 * x_v.shape[0], x_v.shape[1], c_v.shape[1]
    H, D = ctx_v.shape[0], ctx_v.shape[2]
    NB, NX, NPAIR, WT = S // T, S // XC, H // 2, (M + 2 * DC) // T

    def in_copies(j):
        rows = pl.ds(j * XC // 2, XC // 2)
        return [pltpu.make_async_copy(src.bitcast(U32).at[rows], dst.at[rows], xsems.at[2 * j + i])
                for i, (src, dst) in enumerate(((c_hbm, c_v), (x_hbm, x_v)))]

    def pair_copies(g):
        return [pltpu.make_async_copy(src.bitcast(U32).at[:, g, :],
                                      wp_v.at[g, pl.ds(r0, n)], wsems.at[3 * g + i])
                for i, (src, r0, n) in enumerate(
                    ((wuk_hbm, M, DC), (wuv_hbm, M + DC, DC), (wq_hbm, 0, M)))]

    late = [pltpu.make_async_copy(s, d, lsems.at[i]) for i, (s, d) in enumerate(
        ((wg_hbm, wg_v), (wu_hbm, wu_v), (wd_hbm, wd_v), (wo_hbm, wo_v)))]

    def start(cps):
        for cp in cps:
            cp.start()

    def wait(cps):
        for cp in cps:
            cp.wait()

    first_w = pair_copies(0)
    start(first_w[:1] + in_copies(0) + first_w[1:])
    for j in range(1, XF):
        start(in_copies(j))

    lane = lax.broadcasted_iota(jnp.int32, (8, T), 1)
    sub = lax.broadcasted_iota(jnp.int32, (8, T), 0)
    qscale = (D ** -0.5) * math.log2(math.e)

    zero = jnp.min(lane)
    zero8 = pl.multiple_of(zero * 8, 8)
    pending = []

    def anchored(w32):
        top = w32[0:8]
        while pending:
            top = jnp.where(zero > 0, pending.pop()(), top)
        return jnp.concatenate([top, w32[8:]], axis=0)

    scores_r = [jnp.zeros((8, T), F32) for _ in range(S // (8 * T))]
    wr = wr_ref[...].astype(F32).reshape(1, M)

    def layernorm(i):
        xf = _ld(x_v, i * T, T).astype(F32)
        mean = _rowsum(xf) * (1.0 / M)
        cen = xf - mean
        var = _rowsum(cen * cen) * (1.0 / M)
        den = _rb(jnp.sqrt(_rb(_rb(var) + LN_EPS)))
        _st(xn_v, i * T, _rb(xf - _rb(mean)) * _recip(den))

    def router(i):
        r = _rowsum(_ld(xn_v, i * T, T).astype(F32) * wr)
        for g in range(T // 8):
            k, ln = divmod(i * (T // 8) + g, T)
            scores_r[k] = jnp.where(lane == ln, r[g * 8:(g + 1) * 8, :], scores_r[k])
        done = scores_r[k]
        pending.append(lambda: pltpu.bitcast(done, U32))

    def unpack_weights(g, odd_head, t):
        even = wp_v[g, pl.ds(t * T, T // 2, stride=2), :]
        odd = wp_v[g, pl.ds(t * T + 1, T // 2, stride=2), :]
        if odd_head:
            w = (even >> 16) | (odd & U32(0xFFFF0000))
        else:
            w = (even & U32(0xFFFF)) | (odd << 16)
        wh_v[odd_head, pl.ds(t * T // 2, T // 2), :] = w

    def project_q(i, buf):
        _st(q_v, i * T, _dot(_ld(xn_v, i * T, T), _ld(wh_v, 0, M, buf)) * qscale, buf)

    def project_k(i, buf):
        _st(k_v, i * T, _dot(_ld(c_v, i * T, T), _ld(wh_v, M, DC, buf)), buf)

    def project_v(i, buf, after=None):
        c = c_v[i * T // 2:(i + 1) * T // 2, :]
        if after is not None:
            tok = jnp.broadcast_to(pltpu.bitcast(
                jnp.broadcast_to(after[T - 8:T], (8, T)), U32)[None], (DC // T, 8, T))
            top = jnp.where(zero > 0, jnp.concatenate(list(tok), axis=1), c[0:8])
            c = jnp.concatenate([top, c[8:]], axis=0)
        _st(v_v, i * T, _dot(pltpu.bitcast(c, BF16), _ld(wh_v, M + DC, DC, buf)), buf)

    def projections(buf):
        ks = [(DC // T, lambda i=i: project_k(i, buf)) for i in range(NB)]
        qs = [(M // T, lambda i=i: project_q(i, buf)) for i in order]
        vs = [(DC // T, lambda i=i, **kw: project_v(i, buf, **kw)) for i in range(NB)]
        return _merge(ks, qs) + vs

    def scores(i, t, n, buf, st):
        q = anchored(q_v[buf, i * T // 2:(i + 1) * T // 2, :])
        tiles = _tiles(_dot_nt(pltpu.bitcast(q, BF16), _ld(k_v, t * T, n * T, buf)))
        if t + n == i + 1:
            row = lax.broadcasted_iota(jnp.int32, (T, T), 0)
            col = lax.broadcasted_iota(jnp.int32, (T, T), 1)
            tiles[-1] = jnp.where(col <= row, tiles[-1], NEG)
        st[t] = jnp.concatenate(tiles, axis=1) if n > 1 else tiles[0]
        st["m"] = _tree(jnp.maximum, tiles + ([st["m"]] if t else []))
        if t + n == i + 1:
            st["m"] = jnp.max(st["m"], axis=-1, keepdims=True)

    link = {}

    def context(i, t, n, h, buf, st):
        if GATE and t // CK == GATE:
            tok = st["pv"][0][GR:GR + 8]
            st["m"] = jnp.where(zero > 0, jnp.concatenate([tok] * (T // 8), axis=0), st["m"])
        m = st["m"]
        if m.shape[1] == T and n > 1:
            m = jnp.concatenate([m] * n, axis=1)
        d = st[t] - m
        if TIE and t == 0 and "tie" in link:
            d0 = jnp.minimum(d[:, 0:T], link["tie"])
            d = jnp.concatenate([d0, d[:, T:]], axis=1) if n > 1 else d0
        p = jnp.exp2(d)
        lp = _tree(jnp.add, _tiles(p))
        o = _dot(p.astype(BF16), _ld(v_v, t * T, n * T, buf))
        st.setdefault("pv", []).append(o)
        if t:
            lp, o = st["l"] + lp, st["o"] + o
        st["l"], st["o"] = lp, o
        if t + n == i + 1:
            o = o * _recip(jnp.sum(lp, axis=-1, keepdims=True))
            link["tie"] = jnp.abs(o)
            _st(ctx_v, i * T, o, h)

    order = [list(range(NB))[::-1], list(range(NB)),
             list(range(1, NB, 2)) + list(range(0, NB, 2))[::-1],
             [j for i in range(NB // 2) for j in (NB - 1 - i, i)]][ORDER]

    def head(h, buf, fillers, hold=False):
        work = [(i, t, min(CK, i + 1 - t)) for i in order for t in range(0, i + 1, CK)]
        state = {i: {} for i in order}
        held = []
        if hold:
            fillers, held = fillers[:len(fillers) - H1 - H2], fillers[len(fillers) - H1 - H2:]
        att_total = 2 * sum(n for _, _, n in work)
        fill_total = sum(c for c, _ in fillers)
        a = b = f = att = fill = 0
        ready = {}
        last_was_scores = False
        while b < len(work) or f < len(fillers):
            b_ok = b < len(work) and ready.get(work[b][0], 1 << 30) <= att + fill
            if f < len(fillers) and ((fill - BIAS) * att_total < att * fill_total
                                     or (a == len(work) and not b_ok)):
                fillers[f][1]()
                fill += fillers[f][0]
                f += 1
            elif a < len(work) and not (b_ok and last_was_scores):
                i, t, n = work[a]
                scores(i, t, n, buf, state[i])
                a += 1
                att += n
                last_was_scores = True
                if t + n == i + 1:
                    ready[i] = att + fill + LAG
                if a == len(work) and hold:
                    for _, fn in held[:H1]:
                        fn(after=tok)
                tok = state[i][t][:, 0:T]
            else:
                i, t, n = work[b]
                context(i, t, n, h, buf, state[i])
                b += 1
                att += n
                last_was_scores = False

        for _, fn in held[H1:]:
            fn(after=state[order[-1]]["pv"][-GB])

    def unpacking(g, odd_head):
        return [(0, lambda t=t: unpack_weights(g, odd_head, t)) for t in range(WT)]

    for cp, t0, n in ((first_w[0], M // T, DC // T), (first_w[1], (M + DC) // T, DC // T),
                      (first_w[2], 0, M // T)):
        cp.wait()
        for t in range(t0, t0 + n):
            unpack_weights(0, 0, t)
    for i in range(NB):
        if i * T % XC == 0:
            j = i * T // XC
            wait(in_copies(j))
            if j + XF < NX:
                start(in_copies(j + XF))
            elif j + XF == NX:
                start(pair_copies(1))
        if not DEV:
            layernorm(i)
            project_k(i, 0)
            project_v(i, 0)
            if i:
                project_q(i - 1, 0)
    project_q(NB - 1, 0)
    for t in range(WT):
        unpack_weights(0, 1, t)

    wait(pair_copies(1))
    for g in range(2, NPAIR):
        start(pair_copies(g))
    start(late)
    if not DEV:
        head(0, 0, _merge(projections(1),
                          [(0, lambda i=i: router(i)) for i in range(NB)] + unpacking(1, 0)))

    keys = []
    for k, rd in enumerate(scores_r):
        bits = pltpu.bitcast(_rb(rd), jnp.int32) >> 16
        mag = bits & 0x7FFF
        rank = jnp.where(bits < 0, 0x8000 - mag, 0x8000 + mag)
        rank = jnp.where(mag > 0x7F80, 0, rank)
        row = k * 8 * T + lane * 8 + sub
        keys.append(rank * S + (S - 1 - row))

    def pair_body(g, carry):
        pending.clear()
        link.clear()

        @pl.when(g + 1 < NPAIR)
        def _():
            wait(pair_copies(g + 1))

        head(2 * g - 1, 1, _merge(projections(0), unpacking(g, 1)))
        head(2 * g, 0, unpacking(jnp.minimum(g + 1, NPAIR - 1), 0) + projections(1), hold=True)
        return carry

    lax.fori_loop(1, NPAIR, pair_body, 0)
    pending.clear()
    link.clear()
    wait(late)

    sel = []
    ffn = {}

    def select_step():
        top = jnp.max(_tree(jnp.maximum, keys))
        sel.append(top)
        keys[:] = [jnp.where(kk == top, -1, kk) for kk in keys]

    def gather():
        sub16 = lax.broadcasted_iota(jnp.int32, (16, M), 0)
        sub8m = lax.broadcasted_iota(jnp.int32, (TOPC, M), 0)
        xs = jnp.zeros((TOPC, M), F32)
        key_col = jnp.zeros((TOPC, T), jnp.int32)
        for j, top in enumerate(sel):
            row = S - 1 - (top & (S - 1))
            tile = pltpu.bitcast(xn_v[pl.ds(pl.multiple_of((row >> 4) * 8, 8), 8), :], BF16)
            one = jnp.sum(jnp.where(sub16 == (row & 15), tile.astype(F32), 0.0), axis=0, keepdims=True)
            xs = jnp.where(sub8m == j, one, xs)
            key_col = jnp.where(sub == j, top, key_col)
        rank = key_col >> (S.bit_length() - 1)
        bits = jnp.where(rank >= 0x8000, rank - 0x8000, (0x8000 - rank) | 0x8000)
        bits = jnp.where(rank == 0, 0x7FC0, bits)
        ffn["gain"] = jax.nn.sigmoid(pltpu.bitcast(bits << 16, F32))
        ffn["x"] = xs.astype(BF16)

    FF = wd_v.shape[0]

    def ffn_step(f0):
        rows = slice(f0, min(f0 + T, FF))
        g = _dot_nt(ffn["x"], wg_v[rows, :])
        u = _dot_nt(ffn["x"], wu_v[rows, :])
        y = _dot((g * jax.nn.sigmoid(g) * u).astype(BF16), wd_v[rows, :])
        ffn["y"] = ffn["y"] + y if f0 else y

    def out_project(rp, heads):
        ctx = jnp.concatenate(
            [pltpu.bitcast(ctx_v[h, pl.ds(rp, T // 2), :], BF16) for h in heads], axis=1)
        return _dot(ctx, wo_v[heads[0] * D:(heads[-1] + 1) * D, :])

    early = {}

    def early_out(i, h0, h1):
        part = out_project(i * T // 2, range(h0, h1))
        early[i] = early[i] + part if h0 else part

    side = ([(0, select_step)] * TOPC + [(0, gather)]
            + [(2, lambda f0=f0: ffn_step(f0)) for f0 in range(0, FF, T)])
    outs = [(5 * (min(h0 + 4, H - 1) - h0), lambda i=i, h0=h0: early_out(i, h0, min(h0 + 4, H - 1)))
            for i in range(1) for h0 in range(0, H - 1, 4)]
    if not DEV:
        head(H - 1, 1, _merge(outs, side))
    else:
        for _, fn in outs + side:
            fn()
    y = ffn["y"] * jnp.concatenate([ffn["gain"]] * (M // T), axis=1)
    for j in range(TOPC):
        y_v[j] = jnp.broadcast_to(y[j:j + 1, :], (8, M))

    def out_copy(i):
        r0 = pl.multiple_of(i * T, T)
        return pltpu.make_async_copy(o_v.at[pl.ds(r0, T)], out_hbm.at[pl.ds(r0, T)], osems.at[i])

    def finish(i, rp, attn):
        xn = pltpu.bitcast(xn_v[pl.ds(rp, T // 2), :], BF16).astype(F32)
        x = pltpu.bitcast(x_v[pl.ds(rp, T // 2), :], BF16).astype(F32)
        row = lax.broadcasted_iota(jnp.int32, (T, T), 0)
        upd = [jnp.zeros((T, T), F32)] * (M // T)
        for j, top in enumerate(sel):
            hit = row == S - 1 - (top & (S - 1)) - i * T
            yj = jnp.concatenate([y_v[j]] * (T // 8), axis=0)
            upd = [jnp.where(hit, yt, ut) for yt, ut in zip(_tiles(yj), upd)]
        res = (x + attn) + (xn + jnp.concatenate(upd, axis=1))
        o_v[pl.ds(2 * rp, T), :] = res.astype(BF16)
        out_copy(i).start()

    NO = OR // T
    for i in range(NO):
        if i in early:
            finish(i, i * T // 2, early[i] + out_project(i * T // 2, [H - 1]))
        else:
            finish(i, i * T // 2, out_project(i * T // 2, range(H)))

    def out_body(b, carry):
        for u in range(NO):
            i = b * NO + u
            rp = pl.multiple_of(i * (T // 2), T // 2)
            finish(i, rp, out_project(rp, range(H)))
        return carry

    lax.fori_loop(1, S // OR, out_body, 0)
    for i in range(NB):
        out_copy(i).wait()


@jax.jit
def pallas_parallel_sum__compressed_kv_cla__moe_arch_mod__prompt_kernel(
    A_x: jax.Array,
    A_c_kv: jax.Array,
    A_w_q: jax.Array,
    A_w_uk: jax.Array,
    A_w_uv: jax.Array,
    A_w_o: jax.Array,
    B_x: jax.Array,
    B_w_r: jax.Array,
    B_w_gate: jax.Array,
    B_w_up: jax.Array,
    B_w_down: jax.Array,
):
    del B_x
    _, S, M = A_x.shape
    DC = A_c_kv.shape[2]
    H, D = A_w_q.shape[1], A_w_q.shape[2]
    FF = B_w_gate.shape[1]
    hbm = pl.BlockSpec(memory_space=pltpu.HBM)
    out = pl.pallas_call(
        _kernel,
        out_shape=jax.ShapeDtypeStruct((S, M), A_x.dtype),
        in_specs=[hbm] * 6 + [pl.BlockSpec(memory_space=pltpu.VMEM)] + [hbm] * 3,
        out_specs=hbm,
        scratch_shapes=[
            pltpu.VMEM((S // 2, M), U32),
            pltpu.VMEM((S // 2, DC), U32),
            pltpu.VMEM((H // 2, M + 2 * DC, D), U32),
            pltpu.VMEM((H * D, M), BF16),
            pltpu.VMEM((FF, M), BF16),
            pltpu.VMEM((FF, M), BF16),
            pltpu.VMEM((FF, M), BF16),
            pltpu.VMEM((S // 2, M), U32),
            pltpu.VMEM((2, S // 2, D), U32),
            pltpu.VMEM((2, S // 2, D), U32),
            pltpu.VMEM((2, S // 2, D), U32),
            pltpu.VMEM((2, (M + 2 * DC) // 2, D), U32),
            pltpu.VMEM((H, S // 2, D), U32),
            pltpu.VMEM((TOPC, 8, M), F32),
            pltpu.VMEM((S, M), BF16),
            pltpu.SemaphoreType.DMA((2 * S // XC,)),
            pltpu.SemaphoreType.DMA((3 * H // 2,)),
            pltpu.SemaphoreType.DMA((4,)),
            pltpu.SemaphoreType.DMA((S // T,)),
        ],
        compiler_params=pltpu.CompilerParams(vmem_limit_bytes=100 * 1024 * 1024),
    )(
        A_x.reshape(S, M),
        A_c_kv.reshape(S, DC),
        A_w_q,
        A_w_uk,
        A_w_uv,
        A_w_o.reshape(H * D, M),
        B_w_r,
        B_w_gate.T,
        B_w_up.T,
        B_w_down,
    )
    return out.reshape(1, S, M)
```

```python
import math

import numpy as np
import jax
import jax.numpy as jnp
from jax import lax
import jax.experimental.pallas as pl
import jax.experimental.pallas.tpu as pltpu

BF16 = jnp.bfloat16
F32 = jnp.float32
U32 = jnp.uint32
TOPC = 8
LN_EPS = float(np.float32(np.asarray(1e-5, dtype=jnp.bfloat16)))
NEG = -1e30
KEY0 = 0x10000000
T = 128
CK = 4
LAG = 10
ORDER = 1
BIAS = 0
XB = (0, 1, 2, 4, 8, 16)
XA = (-1, 1, 2, 4, 8)
XT = (-1, -1, -1, -1, -1)
XS = -1
PRI = 1
QD = 1
OR = 3
TIE = 1
GATE = 3
GR = 120
AHEAD = 3
VL = 6
OB = 128
OK = 1
NF = 3
NU = 7
LU = 128
DL = 4
TS = 4
RS = 1
RM = 0
WB = 1
PAD = 10
FO = 7
R2 = 32
DS = 12
RU = 128
FL = 2
H1 = 4
H2 = 2
GB = 2
DEV = 0


def _rb(v):
    return v.astype(BF16).astype(F32)


def _dot(a, b):
    return jnp.dot(a, b, preferred_element_type=F32)


def _dot_nt(a, b):
    return lax.dot_general(a, b, (((1,), (1,)), ((), ())), preferred_element_type=F32)


def _recip(v):
    inv = pl.reciprocal(v, approx=True)
    return inv * (2.0 - v * inv)


def _ld(ref, r0, n, *lead):
    return pltpu.bitcast(ref[(*lead, pl.ds(r0 // 2, n // 2), slice(None))], BF16)


def _st(ref, r0, val, *lead):
    n = val.shape[0]
    ref[(*lead, pl.ds(r0 // 2, n // 2), slice(None))] = pltpu.bitcast(val.astype(BF16), U32)


def _pack(pair):
    return pltpu.bitcast(pltpu.pack_elementwise(pair, packed_dtype=BF16), U32)


def _unpack(w32):
    return [pltpu.bitcast(w32 << 16, F32), pltpu.bitcast(w32 & U32(0xFFFF0000), F32)]


def _tree(op, xs):
    while len(xs) > 1:
        xs = [op(xs[i], xs[i + 1]) if i + 1 < len(xs) else xs[i] for i in range(0, len(xs), 2)]
    return xs[0]


def _tiles(v):
    return [v[:, j * T:(j + 1) * T] for j in range(v.shape[1] // T)]


def _rowsum(v):
    return jnp.sum(_tree(jnp.add, _tiles(v)), axis=-1, keepdims=True)


def _merge(*lists):
    keyed = []
    for k, items in enumerate(lists):
        keyed += [((j + 0.5) / len(items), k, j) for j in range(len(items))]
    return [lists[k][j] for _, k, j in sorted(keyed)]


def _kernel(x_hbm, c_hbm, wq_hbm, wuk_hbm, wuv_hbm, wo_hbm, wr_ref, wg_hbm, wu_hbm, wd_hbm,
            out_hbm,
            x_v, c_v, wp_v, wo_v, wg_v, wu_v, wd_v,
            xn_v, q_v, k_v, v_v, wh_v, ctx_v, acc_v, o_v, xsems, wsems, lsems, osem):
    S, M, DC = 2 * x_v.shape[0], x_v.shape[1], c_v.shape[1]
    H, D = ctx_v.shape[0], ctx_v.shape[2]
    NB, NX, NPAIR, WT = S // T, len(XA), H // 2, (M + 2 * DC) // T

    def in_copies(j):
        rows = pl.ds(XB[j] * T // 2, (XB[j + 1] - XB[j]) * T // 2)
        return [pltpu.make_async_copy(src.bitcast(U32).at[rows], dst.at[rows], xsems.at[2 * j + i])
                for i, (src, dst) in enumerate(((c_hbm, c_v), (x_hbm, x_v)))]

    def pair_copies(g):
        return [pltpu.make_async_copy(src.bitcast(U32).at[:, g, :],
                                      wp_v.at[g, pl.ds(r0, n)], wsems.at[3 * g + i])
                for i, (src, r0, n) in enumerate(
                    ((wuk_hbm, M, DC), (wuv_hbm, M + DC, DC), (wq_hbm, 0, M)))]

    late = [pltpu.make_async_copy(s.bitcast(U32), d, lsems.at[i]) for i, (s, d) in enumerate(
        ((wg_hbm, wg_v), (wu_hbm, wu_v), (wd_hbm, wd_v), (wo_hbm, wo_v)))]

    def start(cps):
        for cp in cps:
            cp.start()

    def wait(cps):
        for cp in cps:
            cp.wait()

    first_w = pair_copies(0)
    start(first_w)

    def start_inputs(after):
        for j in range(NX):
            if XT[j] == after:
                for cp in in_copies(j):
                    cp.start(priority=PRI if j else 0)
        if after == XS:
            for cp in [cp for g in range(1, NPAIR) for cp in pair_copies(g)]:
                cp.start(priority=PRI)

    start_inputs(-1)

    lane = lax.broadcasted_iota(jnp.int32, (8, T), 1)
    sub = lax.broadcasted_iota(jnp.int32, (8, T), 0)
    qscale = (D ** -0.5) * math.log2(math.e)

    zero = jnp.min(lane)
    zero8 = pl.multiple_of(zero * 8, 8)
    pending = []

    queue = []
    clock = [0]
    spacing = [0]

    def operand(ref, r0, n, buf=None):
        w32 = ref[(() if buf is None else (buf,)) + (pl.ds(r0 // 2, n // 2), slice(None))]
        clock[0] += 1
        due = [fn for t, fn in pending if t < clock[0]]
        pending[:] = [e for e in pending if e[0] >= clock[0]]
        if due:
            top = w32[0:8, 0:T]
            for fn in due:
                top = jnp.where(zero > 0, fn(), top)
            if w32.shape[1] > T:
                top = jnp.concatenate([top, w32[0:8, T:]], axis=1)
            w32 = jnp.concatenate([top, w32[8:]], axis=0)
        if queue and spacing[0] and clock[0] % spacing[0] == 0:
            queue.pop(0)()
        return pltpu.bitcast(w32, BF16)

    def flush(keep=0):
        while len(queue) > keep:
            queue.pop(0)()

    scores_r = [jnp.zeros((8, T), F32) for _ in range(S // (8 * T))]
    wr = wr_ref[...].astype(F32).reshape(1, M)

    arrived = [0]

    def arrive(j):
        arrived[0] = XB[j + 1]
        wait(in_copies(j))
        if j == 0:
            wait(first_w)
        start_inputs(j)
        for r0 in range(XB[j] * T, XB[j + 1] * T, LU):
            queue.append(lambda r0=r0: layernorm(r0))

    def layernorm(r0):
        rows = slice(r0 // 2, (r0 + LU) // 2)
        cens, invs = [], []
        for xf in _unpack(x_v[rows, :]):
            mean = _rowsum(xf) * (1.0 / M)
            mean_b = _rb(mean)
            cen = xf - mean_b
            off = mean - mean_b
            var = jnp.maximum(_rowsum(cen * cen) * (1.0 / M) - off * off, 0.0)
            cens.append(cen)
            invs.append(_recip(_rb(jnp.sqrt(_rb(_rb(var) + LN_EPS)))))
        xn_v[rows, :] = _pack([cen * inv for cen, inv in zip(_unpack(_pack(cens)), invs)])

    def router(r0):
        if RM == 1:
            residual(r0)
        r = _rowsum(_ld(xn_v, r0, RU).astype(F32) * wr)
        for g in range(RU // 8):
            k, ln = divmod(r0 // 8 + g, T)
            scores_r[k] = jnp.where(lane == ln, r[g * 8:(g + 1) * 8, :], scores_r[k])
        done = scores_r[k]
        pending.append((clock[0] + DL, lambda: pltpu.bitcast(done, U32)))

    def residual(r0):
        acc_v[r0:r0 + R2, :] = _ld(x_v, r0, R2).astype(F32) + _ld(xn_v, r0, R2).astype(F32)
        tok = pltpu.bitcast(acc_v[pl.ds(zero8, 8), 0:T], U32)
        pending.append((clock[0] + DL, lambda: tok))

    def unpack_weights(g, odd_head, t):
        even = wp_v[g, pl.ds(t * T, T // 2, stride=2), :]
        odd = wp_v[g, pl.ds(t * T + 1, T // 2, stride=2), :]
        if odd_head:
            w = (even >> 16) | (odd & U32(0xFFFF0000))
        else:
            w = (even & U32(0xFFFF)) | (odd << 16)
        wh_v[odd_head, pl.ds(t * T // 2, T // 2), :] = w

    def project_q(i, buf):
        _st(q_v, i * T, _dot(operand(xn_v, i * T, T), _ld(wh_v, 0, M, buf)) * qscale, buf)

    def project_k(i, buf):
        _st(k_v, i * T, _dot(operand(c_v, i * T, T), _ld(wh_v, M, DC, buf)), buf)

    def project_v(i, buf, after=None):
        c = pltpu.bitcast(operand(c_v, i * T, T), U32)
        if after is not None:
            tok = jnp.broadcast_to(pltpu.bitcast(
                jnp.broadcast_to(after[T - 8:T], (8, T)), U32)[None], (DC // T, 8, T))
            top = jnp.where(zero > 0, jnp.concatenate(list(tok), axis=1), c[0:8])
            c = jnp.concatenate([top, c[8:]], axis=0)
        _st(v_v, i * T, _dot(pltpu.bitcast(c, BF16), _ld(wh_v, M + DC, DC, buf)), buf)

    def projections(buf):
        ks = [(DC // T, lambda i=i: project_k(i, buf)) for i in range(NB)]
        qs = [(M // T, lambda i=i: project_q(i, buf)) for i in order]
        vs = [(DC // T, lambda i=i, **kw: project_v(i, buf, **kw)) for i in range(NB)]
        return _merge(ks, qs) + vs

    def scores(i, t, n, buf, st):
        tiles = _tiles(_dot_nt(operand(q_v, i * T, T, buf), _ld(k_v, t * T, n * T, buf)))
        if t + n == i + 1:
            row = lax.broadcasted_iota(jnp.int32, (T, T), 0)
            col = lax.broadcasted_iota(jnp.int32, (T, T), 1)
            tiles[-1] = jnp.where(col <= row, tiles[-1], NEG)
        st[t] = jnp.concatenate(tiles, axis=1) if n > 1 else tiles[0]
        st["m"] = _tree(jnp.maximum, tiles + ([st["m"]] if t else []))
        if t + n == i + 1:
            st["m"] = jnp.max(st["m"], axis=-1, keepdims=True)

    link = {}

    def context(i, t, n, h, buf, st):
        if GATE and t // CK == GATE:
            tok = st["pv"][0][GR:GR + 8]
            st["m"] = jnp.where(zero > 0, jnp.concatenate([tok] * (T // 8), axis=0), st["m"])
        m = st["m"]
        if m.shape[1] == T and n > 1:
            m = jnp.concatenate([m] * n, axis=1)
        d = st[t] - m
        if TIE and t == 0 and "tie" in link:
            d0 = jnp.minimum(d[:, 0:T], link["tie"])
            d = jnp.concatenate([d0, d[:, T:]], axis=1) if n > 1 else d0
        p = jnp.exp2(d)
        lp = _tree(jnp.add, _tiles(p))
        o = _dot(p.astype(BF16), operand(v_v, t * T, n * T, buf))
        st.setdefault("pv", []).append(o)
        if t:
            lp, o = st["l"] + lp, st["o"] + o
        st["l"], st["o"] = lp, o
        if t + n == i + 1:
            o = o * _recip(jnp.sum(lp, axis=-1, keepdims=True))
            link["tie"] = jnp.abs(o)
            _st(ctx_v, i * T, o, h)

    order = [list(range(NB))[::-1], list(range(NB)),
             list(range(1, NB, 2)) + list(range(0, NB, 2))[::-1],
             [j for i in range(NB // 2) for j in (NB - 1 - i, i)]][ORDER]

    def head(h, buf, fillers, hold=False, before=None):
        work = [(i, t, min(CK, i + 1 - t)) for i in order for t in range(0, i + 1, CK)]
        state = {i: {} for i in order}
        held = []
        if hold:
            fillers, held = fillers[:len(fillers) - H1 - H2], fillers[len(fillers) - H1 - H2:]
        att_total = 2 * sum(n for _, _, n in work)
        fill_total = sum(c for c, _ in fillers)
        a = b = f = att = fill = 0
        ready = {}
        last_was_scores = False
        while b < len(work) or f < len(fillers):
            b_ok = b < len(work) and ready.get(work[b][0], 1 << 30) <= att + fill
            if f < len(fillers) and ((fill - BIAS) * att_total < att * fill_total
                                     or (a == len(work) and not b_ok)):
                fillers[f][1]()
                fill += fillers[f][0]
                f += 1
            elif a < len(work) and not (b_ok and last_was_scores):
                i, t, n = work[a]
                if before is not None and t == 0:
                    fill += before(i)
                scores(i, t, n, buf, state[i])
                a += 1
                att += n
                last_was_scores = True
                if t + n == i + 1:
                    ready[i] = att + fill + LAG
                if a == len(work) and hold:
                    for _, fn in held[:H1]:
                        fn(after=tok)
                tok = state[i][t][:, 0:T]
            else:
                i, t, n = work[b]
                context(i, t, n, h, buf, state[i])
                b += 1
                att += n
                last_was_scores = False

        for _, fn in held[H1:]:
            fn(after=state[order[-1]]["pv"][-GB])

    def unpacking(g, odd_head):
        return [(0, lambda t=t: unpack_weights(g, odd_head, t)) for t in range(WT)]

    keys = []
    sel = []

    def select_step():
        if not keys:
            for k, rd in enumerate(scores_r):
                bits = pltpu.bitcast(_rb(rd), jnp.int32) >> 16
                mag = bits & 0x7FFF
                rank = jnp.where(bits < 0, 0x8000 - mag, 0x8000 + mag)
                rank = jnp.where(mag > 0x7F80, 0, rank)
                row = k * 8 * T + lane * 8 + sub
                keys.append(pltpu.bitcast(rank * S + (S - 1 - row) + KEY0, F32))
        top = jnp.max(jnp.max(_tree(jnp.maximum, keys), axis=0, keepdims=True), axis=1, keepdims=True)
        top = jnp.broadcast_to(top, (8, T))
        sel.append(pltpu.bitcast(top, jnp.int32) - KEY0)
        keys[:] = [jnp.where(kk == top, 0.0, kk) for kk in keys]
        pending.append((clock[0] + DL, lambda: pltpu.bitcast(top, U32)))

    def first_weights(k):
        t0, n = ((M // T, DC // T), ((M + DC) // T, DC // T), (0, M // T))[k]
        for t in range(t0, t0 + n):
            unpack_weights(0, 0, t)
            unpack_weights(0, 1, t)

    def prepare(i):
        cost = 0
        for j in range(NX):
            if XA[j] == i:
                arrive(j)
        if i < NB:
            if i == 0:
                first_weights(0)
            project_k(i, 0)
            project_k(i, 1)
            if i == 0:
                first_weights(1)
            project_v(i, 0)
            cost += 3 * DC // T
        if 0 <= i - QD < NB:
            if i == QD:
                first_weights(2)
            flush(keep=(arrived[0] - (i - QD + 1)) * T // LU)
            project_q(i - QD, 0)
            project_q(i - QD, 1)
            cost += 2 * M // T
        if i == DS:
            wait(pair_copies(1))
            start(late)
        lo = NB + AHEAD - VL
        if i >= lo:
            for j in range((i - lo) * NB // VL, (i - lo + 1) * NB // VL):
                project_v(j, 1)
                cost += DC // T
        return cost

    for j in range(NX):
        if XA[j] < 0:
            arrive(j)
    for i in range(AHEAD):
        prepare(i)
    if DEV != 1 and DEV != 3:
        head(0, 0, [], before=lambda i: prepare(i + AHEAD))
    else:
        prepare(DS)
    for _, fn in unpacking(1, 0):
        fn()

    def pair_body(g, carry):
        pending.clear()
        link.clear()

        @pl.when(g + 1 < NPAIR)
        def _():
            wait(pair_copies(g + 1))

        if DEV > 1:
            return carry
        head(2 * g - 1, 1, _merge(projections(0), unpacking(g, 1)))
        head(2 * g, 0, unpacking(jnp.minimum(g + 1, NPAIR - 1), 0) + projections(1), hold=True)
        return carry

    lax.fori_loop(1, NPAIR, pair_body, 0)
    pending.clear()
    link.clear()
    wait(late[3:] if WB else late)

    ffn = {}
    rows_sel = []

    def gather():
        sub8m = lax.broadcasted_iota(jnp.int32, (TOPC, M), 0)
        xs = jnp.zeros((TOPC, M), F32)
        key_col = jnp.zeros((TOPC, T), jnp.int32)
        for j, top in enumerate(sel):
            row = S - 1 - (top[0, 0] & (S - 1))
            rows_sel.append(row)
            w32 = xn_v[pl.ds(row >> 1, 1), :] << (16 - 16 * (row & 1)).astype(U32)
            xs = jnp.where(sub8m == j, pltpu.bitcast(w32 & U32(0xFFFF0000), F32), xs)
            key_col = jnp.where(sub == j, top, key_col)
        rank = key_col >> (S.bit_length() - 1)
        bits = jnp.where(rank >= 0x8000, rank - 0x8000, (0x8000 - rank) | 0x8000)
        bits = jnp.where(rank == 0, 0x7FC0, bits)
        ffn["gain"] = jax.nn.sigmoid(pltpu.bitcast(bits << 16, F32))
        ffn["x"] = xs.astype(BF16)

    FF = 2 * wd_v.shape[0]

    FG = 4 * T

    def ffn_in(name, w_v, f0, k):
        w = pltpu.bitcast(w_v[f0 // 2:min(f0 + FG, FF) // 2, k * T:(k + 1) * T], BF16)
        part = _dot_nt(ffn["x"][:, k * T:(k + 1) * T], w)
        ffn[name, f0] = ffn[name, f0] + part if k else part

    def ffn_down(f0, n0, n1):
        if n0 == 0:
            g, u = ffn["g", f0], ffn["u", f0]
            ffn["h", f0] = (g * jax.nn.sigmoid(g) * u).astype(BF16)
        w = pltpu.bitcast(wd_v[f0 // 2:min(f0 + FG, FF) // 2, n0 * T:n1 * T], BF16)
        for n, part in zip(range(n0, n1), _tiles(_dot(ffn["h", f0], w))):
            ffn["y", n] = ffn["y", n] + part if f0 else part

    def out_project(rp, h0, h1):
        ctx = jnp.concatenate(
            [pltpu.bitcast(ctx_v[h, pl.ds(rp, OB // 2), :], BF16) for h in range(h0, h1)], axis=1)
        return _dot(ctx, operand(wo_v, h0 * D, (h1 - h0) * D))

    early = {}

    def early_out(i, h0, h1):
        part = out_project(i * OB // 2, h0, h1)
        early[i] = early[i] + part if h0 else part

    def early_steps(i, nh):
        return [(M // T * OB // T * (min(h0 + OK, nh) - h0),
                 lambda h0=h0: early_out(i, h0, min(h0 + OK, nh))) for h0 in range(0, nh, OK)]

    side = []
    for f0 in range(0, FF, FG):
        for k in range(M // T):
            gate = lambda f0=f0, k=k: ffn_in("g", wg_v, f0, k)
            up = lambda f0=f0, k=k: ffn_in("u", wu_v, f0, k)
            if f0 + FG <= FF:
                side += [(1, gate), (1, up)]
            else:
                side += [(1, lambda gate=gate, up=up: (gate(), up()))]
    for f0 in range(0, FF, FG):
        step = 1 if f0 + FG <= FF else 2
        for n in range(0, M // T, step):
            side += [(1, lambda f0=f0, n=n, step=step: ffn_down(f0, n, min(n + step, M // T)))]
    queue.extend([lambda r0=r0: router(r0) for r0 in range(0, S, RU)])
    queue.extend([select_step] * TOPC + [gather])
    if RM == 2:
        queue.extend(lambda r0=r0: residual(r0) for r0 in range(0, S, R2))
    spacing[0] = TS
    if DEV != 1 and DEV != 2:
        head(H - 1, 1, early_steps(0, H - 1))
    else:
        for _, fn in early_steps(0, H - 1):
            fn()
    flush()
    wait(late[:3] if WB else [])
    early_out(0, H - 1, H)
    if RM == 0:
        queue.extend(lambda r0=r0: residual(r0) for r0 in range(0, S, R2))
    spacing[0] = RS
    for _, fn in _merge([st for i in range(1, NF + 1) for st in early_steps(i, H)],
                        side + [(0, lambda: None)] * PAD):
        fn()
    flush()
    pending.clear()
    y = jnp.concatenate([ffn["y", n] * ffn["gain"] for n in range(M // T)], axis=1)
    olds = [acc_v[pl.ds(row, 1), :] for row in rows_sel]
    for j, row in enumerate(rows_sel):
        acc_v[pl.ds(row, 1), :] = olds[j] + y[j:j + 1, :]

    def finish(rp, attn):
        rows = pl.ds(2 * rp, OB)
        o_v[rows, :] = (acc_v[rows, :] + attn).astype(BF16)
        pltpu.make_async_copy(o_v.at[rows], out_hbm.at[rows], osem).start()

    for i in range(NF + 1, NU):
        steps = early_steps(i, H)
        for n, (_, fn) in enumerate(steps):
            fn()
            if n % 8 == FO and len(early) > 1:
                j = min(early)
                finish(j * OB // 2, early.pop(j))
    for j in sorted(early):
        finish(j * OB // 2, early[j])

    def out_body(b, carry):
        for u in range(OR):
            rp = pl.multiple_of((NU + b * OR + u) * (OB // 2), OB // 2)
            finish(rp, out_project(rp, 0, H))
        return carry

    lax.fori_loop(0, (S // OB - NU) // OR, out_body, 0)
    pltpu.make_async_copy(o_v, out_hbm, osem).wait()


@jax.jit
def pallas_parallel_sum__compressed_kv_cla__moe_arch_mod__prompt_kernel(
    A_x: jax.Array,
    A_c_kv: jax.Array,
    A_w_q: jax.Array,
    A_w_uk: jax.Array,
    A_w_uv: jax.Array,
    A_w_o: jax.Array,
    B_x: jax.Array,
    B_w_r: jax.Array,
    B_w_gate: jax.Array,
    B_w_up: jax.Array,
    B_w_down: jax.Array,
):
    del B_x
    _, S, M = A_x.shape
    DC = A_c_kv.shape[2]
    H, D = A_w_q.shape[1], A_w_q.shape[2]
    FF = B_w_gate.shape[1]
    hbm = pl.BlockSpec(memory_space=pltpu.HBM)
    out = pl.pallas_call(
        _kernel,
        out_shape=jax.ShapeDtypeStruct((S, M), A_x.dtype),
        in_specs=[hbm] * 6 + [pl.BlockSpec(memory_space=pltpu.VMEM)] + [hbm] * 3,
        out_specs=hbm,
        scratch_shapes=[
            pltpu.VMEM((S // 2, M), U32),
            pltpu.VMEM((S // 2, DC), U32),
            pltpu.VMEM((H // 2, M + 2 * DC, D), U32),
            pltpu.VMEM((H * D // 2, M), U32),
            pltpu.VMEM((FF // 2, M), U32),
            pltpu.VMEM((FF // 2, M), U32),
            pltpu.VMEM((FF // 2, M), U32),
            pltpu.VMEM((S // 2, M), U32),
            pltpu.VMEM((2, S // 2, D), U32),
            pltpu.VMEM((2, S // 2, D), U32),
            pltpu.VMEM((2, S // 2, D), U32),
            pltpu.VMEM((2, (M + 2 * DC) // 2, D), U32),
            pltpu.VMEM((H, S // 2, D), U32),
            pltpu.VMEM((S, M), F32),
            pltpu.VMEM((S, M), BF16),
            pltpu.SemaphoreType.DMA((2 * len(XA),)),
            pltpu.SemaphoreType.DMA((3 * H // 2,)),
            pltpu.SemaphoreType.DMA((4,)),
            pltpu.SemaphoreType.DMA(()),
        ],
        compiler_params=pltpu.CompilerParams(vmem_limit_bytes=100 * 1024 * 1024),
    )(
        A_x.reshape(S, M),
        A_c_kv.reshape(S, DC),
        A_w_q,
        A_w_uk,
        A_w_uv,
        A_w_o.reshape(H * D, M),
        B_w_r,
        B_w_gate.T,
        B_w_up.T,
        B_w_down,
    )
    return out.reshape(1, S, M)
```

```python
import math

import numpy as np
import jax
import jax.numpy as jnp
from jax import lax
import jax.experimental.pallas as pl
import jax.experimental.pallas.tpu as pltpu

BF16 = jnp.bfloat16
F32 = jnp.float32
U32 = jnp.uint32
TOPC = 8
LN_EPS = float(np.float32(np.asarray(1e-5, dtype=jnp.bfloat16)))
NEG = -1e30
KEY0 = 0x10000000
T = 128
CK = 4
LAG = 10
ORDER = 1
BIAS = 0
XB = (0, 1, 2, 4, 8, 12, 16)
XA = (-1, 1, 2, 4, 8, 11)
XT = (-1, -1, -1, -1, -1, -1)
XS = -1
PRI = 1
QD = 1
OR = 2
TIE = 1
GATE = 3
GR = 120
AHEAD = 3
VL = 3
OB = 128
OK = 1
NF = 2
NU = 4
OL = 256
PX = 1
PW = 1
LU = 128
DL = 4
TS = 4
RS = 1
RM = 0
WB = 1
PAD = 10
FO = 3
PK = 0
PO = 0
CF = 0
R2 = 32
DS = 13
RU = 128
FL = 2
H1 = 4
H2 = 2
GB = 2
DEV = 0


def _rb(v):
    return v.astype(BF16).astype(F32)


def _dot(a, b):
    return jnp.dot(a, b, preferred_element_type=F32)


def _dot_nt(a, b):
    return lax.dot_general(a, b, (((1,), (1,)), ((), ())), preferred_element_type=F32)


def _recip(v):
    inv = pl.reciprocal(v, approx=True)
    return inv * (2.0 - v * inv)


def _ld(ref, r0, n, *lead):
    return pltpu.bitcast(ref[(*lead, pl.ds(r0 // 2, n // 2), slice(None))], BF16)


def _st(ref, r0, val, *lead):
    n = val.shape[0]
    ref[(*lead, pl.ds(r0 // 2, n // 2), slice(None))] = pltpu.bitcast(val.astype(BF16), U32)


def _pack(pair):
    return pltpu.bitcast(pltpu.pack_elementwise(pair, packed_dtype=BF16), U32)


def _st_keys(ref, r0, val, buf):
    if not PK:
        return _st(ref, r0, val, buf)
    words = [_pack([val[r:r + 8], val[r + 8:r + 16]]) for r in range(0, val.shape[0], 16)]
    ref[buf, pl.ds(r0 // 2, val.shape[0] // 2), :] = jnp.concatenate(words, axis=0)


def _key_order(pos):
    if not PK:
        return pos
    return (pos & ~15) | ((pos & 1) << 3) | ((pos & 15) >> 1)


def _unpack(w32):
    return [pltpu.bitcast(w32 << 16, F32), pltpu.bitcast(w32 & U32(0xFFFF0000), F32)]


def _tree(op, xs):
    while len(xs) > 1:
        xs = [op(xs[i], xs[i + 1]) if i + 1 < len(xs) else xs[i] for i in range(0, len(xs), 2)]
    return xs[0]


def _tiles(v):
    return [v[:, j * T:(j + 1) * T] for j in range(v.shape[1] // T)]


def _rowsum(v):
    return jnp.sum(_tree(jnp.add, _tiles(v)), axis=-1, keepdims=True)


def _merge(*lists):
    keyed = []
    for k, items in enumerate(lists):
        keyed += [((j + 0.5) / len(items), k, j) for j in range(len(items))]
    return [lists[k][j] for _, k, j in sorted(keyed)]


def _kernel(x_hbm, c_hbm, wq_hbm, wuk_hbm, wuv_hbm, wo_hbm, wr_ref, wg_hbm, wu_hbm, wd_hbm,
            out_hbm,
            x_v, c_v, wp_v, wo_v, wg_v, wu_v, wd_v,
            xn_v, q_v, k_v, v_v, wh_v, ctx_v, acc_v, o_v, xsems, wsems, lsems, osem):
    S, M, DC = 2 * x_v.shape[0], x_v.shape[1], c_v.shape[1]
    H, D = ctx_v.shape[0], ctx_v.shape[2]
    NB, NX, NPAIR, WT = S // T, len(XA), H // 2, (M + 2 * DC) // T

    def in_copies(j):
        rows = pl.ds(XB[j] * T // 2, (XB[j + 1] - XB[j]) * T // 2)
        return [pltpu.make_async_copy(src.bitcast(U32).at[rows], dst.at[rows], xsems.at[2 * j + i])
                for i, (src, dst) in enumerate(((c_hbm, c_v), (x_hbm, x_v)))]

    def pair_copies(g):
        return [pltpu.make_async_copy(src.bitcast(U32).at[:, g, :],
                                      wp_v.at[g, pl.ds(r0, n)], wsems.at[3 * g + i])
                for i, (src, r0, n) in enumerate(
                    ((wuk_hbm, M, DC), (wuv_hbm, M + DC, DC), (wq_hbm, 0, M)))]

    late = [pltpu.make_async_copy(s.bitcast(U32), d, lsems.at[i]) for i, (s, d) in enumerate(
        ((wg_hbm, wg_v), (wu_hbm, wu_v), (wd_hbm, wd_v), (wo_hbm, wo_v)))]

    def start(cps):
        for cp in cps:
            cp.start()

    def wait(cps):
        for cp in cps:
            cp.wait()

    first_w = pair_copies(0)
    start(first_w)

    def start_inputs(after):
        for j in range(NX):
            if XT[j] == after:
                for cp, pri in zip(in_copies(j), (PRI, PX)):
                    cp.start(priority=pri if j else 0)
        if after == XS:
            for cp in [cp for g in range(1, NPAIR) for cp in pair_copies(g)]:
                cp.start(priority=PW)

    start_inputs(-1)

    lane = lax.broadcasted_iota(jnp.int32, (8, T), 1)
    sub = lax.broadcasted_iota(jnp.int32, (8, T), 0)
    qscale = (D ** -0.5) * math.log2(math.e)

    zero = jnp.min(lane)
    zero8 = pl.multiple_of(zero * 8, 8)
    pending = []

    queue = []
    clock = [0]
    spacing = [0]

    def operand(ref, r0, n, buf=None):
        w32 = ref[(() if buf is None else (buf,)) + (pl.ds(r0 // 2, n // 2), slice(None))]
        clock[0] += 1
        due = [fn for t, fn in pending if t < clock[0]]
        pending[:] = [e for e in pending if e[0] >= clock[0]]
        if due:
            top = w32[0:8, 0:T]
            for fn in due:
                top = jnp.where(zero > 0, fn(), top)
            if w32.shape[1] > T:
                top = jnp.concatenate([top, w32[0:8, T:]], axis=1)
            w32 = jnp.concatenate([top, w32[8:]], axis=0)
        if queue and spacing[0] and clock[0] % spacing[0] == 0:
            queue.pop(0)()
        return pltpu.bitcast(w32, BF16)

    def flush(keep=0):
        while len(queue) > keep:
            queue.pop(0)()

    scores_r = [jnp.zeros((8, T), F32) for _ in range(S // (8 * T))]
    wr = wr_ref[...].astype(F32).reshape(1, M)

    arrived = [0]

    def arrive(j):
        arrived[0] = XB[j + 1]
        wait(in_copies(j))
        if j == 0:
            wait(first_w)
        start_inputs(j)
        for r0 in range(XB[j] * T, XB[j + 1] * T, LU):
            queue.append(lambda r0=r0: layernorm(r0))

    def layernorm(r0):
        rows = slice(r0 // 2, (r0 + LU) // 2)
        cens, invs = [], []
        for xf in _unpack(x_v[rows, :]):
            mean = _rowsum(xf) * (1.0 / M)
            mean_b = _rb(mean)
            cen = xf - mean_b
            off = mean - mean_b
            var = jnp.maximum(_rowsum(cen * cen) * (1.0 / M) - off * off, 0.0)
            cens.append(cen)
            invs.append(_recip(_rb(jnp.sqrt(_rb(_rb(var) + LN_EPS)))))
        xn_v[rows, :] = _pack([cen * inv for cen, inv in zip(_unpack(_pack(cens)), invs)])

    def router(r0):
        if RM == 1:
            residual(r0)
        r = _rowsum(_ld(xn_v, r0, RU).astype(F32) * wr)
        for g in range(RU // 8):
            k, ln = divmod(r0 // 8 + g, T)
            scores_r[k] = jnp.where(lane == ln, r[g * 8:(g + 1) * 8, :], scores_r[k])
        done = scores_r[k]
        pending.append((clock[0] + DL, lambda: pltpu.bitcast(done, U32)))

    def residual(r0):
        acc_v[r0:r0 + R2, :] = _ld(x_v, r0, R2).astype(F32) + _ld(xn_v, r0, R2).astype(F32)
        tok = pltpu.bitcast(acc_v[pl.ds(zero8, 8), 0:T], U32)
        pending.append((clock[0] + DL, lambda: tok))

    def unpack_weights(g, odd_head, t):
        even = wp_v[g, pl.ds(t * T, T // 2, stride=2), :]
        odd = wp_v[g, pl.ds(t * T + 1, T // 2, stride=2), :]
        if odd_head:
            w = (even >> 16) | (odd & U32(0xFFFF0000))
        else:
            w = (even & U32(0xFFFF)) | (odd << 16)
        wh_v[odd_head, pl.ds(t * T // 2, T // 2), :] = w

    def project_q(i, buf):
        _st(q_v, i * T, _dot(operand(xn_v, i * T, T), _ld(wh_v, 0, M, buf)) * qscale, buf)

    def project_k(i, buf):
        _st_keys(k_v, i * T, _dot(operand(c_v, i * T, T), _ld(wh_v, M, DC, buf)), buf)

    def project_v(i, buf, after=None):
        c = pltpu.bitcast(operand(c_v, i * T, T), U32)
        if after is not None:
            tok = jnp.broadcast_to(pltpu.bitcast(
                jnp.broadcast_to(after[T - 8:T], (8, T)), U32)[None], (DC // T, 8, T))
            top = jnp.where(zero > 0, jnp.concatenate(list(tok), axis=1), c[0:8])
            c = jnp.concatenate([top, c[8:]], axis=0)
        _st_keys(v_v, i * T, _dot(pltpu.bitcast(c, BF16), _ld(wh_v, M + DC, DC, buf)), buf)

    def projections(buf):
        ks = [(DC // T, lambda i=i: project_k(i, buf)) for i in range(NB)]
        qs = [(M // T, lambda i=i: project_q(i, buf)) for i in order]
        vs = [(DC // T, lambda i=i, **kw: project_v(i, buf, **kw)) for i in range(NB)]
        if PO == 1:
            return ks + qs + vs
        if PO == 2:
            return qs + ks + vs
        if PO == 3:
            return _merge(ks, qs, vs[:NB - H1 - H2]) + vs[NB - H1 - H2:]
        return _merge(ks, qs) + vs

    def scores(i, t, n, buf, st):
        tiles = _tiles(_dot_nt(operand(q_v, i * T, T, buf), _ld(k_v, t * T, n * T, buf)))
        if t + n == i + 1:
            row = lax.broadcasted_iota(jnp.int32, (T, T), 0)
            col = _key_order(lax.broadcasted_iota(jnp.int32, (T, T), 1))
            tiles[-1] = jnp.where(col <= row, tiles[-1], NEG)
        st[t] = jnp.concatenate(tiles, axis=1) if n > 1 else tiles[0]
        st["m"] = _tree(jnp.maximum, tiles + ([st["m"]] if t else []))
        if t + n == i + 1:
            st["m"] = jnp.max(st["m"], axis=-1, keepdims=True)

    link = {}

    def context(i, t, n, h, buf, st):
        if GATE and t // CK == GATE:
            tok = st["pv"][0][GR:GR + 8]
            st["m"] = jnp.where(zero > 0, jnp.concatenate([tok] * (T // 8), axis=0), st["m"])
        m = st["m"]
        if m.shape[1] == T and n > 1:
            m = jnp.concatenate([m] * n, axis=1)
        d = st[t] - m
        if TIE and t == 0 and "tie" in link:
            d0 = jnp.minimum(d[:, 0:T], link["tie"])
            d = jnp.concatenate([d0, d[:, T:]], axis=1) if n > 1 else d0
        p = jnp.exp2(d)
        lp = _tree(jnp.add, _tiles(p))
        o = _dot(p.astype(BF16), operand(v_v, t * T, n * T, buf))
        st.setdefault("pv", []).append(o)
        if t:
            lp, o = st["l"] + lp, st["o"] + o
        st["l"], st["o"] = lp, o
        if t + n == i + 1:
            o = o * _recip(jnp.sum(lp, axis=-1, keepdims=True))
            link["tie"] = jnp.abs(o)
            _st(ctx_v, i * T, o, h)

    order = [list(range(NB))[::-1], list(range(NB)),
             list(range(1, NB, 2)) + list(range(0, NB, 2))[::-1],
             [j for i in range(NB // 2) for j in (NB - 1 - i, i)]][ORDER]

    def head(h, buf, fillers, hold=False, before=None):
        work = [(i, t, min(CK, i + 1 - t)) for i in order for t in range(0, i + 1, CK)]
        state = {i: {} for i in order}
        held = []
        if hold:
            fillers, held = fillers[:len(fillers) - H1 - H2], fillers[len(fillers) - H1 - H2:]
        att_total = 2 * sum(n for _, _, n in work)
        fill_total = sum(c for c, _ in fillers)
        a = b = f = att = fill = 0
        ready = {}
        last_was_scores = False
        while b < len(work) or f < len(fillers):
            b_ok = b < len(work) and ready.get(work[b][0], 1 << 30) <= att + fill
            if f < len(fillers) and ((fill - BIAS) * att_total < att * fill_total
                                     or (a == len(work) and not b_ok)):
                fillers[f][1]()
                fill += fillers[f][0]
                f += 1
            elif a < len(work) and not (b_ok and last_was_scores):
                i, t, n = work[a]
                if before is not None and t == 0:
                    fill += before(i)
                scores(i, t, n, buf, state[i])
                a += 1
                att += n
                last_was_scores = True
                if t + n == i + 1:
                    ready[i] = att + fill + LAG
                if a == len(work) and hold:
                    for _, fn in held[:H1]:
                        fn(after=tok)
                tok = state[i][t][:, 0:T]
            else:
                i, t, n = work[b]
                context(i, t, n, h, buf, state[i])
                b += 1
                att += n
                last_was_scores = False

        for _, fn in held[H1:]:
            fn(after=state[order[-1]]["pv"][-GB])

    def unpacking(g, odd_head):
        return [(0, lambda t=t: unpack_weights(g, odd_head, t)) for t in range(WT)]

    keys = []
    sel = []

    def select_step():
        if not keys:
            for k, rd in enumerate(scores_r):
                bits = pltpu.bitcast(_rb(rd), jnp.int32) >> 16
                mag = bits & 0x7FFF
                rank = jnp.where(bits < 0, 0x8000 - mag, 0x8000 + mag)
                rank = jnp.where(mag > 0x7F80, 0, rank)
                row = k * 8 * T + lane * 8 + sub
                keys.append(pltpu.bitcast(rank * S + (S - 1 - row) + KEY0, F32))
        top = jnp.max(jnp.max(_tree(jnp.maximum, keys), axis=0, keepdims=True), axis=1, keepdims=True)
        top = jnp.broadcast_to(top, (8, T))
        sel.append(pltpu.bitcast(top, jnp.int32) - KEY0)
        keys[:] = [jnp.where(kk == top, 0.0, kk) for kk in keys]
        pending.append((clock[0] + DL, lambda: pltpu.bitcast(top, U32)))

    def first_weights(k):
        t0, n = ((M // T, DC // T), ((M + DC) // T, DC // T), (0, M // T))[k]
        for t in range(t0, t0 + n):
            unpack_weights(0, 0, t)
            unpack_weights(0, 1, t)

    def prepare(i):
        cost = 0
        for j in range(NX):
            if XA[j] == i:
                arrive(j)
        if i < NB:
            if i == 0:
                first_weights(0)
            project_k(i, 0)
            project_k(i, 1)
            if i == 0:
                first_weights(1)
            project_v(i, 0)
            cost += 3 * DC // T
        if 0 <= i - QD < NB:
            if i == QD:
                first_weights(2)
            flush(keep=(arrived[0] - (i - QD + 1)) * T // LU)
            project_q(i - QD, 0)
            project_q(i - QD, 1)
            cost += 2 * M // T
        if i == DS:
            wait(pair_copies(1))
            start(late)
        lo = NB + AHEAD - VL
        if i >= lo:
            for j in range((i - lo) * NB // VL, (i - lo + 1) * NB // VL):
                project_v(j, 1)
                cost += DC // T
        return cost

    for j in range(NX):
        if XA[j] < 0:
            arrive(j)
    for i in range(AHEAD):
        prepare(i)
    if DEV != 1 and DEV != 3:
        head(0, 0, [], before=lambda i: prepare(i + AHEAD))
    else:
        prepare(DS)
    for _, fn in unpacking(1, 0):
        fn()

    def pair_body(g, carry):
        pending.clear()
        link.clear()

        @pl.when(g + 1 < NPAIR)
        def _():
            wait(pair_copies(g + 1))

        if DEV > 1:
            return carry
        head(2 * g - 1, 1, _merge(projections(0), unpacking(g, 1)))
        head(2 * g, 0, unpacking(jnp.minimum(g + 1, NPAIR - 1), 0) + projections(1), hold=True)
        return carry

    lax.fori_loop(1, NPAIR, pair_body, 0)
    pending.clear()
    link.clear()
    wait(late[3:] if WB else late)

    ffn = {}
    rows_sel = []

    def gather():
        sub8m = lax.broadcasted_iota(jnp.int32, (TOPC, M), 0)
        xs = jnp.zeros((TOPC, M), F32)
        key_col = jnp.zeros((TOPC, T), jnp.int32)
        for j, top in enumerate(sel):
            row = S - 1 - (top[0, 0] & (S - 1))
            rows_sel.append(row)
            w32 = xn_v[pl.ds(row >> 1, 1), :] << (16 - 16 * (row & 1)).astype(U32)
            xs = jnp.where(sub8m == j, pltpu.bitcast(w32 & U32(0xFFFF0000), F32), xs)
            key_col = jnp.where(sub == j, top, key_col)
        rank = key_col >> (S.bit_length() - 1)
        bits = jnp.where(rank >= 0x8000, rank - 0x8000, (0x8000 - rank) | 0x8000)
        bits = jnp.where(rank == 0, 0x7FC0, bits)
        ffn["gain"] = jax.nn.sigmoid(pltpu.bitcast(bits << 16, F32))
        ffn["x"] = xs.astype(BF16)

    FF = 2 * wd_v.shape[0]

    FG = 4 * T

    def ffn_in(name, w_v, f0, k):
        w = pltpu.bitcast(w_v[f0 // 2:min(f0 + FG, FF) // 2, k * T:(k + 1) * T], BF16)
        part = _dot_nt(ffn["x"][:, k * T:(k + 1) * T], w)
        ffn[name, f0] = ffn[name, f0] + part if k else part

    def ffn_down(f0, n0, n1):
        if n0 == 0:
            g, u = ffn["g", f0], ffn["u", f0]
            ffn["h", f0] = (g * jax.nn.sigmoid(g) * u).astype(BF16)
        w = pltpu.bitcast(wd_v[f0 // 2:min(f0 + FG, FF) // 2, n0 * T:n1 * T], BF16)
        for n, part in zip(range(n0, n1), _tiles(_dot(ffn["h", f0], w))):
            ffn["y", n] = ffn["y", n] + part if f0 else part

    def out_project(rp, h0, h1, n=OB):
        ctx = jnp.concatenate(
            [pltpu.bitcast(ctx_v[h, pl.ds(rp, n // 2), :], BF16) for h in range(h0, h1)], axis=1)
        return _dot(ctx, operand(wo_v, h0 * D, (h1 - h0) * D))

    early = {}

    def early_out(i, h0, h1):
        part = out_project(i * OB // 2, h0, h1)
        early[i] = early[i] + part if h0 else part

    def early_steps(i, nh):
        return [(M // T * OB // T * (min(h0 + OK, nh) - h0),
                 lambda h0=h0: early_out(i, h0, min(h0 + OK, nh))) for h0 in range(0, nh, OK)]

    side = []
    for f0 in range(0, FF, FG):
        for k in range(M // T):
            gate = lambda f0=f0, k=k: ffn_in("g", wg_v, f0, k)
            up = lambda f0=f0, k=k: ffn_in("u", wu_v, f0, k)
            if f0 + FG <= FF:
                side += [(1, gate), (1, up)]
            else:
                side += [(1, lambda gate=gate, up=up: (gate(), up()))]
    for f0 in range(0, FF, FG):
        step = 1 if f0 + FG <= FF else 2
        for n in range(0, M // T, step):
            side += [(1, lambda f0=f0, n=n, step=step: ffn_down(f0, n, min(n + step, M // T)))]
    queue.extend([lambda r0=r0: router(r0) for r0 in range(0, S, RU)])
    queue.extend([select_step] * TOPC + [gather])
    if RM == 2:
        queue.extend(lambda r0=r0: residual(r0) for r0 in range(0, S, R2))
    spacing[0] = TS
    if DEV != 1 and DEV != 2:
        head(H - 1, 1, early_steps(0, H - 1))
    else:
        for _, fn in early_steps(0, H - 1):
            fn()
    flush()
    wait(late[:3] if WB else [])
    early_out(0, H - 1, H)
    if RM == 0:
        queue.extend(lambda r0=r0: residual(r0) for r0 in range(0, S, R2))
    spacing[0] = RS
    for _, fn in _merge([st for i in range(1, NF + 1) for st in early_steps(i, H)],
                        side + [(0, lambda: None)] * PAD):
        fn()
    flush()
    pending.clear()
    y = jnp.concatenate([ffn["y", n] * ffn["gain"] for n in range(M // T)], axis=1)
    olds = [acc_v[pl.ds(row, 1), :] for row in rows_sel]
    for j, row in enumerate(rows_sel):
        acc_v[pl.ds(row, 1), :] = olds[j] + y[j:j + 1, :]

    def finish(rp, attn):
        rows = pl.ds(2 * rp, attn.shape[0])
        o_v[rows, :] = (acc_v[rows, :] + attn).astype(BF16)
        pltpu.make_async_copy(o_v.at[rows], out_hbm.at[rows], osem).start()

    for i in range(NF + 1, NU):
        steps = early_steps(i, H)
        for n, (_, fn) in enumerate(steps):
            fn()
            if n % 8 == FO and len(early) > 1:
                j = min(early)
                finish(j * OB // 2, early.pop(j))
    for j in sorted(early):
        finish(j * OB // 2, early[j])

    def out_body(b, carry):
        for u in range(OR):
            rp = pl.multiple_of((NU * OB + (b * OR + u) * OL) // 2, OB // 2)
            finish(rp, out_project(rp, 0, H, OL))
        return carry

    lax.fori_loop(0, (S - NU * OB) // (OR * OL), out_body, 0)
    pltpu.make_async_copy(o_v, out_hbm, osem).wait()


@jax.jit
def pallas_parallel_sum__compressed_kv_cla__moe_arch_mod__prompt_kernel(
    A_x: jax.Array,
    A_c_kv: jax.Array,
    A_w_q: jax.Array,
    A_w_uk: jax.Array,
    A_w_uv: jax.Array,
    A_w_o: jax.Array,
    B_x: jax.Array,
    B_w_r: jax.Array,
    B_w_gate: jax.Array,
    B_w_up: jax.Array,
    B_w_down: jax.Array,
):
    del B_x
    _, S, M = A_x.shape
    DC = A_c_kv.shape[2]
    H, D = A_w_q.shape[1], A_w_q.shape[2]
    FF = B_w_gate.shape[1]
    hbm = pl.BlockSpec(memory_space=pltpu.HBM)
    out = pl.pallas_call(
        _kernel,
        out_shape=jax.ShapeDtypeStruct((S, M), A_x.dtype),
        in_specs=[hbm] * 6 + [pl.BlockSpec(memory_space=pltpu.VMEM)] + [hbm] * 3,
        out_specs=hbm,
        scratch_shapes=[
            pltpu.VMEM((S // 2, M), U32),
            pltpu.VMEM((S // 2, DC), U32),
            pltpu.VMEM((H // 2, M + 2 * DC, D), U32),
            pltpu.VMEM((H * D // 2, M), U32),
            pltpu.VMEM((FF // 2, M), U32),
            pltpu.VMEM((FF // 2, M), U32),
            pltpu.VMEM((FF // 2, M), U32),
            pltpu.VMEM((S // 2, M), U32),
            pltpu.VMEM((2, S // 2, D), U32),
            pltpu.VMEM((2, S // 2, D), U32),
            pltpu.VMEM((2, S // 2, D), U32),
            pltpu.VMEM((2, (M + 2 * DC) // 2, D), U32),
            pltpu.VMEM((H, S // 2, D), U32),
            pltpu.VMEM((S, M), F32),
            pltpu.VMEM((S, M), BF16),
            pltpu.SemaphoreType.DMA((2 * len(XA),)),
            pltpu.SemaphoreType.DMA((3 * H // 2,)),
            pltpu.SemaphoreType.DMA((4,)),
            pltpu.SemaphoreType.DMA(()),
        ],
        compiler_params=pltpu.CompilerParams(vmem_limit_bytes=100 * 1024 * 1024),
    )(
        A_x.reshape(S, M),
        A_c_kv.reshape(S, DC),
        A_w_q,
        A_w_uk,
        A_w_uv,
        A_w_o.reshape(H * D, M),
        B_w_r,
        B_w_gate.T,
        B_w_up.T,
        B_w_down,
    )
    return out.reshape(1, S, M)
```

```python
import math

import numpy as np
import jax
import jax.numpy as jnp
from jax import lax
import jax.experimental.pallas as pl
import jax.experimental.pallas.tpu as pltpu

BF16 = jnp.bfloat16
F32 = jnp.float32
U32 = jnp.uint32
TOPC = 8
LN_EPS = float(np.float32(np.asarray(1e-5, dtype=jnp.bfloat16)))
NEG = -1e30
KEY0 = 0x10000000
T = 128
CK = 4
LAG = 10
ORDER = 1
BIAS = 0
XB = (0, 1, 3, 6, 10, 16)
XA = (-1, 1, 3, 6, 10)
XT = (-1, -1, -1, -1, -1)
XS = -1
PRI = 1
QD = 1
OR = 2
TIE = 1
GATE = 3
GR = 120
AHEAD = 3
VL = 3
OB = 128
OK = 1
NF = 2
NU = 4
OL = 256
PX = 1
PW = 1
LU = 128
DL = 4
TS = 4
RS = 1
RM = 0
WB = 1
PAD = 10
FO = 3
SW = 1
PO = 1
CF = 0
R2 = 32
RU = 128
FL = 2
H1 = 4
H2 = 2
GB = 2
DEV = 0


def _rb(v):
    return v.astype(BF16).astype(F32)


def _dot(a, b):
    return jnp.dot(a, b, preferred_element_type=F32)


def _dot_nt(a, b):
    return lax.dot_general(a, b, (((1,), (1,)), ((), ())), preferred_element_type=F32)


def _recip(v):
    inv = pl.reciprocal(v, approx=True)
    return inv * (2.0 - v * inv)


def _ld(ref, r0, n, *lead):
    return pltpu.bitcast(ref[(*lead, pl.ds(r0 // 2, n // 2), slice(None))], BF16)


def _st(ref, r0, val, *lead):
    n = val.shape[0]
    ref[(*lead, pl.ds(r0 // 2, n // 2), slice(None))] = pltpu.bitcast(val.astype(BF16), U32)


def _tree(op, xs):
    while len(xs) > 1:
        xs = [op(xs[i], xs[i + 1]) if i + 1 < len(xs) else xs[i] for i in range(0, len(xs), 2)]
    return xs[0]


def _tiles(v):
    return [v[:, j * T:(j + 1) * T] for j in range(v.shape[1] // T)]


def _rowsum(v):
    return jnp.sum(_tree(jnp.add, _tiles(v)), axis=-1, keepdims=True)


def _merge(*lists):
    keyed = []
    for k, items in enumerate(lists):
        keyed += [((j + 0.5) / len(items), k, j) for j in range(len(items))]
    return [lists[k][j] for _, k, j in sorted(keyed)]


def _kernel(x_hbm, c_hbm, wq_hbm, wuk_hbm, wuv_hbm, wo_hbm, wr_ref, wg_hbm, wu_hbm, wd_hbm,
            out_hbm,
            x_v, c_v, wp_v, wo_v, wg_v, wu_v, wd_v,
            xn_v, q_v, k_v, v_v, wh_v, ctx_v, acc_v, o_v, xsems, wsems, lsems, osem):
    S, M, DC = 2 * x_v.shape[0], x_v.shape[1], c_v.shape[1]
    H, D = ctx_v.shape[0], ctx_v.shape[2]
    NB, NX, NPAIR, WT = S // T, len(XA), H // 2, (M + 2 * DC) // T

    def in_copies(j):
        rows = pl.ds(XB[j] * T // 2, (XB[j + 1] - XB[j]) * T // 2)
        return [pltpu.make_async_copy(src.bitcast(U32).at[rows], dst.at[rows], xsems.at[2 * j + i])
                for i, (src, dst) in enumerate(((c_hbm, c_v), (x_hbm, x_v)))]

    def pair_copies(g):
        return [pltpu.make_async_copy(src.bitcast(U32).at[:, g, :],
                                      wp_v.at[g, pl.ds(r0, n)], wsems.at[3 * g + i])
                for i, (src, r0, n) in enumerate(
                    ((wuk_hbm, M, DC), (wuv_hbm, M + DC, DC), (wq_hbm, 0, M)))]

    late = [pltpu.make_async_copy(s.bitcast(U32), d, lsems.at[i]) for i, (s, d) in enumerate(
        ((wg_hbm, wg_v), (wu_hbm, wu_v), (wd_hbm, wd_v), (wo_hbm, wo_v)))]

    def start(cps):
        for cp in cps:
            cp.start()

    def wait(cps):
        for cp in cps:
            cp.wait()

    first_w = pair_copies(0)
    start(first_w)

    def start_inputs(after):
        for j in range(NX):
            if XT[j] == after:
                for cp, pri in zip(in_copies(j), (PRI, PX)):
                    cp.start(priority=pri if j else 0)
        if after == XS:
            for cp in [cp for g in range(1, NPAIR) for cp in pair_copies(g)]:
                cp.start(priority=PW)

    start_inputs(-1)

    lane = lax.broadcasted_iota(jnp.int32, (8, T), 1)
    sub = lax.broadcasted_iota(jnp.int32, (8, T), 0)
    qscale = (D ** -0.5) * math.log2(math.e)

    zero = jnp.min(lane)
    zero8 = pl.multiple_of(zero * 8, 8)
    pending = []

    queue = []
    clock = [0]
    spacing = [0]

    def operand(ref, r0, n, buf=None):
        w32 = ref[(() if buf is None else (buf,)) + (pl.ds(r0 // 2, n // 2), slice(None))]
        clock[0] += 1
        due = [fn for t, fn in pending if t < clock[0]]
        pending[:] = [e for e in pending if e[0] >= clock[0]]
        if due:
            top = w32[0:8, 0:T]
            for fn in due:
                top = jnp.where(zero > 0, fn(), top)
            if w32.shape[1] > T:
                top = jnp.concatenate([top, w32[0:8, T:]], axis=1)
            w32 = jnp.concatenate([top, w32[8:]], axis=0)
        if queue and spacing[0] and clock[0] % spacing[0] == 0:
            queue.pop(0)()
        return pltpu.bitcast(w32, BF16)

    def flush(keep=0):
        while len(queue) > keep:
            queue.pop(0)()

    scores_r = [jnp.zeros((8, T), F32) for _ in range(S // (8 * T))]
    wr = wr_ref[...].astype(F32).reshape(1, M)

    arrived = [0]

    def arrive(j):
        arrived[0] = XB[j + 1]
        wait(in_copies(j))
        if j == 0:
            wait(first_w[:1] if SW else first_w)
        if j == 1 and SW:
            wait(first_w[1:])
        start_inputs(j)
        for r0 in range(XB[j] * T, XB[j + 1] * T, LU):
            queue.append(lambda r0=r0: layernorm(r0))

    def layernorm(r0):
        xf = _ld(x_v, r0, LU).astype(F32)
        mean = _rowsum(xf) * (1.0 / M)
        mean_b = _rb(mean)
        cen = xf - mean_b
        off = mean - mean_b
        var = jnp.maximum(_rowsum(cen * cen) * (1.0 / M) - off * off, 0.0)
        _st(xn_v, r0, _rb(cen) * _recip(_rb(jnp.sqrt(_rb(_rb(var) + LN_EPS)))))

    def router(r0):
        if RM == 1:
            residual(r0)
        r = _rowsum(_ld(xn_v, r0, RU).astype(F32) * wr)
        for g in range(RU // 8):
            k, ln = divmod(r0 // 8 + g, T)
            scores_r[k] = jnp.where(lane == ln, r[g * 8:(g + 1) * 8, :], scores_r[k])
        done = scores_r[k]
        pending.append((clock[0] + DL, lambda: pltpu.bitcast(done, U32)))

    def residual(r0):
        acc_v[r0:r0 + R2, :] = _ld(x_v, r0, R2).astype(F32) + _ld(xn_v, r0, R2).astype(F32)
        tok = pltpu.bitcast(acc_v[pl.ds(zero8, 8), 0:T], U32)
        pending.append((clock[0] + DL, lambda: tok))

    def unpack_weights(g, odd_head, t):
        even = wp_v[g, pl.ds(t * T, T // 2, stride=2), :]
        odd = wp_v[g, pl.ds(t * T + 1, T // 2, stride=2), :]
        if odd_head:
            w = (even >> 16) | (odd & U32(0xFFFF0000))
        else:
            w = (even & U32(0xFFFF)) | (odd << 16)
        wh_v[odd_head, pl.ds(t * T // 2, T // 2), :] = w

    def project_q(i, buf):
        _st(q_v, i * T, _dot(operand(xn_v, i * T, T), _ld(wh_v, 0, M, buf)) * qscale, buf)

    def project_k(i, buf):
        _st(k_v, i * T, _dot(operand(c_v, i * T, T), _ld(wh_v, M, DC, buf)), buf)

    def project_v(i, buf, after=None):
        c = pltpu.bitcast(operand(c_v, i * T, T), U32)
        if after is not None:
            tok = jnp.broadcast_to(pltpu.bitcast(
                jnp.broadcast_to(after[T - 8:T], (8, T)), U32)[None], (DC // T, 8, T))
            top = jnp.where(zero > 0, jnp.concatenate(list(tok), axis=1), c[0:8])
            c = jnp.concatenate([top, c[8:]], axis=0)
        _st(v_v, i * T, _dot(pltpu.bitcast(c, BF16), _ld(wh_v, M + DC, DC, buf)), buf)

    def projections(buf):
        ks = [(DC // T, lambda i=i: project_k(i, buf)) for i in range(NB)]
        qs = [(M // T, lambda i=i: project_q(i, buf)) for i in order]
        vs = [(DC // T, lambda i=i, **kw: project_v(i, buf, **kw)) for i in range(NB)]
        if PO == 1:
            return ks + qs + vs
        if PO == 2:
            return qs + ks + vs
        if PO == 3:
            return _merge(ks, qs, vs[:NB - H1 - H2]) + vs[NB - H1 - H2:]
        return _merge(ks, qs) + vs

    def scores(i, t, n, buf, st):
        tiles = _tiles(_dot_nt(operand(q_v, i * T, T, buf), _ld(k_v, t * T, n * T, buf)))
        if t + n == i + 1:
            row = lax.broadcasted_iota(jnp.int32, (T, T), 0)
            col = lax.broadcasted_iota(jnp.int32, (T, T), 1)
            tiles[-1] = jnp.where(col <= row, tiles[-1], NEG)
        st[t] = jnp.concatenate(tiles, axis=1) if n > 1 else tiles[0]
        st["m"] = _tree(jnp.maximum, tiles + ([st["m"]] if t else []))
        if t + n == i + 1:
            st["m"] = jnp.max(st["m"], axis=-1, keepdims=True)

    link = {}

    def context(i, t, n, h, buf, st):
        if GATE and t // CK == GATE:
            tok = st["pv"][0][GR:GR + 8]
            st["m"] = jnp.where(zero > 0, jnp.concatenate([tok] * (T // 8), axis=0), st["m"])
        m = st["m"]
        if m.shape[1] == T and n > 1:
            m = jnp.concatenate([m] * n, axis=1)
        d = st[t] - m
        if TIE and t == 0 and "tie" in link:
            d0 = jnp.minimum(d[:, 0:T], link["tie"])
            d = jnp.concatenate([d0, d[:, T:]], axis=1) if n > 1 else d0
        p = jnp.exp2(d)
        lp = _tree(jnp.add, _tiles(p))
        o = _dot(p.astype(BF16), operand(v_v, t * T, n * T, buf))
        st.setdefault("pv", []).append(o)
        if t:
            lp, o = st["l"] + lp, st["o"] + o
        st["l"], st["o"] = lp, o
        if t + n == i + 1:
            o = o * _recip(jnp.sum(lp, axis=-1, keepdims=True))
            link["tie"] = jnp.abs(o)
            _st(ctx_v, i * T, o, h)

    order = [list(range(NB))[::-1], list(range(NB)),
             list(range(1, NB, 2)) + list(range(0, NB, 2))[::-1],
             [j for i in range(NB // 2) for j in (NB - 1 - i, i)]][ORDER]

    def head(h, buf, fillers, hold=False, before=None):
        work = [(i, t, min(CK, i + 1 - t)) for i in order for t in range(0, i + 1, CK)]
        state = {i: {} for i in order}
        held = []
        if hold:
            fillers, held = fillers[:len(fillers) - H1 - H2], fillers[len(fillers) - H1 - H2:]
        att_total = 2 * sum(n for _, _, n in work)
        fill_total = sum(c for c, _ in fillers)
        a = b = f = att = fill = 0
        ready = {}
        last_was_scores = False
        while b < len(work) or f < len(fillers):
            b_ok = b < len(work) and ready.get(work[b][0], 1 << 30) <= att + fill
            if f < len(fillers) and ((fill - BIAS) * att_total < att * fill_total
                                     or (a == len(work) and not b_ok)):
                fillers[f][1]()
                fill += fillers[f][0]
                f += 1
            elif a < len(work) and not (b_ok and last_was_scores):
                i, t, n = work[a]
                if before is not None and t == 0:
                    fill += before(i)
                scores(i, t, n, buf, state[i])
                a += 1
                att += n
                last_was_scores = True
                if t + n == i + 1:
                    ready[i] = att + fill + LAG
                if a == len(work) and hold:
                    for _, fn in held[:H1]:
                        fn(after=tok)
                tok = state[i][t][:, 0:T]
            else:
                i, t, n = work[b]
                context(i, t, n, h, buf, state[i])
                b += 1
                att += n
                last_was_scores = False

        for _, fn in held[H1:]:
            fn(after=state[order[-1]]["pv"][-GB])

    def unpacking(g, odd_head):
        return [(0, lambda t=t: unpack_weights(g, odd_head, t)) for t in range(WT)]

    keys = []
    sel = []

    def select_step():
        if not keys:
            for k, rd in enumerate(scores_r):
                bits = pltpu.bitcast(_rb(rd), jnp.int32) >> 16
                mag = bits & 0x7FFF
                rank = jnp.where(bits < 0, 0x8000 - mag, 0x8000 + mag)
                rank = jnp.where(mag > 0x7F80, 0, rank)
                row = k * 8 * T + lane * 8 + sub
                keys.append(pltpu.bitcast(rank * S + (S - 1 - row) + KEY0, F32))
        top = jnp.max(jnp.max(_tree(jnp.maximum, keys), axis=0, keepdims=True), axis=1, keepdims=True)
        top = jnp.broadcast_to(top, (8, T))
        sel.append(pltpu.bitcast(top, jnp.int32) - KEY0)
        keys[:] = [jnp.where(kk == top, 0.0, kk) for kk in keys]
        pending.append((clock[0] + DL, lambda: pltpu.bitcast(top, U32)))

    def first_weights(k):
        t0, n = ((M // T, DC // T), ((M + DC) // T, DC // T), (0, M // T))[k]
        for t in range(t0, t0 + n):
            unpack_weights(0, 0, t)
            unpack_weights(0, 1, t)

    def prepare(i):
        cost = 0
        for j in range(NX):
            if XA[j] == i:
                arrive(j)
        if i < NB:
            if i == 0:
                first_weights(0)
            project_k(i, 0)
            project_k(i, 1)
            cost += 2 * DC // T
        if 0 <= i - QD < NB:
            if i == QD:
                first_weights(1)
                first_weights(2)
            project_v(i - QD, 0)
            cost += DC // T
            flush(keep=(arrived[0] - (i - QD + 1)) * T // LU)
            project_q(i - QD, 0)
            project_q(i - QD, 1)
            cost += 2 * M // T
        lo = NB + AHEAD - VL
        if i >= lo:
            for j in range((i - lo) * NB // VL, (i - lo + 1) * NB // VL):
                project_v(j, 1)
                cost += DC // T
        return cost

    for j in range(NX):
        if XA[j] < 0:
            arrive(j)
    for i in range(AHEAD):
        prepare(i)
    if DEV != 1 and DEV != 3:
        head(0, 0, [], before=lambda i: prepare(i + AHEAD))
    else:
        prepare(0)
    wait(pair_copies(1))
    start(late)
    for _, fn in unpacking(1, 0):
        fn()

    def pair_body(g, carry):
        pending.clear()
        link.clear()

        @pl.when(g + 1 < NPAIR)
        def _():
            wait(pair_copies(g + 1))

        if DEV > 1:
            return carry
        head(2 * g - 1, 1, _merge(projections(0), unpacking(g, 1)))
        head(2 * g, 0, unpacking(jnp.minimum(g + 1, NPAIR - 1), 0) + projections(1), hold=True)
        return carry

    lax.fori_loop(1, NPAIR, pair_body, 0)
    pending.clear()
    link.clear()
    wait(late[3:] if WB else late)

    ffn = {}
    rows_sel = []

    def gather():
        sub8m = lax.broadcasted_iota(jnp.int32, (TOPC, M), 0)
        xs = jnp.zeros((TOPC, M), F32)
        key_col = jnp.zeros((TOPC, T), jnp.int32)
        for j, top in enumerate(sel):
            row = S - 1 - (top[0, 0] & (S - 1))
            rows_sel.append(row)
            w32 = xn_v[pl.ds(row >> 1, 1), :] << (16 - 16 * (row & 1)).astype(U32)
            xs = jnp.where(sub8m == j, pltpu.bitcast(w32 & U32(0xFFFF0000), F32), xs)
            key_col = jnp.where(sub == j, top, key_col)
        rank = key_col >> (S.bit_length() - 1)
        bits = jnp.where(rank >= 0x8000, rank - 0x8000, (0x8000 - rank) | 0x8000)
        bits = jnp.where(rank == 0, 0x7FC0, bits)
        ffn["gain"] = jax.nn.sigmoid(pltpu.bitcast(bits << 16, F32))
        ffn["x"] = xs.astype(BF16)

    FF = 2 * wd_v.shape[0]

    FG = 4 * T

    def ffn_in(name, w_v, f0, k):
        w = pltpu.bitcast(w_v[f0 // 2:min(f0 + FG, FF) // 2, k * T:(k + 1) * T], BF16)
        part = _dot_nt(ffn["x"][:, k * T:(k + 1) * T], w)
        ffn[name, f0] = ffn[name, f0] + part if k else part

    def ffn_down(f0, n0, n1):
        if n0 == 0:
            g, u = ffn["g", f0], ffn["u", f0]
            ffn["h", f0] = (g * jax.nn.sigmoid(g) * u).astype(BF16)
        w = pltpu.bitcast(wd_v[f0 // 2:min(f0 + FG, FF) // 2, n0 * T:n1 * T], BF16)
        for n, part in zip(range(n0, n1), _tiles(_dot(ffn["h", f0], w))):
            ffn["y", n] = ffn["y", n] + part if f0 else part

    def out_project(rp, h0, h1, n=OB):
        ctx = jnp.concatenate(
            [pltpu.bitcast(ctx_v[h, pl.ds(rp, n // 2), :], BF16) for h in range(h0, h1)], axis=1)
        return _dot(ctx, operand(wo_v, h0 * D, (h1 - h0) * D))

    early = {}

    def early_out(i, h0, h1):
        part = out_project(i * OB // 2, h0, h1)
        early[i] = early[i] + part if h0 else part

    def early_steps(i, nh):
        return [(M // T * OB // T * (min(h0 + OK, nh) - h0),
                 lambda h0=h0: early_out(i, h0, min(h0 + OK, nh))) for h0 in range(0, nh, OK)]

    side = []
    for f0 in range(0, FF, FG):
        for k in range(M // T):
            gate = lambda f0=f0, k=k: ffn_in("g", wg_v, f0, k)
            up = lambda f0=f0, k=k: ffn_in("u", wu_v, f0, k)
            if f0 + FG <= FF:
                side += [(1, gate), (1, up)]
            else:
                side += [(1, lambda gate=gate, up=up: (gate(), up()))]
    for f0 in range(0, FF, FG):
        step = 1 if f0 + FG <= FF else 2
        for n in range(0, M // T, step):
            side += [(1, lambda f0=f0, n=n, step=step: ffn_down(f0, n, min(n + step, M // T)))]
    queue.extend([lambda r0=r0: router(r0) for r0 in range(0, S, RU)])
    queue.extend([select_step] * TOPC + [gather])
    if RM == 2:
        queue.extend(lambda r0=r0: residual(r0) for r0 in range(0, S, R2))
    spacing[0] = TS
    if DEV != 1 and DEV != 2:
        head(H - 1, 1, early_steps(0, H - 1))
    else:
        for _, fn in early_steps(0, H - 1):
            fn()
    flush()
    wait(late[:3] if WB else [])
    early_out(0, H - 1, H)
    if RM == 0:
        queue.extend(lambda r0=r0: residual(r0) for r0 in range(0, S, R2))
    spacing[0] = RS
    for _, fn in _merge([st for i in range(1, NF + 1) for st in early_steps(i, H)],
                        side + [(0, lambda: None)] * PAD):
        fn()
    flush()
    pending.clear()
    y = jnp.concatenate([ffn["y", n] * ffn["gain"] for n in range(M // T)], axis=1)
    olds = [acc_v[pl.ds(row, 1), :] for row in rows_sel]
    for j, row in enumerate(rows_sel):
        acc_v[pl.ds(row, 1), :] = olds[j] + y[j:j + 1, :]

    def finish(rp, attn):
        rows = pl.ds(2 * rp, attn.shape[0])
        o_v[rows, :] = (acc_v[rows, :] + attn).astype(BF16)
        pltpu.make_async_copy(o_v.at[rows], out_hbm.at[rows], osem).start()

    for i in range(NF + 1, NU):
        steps = early_steps(i, H)
        for n, (_, fn) in enumerate(steps):
            fn()
            if n % 8 == FO and len(early) > 1:
                j = min(early)
                finish(j * OB // 2, early.pop(j))
    for j in sorted(early):
        finish(j * OB // 2, early[j])

    def out_body(b, carry):
        for u in range(OR):
            rp = pl.multiple_of((NU * OB + (b * OR + u) * OL) // 2, OB // 2)
            finish(rp, out_project(rp, 0, H, OL))
        return carry

    lax.fori_loop(0, (S - NU * OB) // (OR * OL), out_body, 0)
    pltpu.make_async_copy(o_v, out_hbm, osem).wait()


@jax.jit
def pallas_parallel_sum__compressed_kv_cla__moe_arch_mod__prompt_kernel(
    A_x: jax.Array,
    A_c_kv: jax.Array,
    A_w_q: jax.Array,
    A_w_uk: jax.Array,
    A_w_uv: jax.Array,
    A_w_o: jax.Array,
    B_x: jax.Array,
    B_w_r: jax.Array,
    B_w_gate: jax.Array,
    B_w_up: jax.Array,
    B_w_down: jax.Array,
):
    del B_x
    _, S, M = A_x.shape
    DC = A_c_kv.shape[2]
    H, D = A_w_q.shape[1], A_w_q.shape[2]
    FF = B_w_gate.shape[1]
    hbm = pl.BlockSpec(memory_space=pltpu.HBM)
    out = pl.pallas_call(
        _kernel,
        out_shape=jax.ShapeDtypeStruct((S, M), A_x.dtype),
        in_specs=[hbm] * 6 + [pl.BlockSpec(memory_space=pltpu.VMEM)] + [hbm] * 3,
        out_specs=hbm,
        scratch_shapes=[
            pltpu.VMEM((S // 2, M), U32),
            pltpu.VMEM((S // 2, DC), U32),
            pltpu.VMEM((H // 2, M + 2 * DC, D), U32),
            pltpu.VMEM((H * D // 2, M), U32),
            pltpu.VMEM((FF // 2, M), U32),
            pltpu.VMEM((FF // 2, M), U32),
            pltpu.VMEM((FF // 2, M), U32),
            pltpu.VMEM((S // 2, M), U32),
            pltpu.VMEM((2, S // 2, D), U32),
            pltpu.VMEM((2, S // 2, D), U32),
            pltpu.VMEM((2, S // 2, D), U32),
            pltpu.VMEM((2, (M + 2 * DC) // 2, D), U32),
            pltpu.VMEM((H, S // 2, D), U32),
            pltpu.VMEM((S, M), F32),
            pltpu.VMEM((S, M), BF16),
            pltpu.SemaphoreType.DMA((2 * len(XA),)),
            pltpu.SemaphoreType.DMA((3 * H // 2,)),
            pltpu.SemaphoreType.DMA((4,)),
            pltpu.SemaphoreType.DMA(()),
        ],
        compiler_params=pltpu.CompilerParams(vmem_limit_bytes=100 * 1024 * 1024),
    )(
        A_x.reshape(S, M),
        A_c_kv.reshape(S, DC),
        A_w_q,
        A_w_uk,
        A_w_uv,
        A_w_o.reshape(H * D, M),
        B_w_r,
        B_w_gate.T,
        B_w_up.T,
        B_w_down,
    )
    return out.reshape(1, S, M)
```

```python
import math

import numpy as np
import jax
import jax.numpy as jnp
from jax import lax
import jax.experimental.pallas as pl
import jax.experimental.pallas.tpu as pltpu

BF16 = jnp.bfloat16
F32 = jnp.float32
U32 = jnp.uint32
TOPC = 8
LN_EPS = float(np.float32(np.asarray(1e-5, dtype=jnp.bfloat16)))
NEG = -1e30
KEY0 = 0x10000000
T = 128
CK = 4
LAG = (12,10)
ORDER = 1
BIAS = (-1,0)
XB = (0, 1, 3, 6, 10, 16)
XA = (-1, 1, 3, 6, 10)
XT = (-1, -1, -1, -1, -1)
XS = -1
PRI = 1
QD = 1
OR = 2
TIE = 1
GATE = (2,0)
GR = (64,96)
AHEAD = 3
VL = 3
OB = 128
OK = 1
NF = 2
NU = 4
OL = 256
PX = 1
PW = 1
LU = 128
DL = 4
TS = 4
RS = 1
RM = 0
WB = 1
PAD = 10
FO = 3
SW = 1
PO = (1,2)
CF = 0
R2 = 32
RU = 128
FL = 2
H1 = 5
H2 = 2
GB = 3
DEV = 0


def _rb(v):
    return v.astype(BF16).astype(F32)


def _dot(a, b):
    return jnp.dot(a, b, preferred_element_type=F32)


def _dot_nt(a, b):
    return lax.dot_general(a, b, (((1,), (1,)), ((), ())), preferred_element_type=F32)


def _recip(v):
    inv = pl.reciprocal(v, approx=True)
    return inv * (2.0 - v * inv)


def _ld(ref, r0, n, *lead):
    return pltpu.bitcast(ref[(*lead, pl.ds(r0 // 2, n // 2), slice(None))], BF16)


def _st(ref, r0, val, *lead):
    n = val.shape[0]
    ref[(*lead, pl.ds(r0 // 2, n // 2), slice(None))] = pltpu.bitcast(val.astype(BF16), U32)


def _tree(op, xs):
    while len(xs) > 1:
        xs = [op(xs[i], xs[i + 1]) if i + 1 < len(xs) else xs[i] for i in range(0, len(xs), 2)]
    return xs[0]


def _tiles(v):
    return [v[:, j * T:(j + 1) * T] for j in range(v.shape[1] // T)]


def _rowsum(v):
    return jnp.sum(_tree(jnp.add, _tiles(v)), axis=-1, keepdims=True)


def _merge(*lists):
    keyed = []
    for k, items in enumerate(lists):
        keyed += [((j + 0.5) / len(items), k, j) for j in range(len(items))]
    return [lists[k][j] for _, k, j in sorted(keyed)]


def _kernel(x_hbm, c_hbm, wq_hbm, wuk_hbm, wuv_hbm, wo_hbm, wr_ref, wg_hbm, wu_hbm, wd_hbm,
            out_hbm,
            x_v, c_v, wp_v, wo_v, wg_v, wu_v, wd_v,
            xn_v, q_v, k_v, v_v, wh_v, ctx_v, acc_v, o_v, xsems, wsems, lsems, osem):
    S, M, DC = 2 * x_v.shape[0], x_v.shape[1], c_v.shape[1]
    H, D = ctx_v.shape[0], ctx_v.shape[2]
    NB, NX, NPAIR, WT = S // T, len(XA), H // 2, (M + 2 * DC) // T

    def in_copies(j):
        rows = pl.ds(XB[j] * T // 2, (XB[j + 1] - XB[j]) * T // 2)
        return [pltpu.make_async_copy(src.bitcast(U32).at[rows], dst.at[rows], xsems.at[2 * j + i])
                for i, (src, dst) in enumerate(((c_hbm, c_v), (x_hbm, x_v)))]

    def pair_copies(g):
        return [pltpu.make_async_copy(src.bitcast(U32).at[:, g, :],
                                      wp_v.at[g, pl.ds(r0, n)], wsems.at[3 * g + i])
                for i, (src, r0, n) in enumerate(
                    ((wuk_hbm, M, DC), (wuv_hbm, M + DC, DC), (wq_hbm, 0, M)))]

    late = [pltpu.make_async_copy(s.bitcast(U32), d, lsems.at[i]) for i, (s, d) in enumerate(
        ((wg_hbm, wg_v), (wu_hbm, wu_v), (wd_hbm, wd_v), (wo_hbm, wo_v)))]

    def start(cps):
        for cp in cps:
            cp.start()

    def wait(cps):
        for cp in cps:
            cp.wait()

    first_w = pair_copies(0)
    start(first_w)

    def start_inputs(after):
        for j in range(NX):
            if XT[j] == after:
                for cp, pri in zip(in_copies(j), (PRI, PX)):
                    cp.start(priority=pri if j else 0)
        if after == XS:
            for cp in [cp for g in range(1, NPAIR) for cp in pair_copies(g)]:
                cp.start(priority=PW)

    start_inputs(-1)

    lane = lax.broadcasted_iota(jnp.int32, (8, T), 1)
    sub = lax.broadcasted_iota(jnp.int32, (8, T), 0)
    qscale = (D ** -0.5) * math.log2(math.e)

    zero = jnp.min(lane)
    zero8 = pl.multiple_of(zero * 8, 8)
    pending = []

    queue = []
    clock = [0]
    spacing = [0]

    def operand(ref, r0, n, buf=None):
        w32 = ref[(() if buf is None else (buf,)) + (pl.ds(r0 // 2, n // 2), slice(None))]
        clock[0] += 1
        due = [fn for t, fn in pending if t < clock[0]]
        pending[:] = [e for e in pending if e[0] >= clock[0]]
        if due:
            top = w32[0:8, 0:T]
            for fn in due:
                top = jnp.where(zero > 0, fn(), top)
            if w32.shape[1] > T:
                top = jnp.concatenate([top, w32[0:8, T:]], axis=1)
            w32 = jnp.concatenate([top, w32[8:]], axis=0)
        if queue and spacing[0] and clock[0] % spacing[0] == 0:
            queue.pop(0)()
        return pltpu.bitcast(w32, BF16)

    def flush(keep=0):
        while len(queue) > keep:
            queue.pop(0)()

    scores_r = [jnp.zeros((8, T), F32) for _ in range(S // (8 * T))]
    wr = wr_ref[...].astype(F32).reshape(1, M)

    arrived = [0]

    def arrive(j):
        arrived[0] = XB[j + 1]
        wait(in_copies(j))
        if j == 0:
            wait(first_w[:1] if SW else first_w)
        if j == 1 and SW:
            wait(first_w[1:])
        start_inputs(j)
        for r0 in range(XB[j] * T, XB[j + 1] * T, LU):
            queue.append(lambda r0=r0: layernorm(r0))

    def layernorm(r0):
        xf = _ld(x_v, r0, LU).astype(F32)
        mean = _rowsum(xf) * (1.0 / M)
        mean_b = _rb(mean)
        cen = xf - mean_b
        off = mean - mean_b
        var = jnp.maximum(_rowsum(cen * cen) * (1.0 / M) - off * off, 0.0)
        _st(xn_v, r0, _rb(cen) * _recip(_rb(jnp.sqrt(_rb(_rb(var) + LN_EPS)))))

    def router(r0):
        if RM == 1:
            residual(r0)
        r = _rowsum(_ld(xn_v, r0, RU).astype(F32) * wr)
        for g in range(RU // 8):
            k, ln = divmod(r0 // 8 + g, T)
            scores_r[k] = jnp.where(lane == ln, r[g * 8:(g + 1) * 8, :], scores_r[k])
        done = scores_r[k]
        pending.append((clock[0] + DL, lambda: pltpu.bitcast(done, U32)))

    def residual(r0):
        acc_v[r0:r0 + R2, :] = _ld(x_v, r0, R2).astype(F32) + _ld(xn_v, r0, R2).astype(F32)
        tok = pltpu.bitcast(acc_v[pl.ds(zero8, 8), 0:T], U32)
        pending.append((clock[0] + DL, lambda: tok))

    def unpack_weights(g, odd_head, t):
        even = wp_v[g, pl.ds(t * T, T // 2, stride=2), :]
        odd = wp_v[g, pl.ds(t * T + 1, T // 2, stride=2), :]
        if odd_head:
            w = (even >> 16) | (odd & U32(0xFFFF0000))
        else:
            w = (even & U32(0xFFFF)) | (odd << 16)
        wh_v[odd_head, pl.ds(t * T // 2, T // 2), :] = w

    def project_q(i, buf):
        _st(q_v, i * T, _dot(operand(xn_v, i * T, T), _ld(wh_v, 0, M, buf)) * qscale, buf)

    def project_k(i, buf):
        _st(k_v, i * T, _dot(operand(c_v, i * T, T), _ld(wh_v, M, DC, buf)), buf)

    def project_v(i, buf, after=None):
        c = pltpu.bitcast(operand(c_v, i * T, T), U32)
        if after is not None:
            tok = jnp.broadcast_to(pltpu.bitcast(
                jnp.broadcast_to(after[T - 8:T], (8, T)), U32)[None], (DC // T, 8, T))
            top = jnp.where(zero > 0, jnp.concatenate(list(tok), axis=1), c[0:8])
            c = jnp.concatenate([top, c[8:]], axis=0)
        _st(v_v, i * T, _dot(pltpu.bitcast(c, BF16), _ld(wh_v, M + DC, DC, buf)), buf)

    def projections(buf):
        ks = [(DC // T, lambda i=i: project_k(i, buf)) for i in range(NB)]
        qs = [(M // T, lambda i=i: project_q(i, buf)) for i in order]
        vs = [(DC // T, lambda i=i, **kw: project_v(i, buf, **kw)) for i in range(NB)]
        if PO[buf] == 1:
            return ks + qs + vs
        if PO[buf] == 2:
            return qs + ks + vs
        if PO[buf] == 3:
            return _merge(ks, qs, vs[:NB - H1 - H2]) + vs[NB - H1 - H2:]
        return _merge(ks, qs) + vs

    def scores(i, t, n, buf, st):
        tiles = _tiles(_dot_nt(operand(q_v, i * T, T, buf), _ld(k_v, t * T, n * T, buf)))
        if t + n == i + 1:
            row = lax.broadcasted_iota(jnp.int32, (T, T), 0)
            col = lax.broadcasted_iota(jnp.int32, (T, T), 1)
            tiles[-1] = jnp.where(col <= row, tiles[-1], NEG)
        st[t] = jnp.concatenate(tiles, axis=1) if n > 1 else tiles[0]
        st["m"] = _tree(jnp.maximum, tiles + ([st["m"]] if t else []))
        if t + n == i + 1:
            st["m"] = jnp.max(st["m"], axis=-1, keepdims=True)

    link = {}

    def context(i, t, n, h, buf, st):
        if GATE[buf] and t // CK == GATE[buf]:
            tok = st["pv"][0][GR[buf]:GR[buf] + 8]
            st["m"] = jnp.where(zero > 0, jnp.concatenate([tok] * (T // 8), axis=0), st["m"])
        m = st["m"]
        if m.shape[1] == T and n > 1:
            m = jnp.concatenate([m] * n, axis=1)
        d = st[t] - m
        if TIE and t == 0 and "tie" in link:
            d0 = jnp.minimum(d[:, 0:T], link["tie"])
            d = jnp.concatenate([d0, d[:, T:]], axis=1) if n > 1 else d0
        p = jnp.exp2(d)
        lp = _tree(jnp.add, _tiles(p))
        o = _dot(p.astype(BF16), operand(v_v, t * T, n * T, buf))
        st.setdefault("pv", []).append(o)
        if t:
            lp, o = st["l"] + lp, st["o"] + o
        st["l"], st["o"] = lp, o
        if t + n == i + 1:
            o = o * _recip(jnp.sum(lp, axis=-1, keepdims=True))
            link["tie"] = jnp.abs(o)
            _st(ctx_v, i * T, o, h)

    order = [list(range(NB))[::-1], list(range(NB)),
             list(range(1, NB, 2)) + list(range(0, NB, 2))[::-1],
             [j for i in range(NB // 2) for j in (NB - 1 - i, i)]][ORDER]

    def head(h, buf, fillers, hold=False, before=None):
        work = [(i, t, min(CK, i + 1 - t)) for i in order for t in range(0, i + 1, CK)]
        state = {i: {} for i in order}
        held = []
        if hold:
            fillers, held = fillers[:len(fillers) - H1 - H2], fillers[len(fillers) - H1 - H2:]
        att_total = 2 * sum(n for _, _, n in work)
        fill_total = sum(c for c, _ in fillers)
        a = b = f = att = fill = 0
        ready = {}
        last_was_scores = False
        while b < len(work) or f < len(fillers):
            b_ok = b < len(work) and ready.get(work[b][0], 1 << 30) <= att + fill
            if f < len(fillers) and ((fill - BIAS[buf]) * att_total < att * fill_total
                                     or (a == len(work) and not b_ok)):
                fillers[f][1]()
                fill += fillers[f][0]
                f += 1
            elif a < len(work) and not (b_ok and last_was_scores):
                i, t, n = work[a]
                if before is not None and t == 0:
                    fill += before(i)
                scores(i, t, n, buf, state[i])
                a += 1
                att += n
                last_was_scores = True
                if t + n == i + 1:
                    ready[i] = att + fill + LAG[buf]
                if a == len(work) and hold:
                    for _, fn in held[:H1]:
                        fn(after=tok)
                tok = state[i][t][:, 0:T]
            else:
                i, t, n = work[b]
                context(i, t, n, h, buf, state[i])
                b += 1
                att += n
                last_was_scores = False

        for _, fn in held[H1:]:
            fn(after=state[order[-1]]["pv"][-GB])

    def unpacking(g, odd_head):
        return [(0, lambda t=t: unpack_weights(g, odd_head, t)) for t in range(WT)]

    keys = []
    sel = []

    def select_step():
        if not keys:
            for k, rd in enumerate(scores_r):
                bits = pltpu.bitcast(_rb(rd), jnp.int32) >> 16
                mag = bits & 0x7FFF
                rank = jnp.where(bits < 0, 0x8000 - mag, 0x8000 + mag)
                rank = jnp.where(mag > 0x7F80, 0, rank)
                row = k * 8 * T + lane * 8 + sub
                keys.append(pltpu.bitcast(rank * S + (S - 1 - row) + KEY0, F32))
        top = jnp.max(jnp.max(_tree(jnp.maximum, keys), axis=0, keepdims=True), axis=1, keepdims=True)
        top = jnp.broadcast_to(top, (8, T))
        sel.append(pltpu.bitcast(top, jnp.int32) - KEY0)
        keys[:] = [jnp.where(kk == top, 0.0, kk) for kk in keys]
        pending.append((clock[0] + DL, lambda: pltpu.bitcast(top, U32)))

    def first_weights(k):
        t0, n = ((M // T, DC // T), ((M + DC) // T, DC // T), (0, M // T))[k]
        for t in range(t0, t0 + n):
            unpack_weights(0, 0, t)
            unpack_weights(0, 1, t)

    def prepare(i):
        cost = 0
        for j in range(NX):
            if XA[j] == i:
                arrive(j)
        if i < NB:
            if i == 0:
                first_weights(0)
            project_k(i, 0)
            project_k(i, 1)
            cost += 2 * DC // T
        if 0 <= i - QD < NB:
            if i == QD:
                first_weights(1)
                first_weights(2)
            project_v(i - QD, 0)
            cost += DC // T
            flush(keep=(arrived[0] - (i - QD + 1)) * T // LU)
            project_q(i - QD, 0)
            project_q(i - QD, 1)
            cost += 2 * M // T
        lo = NB + AHEAD - VL
        if i >= lo:
            for j in range((i - lo) * NB // VL, (i - lo + 1) * NB // VL):
                project_v(j, 1)
                cost += DC // T
        return cost

    for j in range(NX):
        if XA[j] < 0:
            arrive(j)
    for i in range(AHEAD):
        prepare(i)
    if DEV != 1 and DEV != 3:
        head(0, 0, [], before=lambda i: prepare(i + AHEAD))
    else:
        prepare(0)
    wait(pair_copies(1))
    start(late)
    for _, fn in unpacking(1, 0):
        fn()

    def pair_body(g, carry):
        pending.clear()
        link.clear()

        @pl.when(g + 1 < NPAIR)
        def _():
            wait(pair_copies(g + 1))

        if DEV > 1:
            return carry
        head(2 * g - 1, 1, _merge(projections(0), unpacking(g, 1)))
        head(2 * g, 0, unpacking(jnp.minimum(g + 1, NPAIR - 1), 0) + projections(1), hold=True)
        return carry

    lax.fori_loop(1, NPAIR, pair_body, 0)
    pending.clear()
    link.clear()
    wait(late[3:] if WB else late)

    ffn = {}
    rows_sel = []

    def gather():
        sub8m = lax.broadcasted_iota(jnp.int32, (TOPC, M), 0)
        xs = jnp.zeros((TOPC, M), F32)
        key_col = jnp.zeros((TOPC, T), jnp.int32)
        for j, top in enumerate(sel):
            row = S - 1 - (top[0, 0] & (S - 1))
            rows_sel.append(row)
            w32 = xn_v[pl.ds(row >> 1, 1), :] << (16 - 16 * (row & 1)).astype(U32)
            xs = jnp.where(sub8m == j, pltpu.bitcast(w32 & U32(0xFFFF0000), F32), xs)
            key_col = jnp.where(sub == j, top, key_col)
        rank = key_col >> (S.bit_length() - 1)
        bits = jnp.where(rank >= 0x8000, rank - 0x8000, (0x8000 - rank) | 0x8000)
        bits = jnp.where(rank == 0, 0x7FC0, bits)
        ffn["gain"] = jax.nn.sigmoid(pltpu.bitcast(bits << 16, F32))
        ffn["x"] = xs.astype(BF16)

    FF = 2 * wd_v.shape[0]

    FG = 4 * T

    def ffn_in(name, w_v, f0, k):
        w = pltpu.bitcast(w_v[f0 // 2:min(f0 + FG, FF) // 2, k * T:(k + 1) * T], BF16)
        part = _dot_nt(ffn["x"][:, k * T:(k + 1) * T], w)
        ffn[name, f0] = ffn[name, f0] + part if k else part

    def ffn_down(f0, n0, n1):
        if n0 == 0:
            g, u = ffn["g", f0], ffn["u", f0]
            ffn["h", f0] = (g * jax.nn.sigmoid(g) * u).astype(BF16)
        w = pltpu.bitcast(wd_v[f0 // 2:min(f0 + FG, FF) // 2, n0 * T:n1 * T], BF16)
        for n, part in zip(range(n0, n1), _tiles(_dot(ffn["h", f0], w))):
            ffn["y", n] = ffn["y", n] + part if f0 else part

    def out_project(rp, h0, h1, n=OB):
        ctx = jnp.concatenate(
            [pltpu.bitcast(ctx_v[h, pl.ds(rp, n // 2), :], BF16) for h in range(h0, h1)], axis=1)
        return _dot(ctx, operand(wo_v, h0 * D, (h1 - h0) * D))

    early = {}

    def early_out(i, h0, h1):
        part = out_project(i * OB // 2, h0, h1)
        early[i] = early[i] + part if h0 else part

    def early_steps(i, nh):
        return [(M // T * OB // T * (min(h0 + OK, nh) - h0),
                 lambda h0=h0: early_out(i, h0, min(h0 + OK, nh))) for h0 in range(0, nh, OK)]

    side = []
    for f0 in range(0, FF, FG):
        for k in range(M // T):
            gate = lambda f0=f0, k=k: ffn_in("g", wg_v, f0, k)
            up = lambda f0=f0, k=k: ffn_in("u", wu_v, f0, k)
            if f0 + FG <= FF:
                side += [(1, gate), (1, up)]
            else:
                side += [(1, lambda gate=gate, up=up: (gate(), up()))]
    for f0 in range(0, FF, FG):
        step = 1 if f0 + FG <= FF else 2
        for n in range(0, M // T, step):
            side += [(1, lambda f0=f0, n=n, step=step: ffn_down(f0, n, min(n + step, M // T)))]
    queue.extend([lambda r0=r0: router(r0) for r0 in range(0, S, RU)])
    queue.extend([select_step] * TOPC + [gather])
    if RM == 2:
        queue.extend(lambda r0=r0: residual(r0) for r0 in range(0, S, R2))
    spacing[0] = TS
    if DEV != 1 and DEV != 2:
        head(H - 1, 1, early_steps(0, H - 1))
    else:
        for _, fn in early_steps(0, H - 1):
            fn()
    flush()
    wait(late[:3] if WB else [])
    early_out(0, H - 1, H)
    if RM == 0:
        queue.extend(lambda r0=r0: residual(r0) for r0 in range(0, S, R2))
    spacing[0] = RS
    for _, fn in _merge([st for i in range(1, NF + 1) for st in early_steps(i, H)],
                        side + [(0, lambda: None)] * PAD):
        fn()
    flush()
    pending.clear()
    y = jnp.concatenate([ffn["y", n] * ffn["gain"] for n in range(M // T)], axis=1)
    olds = [acc_v[pl.ds(row, 1), :] for row in rows_sel]
    for j, row in enumerate(rows_sel):
        acc_v[pl.ds(row, 1), :] = olds[j] + y[j:j + 1, :]

    def finish(rp, attn):
        rows = pl.ds(2 * rp, attn.shape[0])
        o_v[rows, :] = (acc_v[rows, :] + attn).astype(BF16)
        pltpu.make_async_copy(o_v.at[rows], out_hbm.at[rows], osem).start()

    for i in range(NF + 1, NU):
        steps = early_steps(i, H)
        for n, (_, fn) in enumerate(steps):
            fn()
            if n % 8 == FO and len(early) > 1:
                j = min(early)
                finish(j * OB // 2, early.pop(j))
    for j in sorted(early):
        finish(j * OB // 2, early[j])

    def out_body(b, carry):
        for u in range(OR):
            rp = pl.multiple_of((NU * OB + (b * OR + u) * OL) // 2, OB // 2)
            finish(rp, out_project(rp, 0, H, OL))
        return carry

    lax.fori_loop(0, (S - NU * OB) // (OR * OL), out_body, 0)
    pltpu.make_async_copy(o_v, out_hbm, osem).wait()


@jax.jit
def pallas_parallel_sum__compressed_kv_cla__moe_arch_mod__prompt_kernel(
    A_x: jax.Array,
    A_c_kv: jax.Array,
    A_w_q: jax.Array,
    A_w_uk: jax.Array,
    A_w_uv: jax.Array,
    A_w_o: jax.Array,
    B_x: jax.Array,
    B_w_r: jax.Array,
    B_w_gate: jax.Array,
    B_w_up: jax.Array,
    B_w_down: jax.Array,
):
    del B_x
    _, S, M = A_x.shape
    DC = A_c_kv.shape[2]
    H, D = A_w_q.shape[1], A_w_q.shape[2]
    FF = B_w_gate.shape[1]
    hbm = pl.BlockSpec(memory_space=pltpu.HBM)
    out = pl.pallas_call(
        _kernel,
        out_shape=jax.ShapeDtypeStruct((S, M), A_x.dtype),
        in_specs=[hbm] * 6 + [pl.BlockSpec(memory_space=pltpu.VMEM)] + [hbm] * 3,
        out_specs=hbm,
        scratch_shapes=[
            pltpu.VMEM((S // 2, M), U32),
            pltpu.VMEM((S // 2, DC), U32),
            pltpu.VMEM((H // 2, M + 2 * DC, D), U32),
            pltpu.VMEM((H * D // 2, M), U32),
            pltpu.VMEM((FF // 2, M), U32),
            pltpu.VMEM((FF // 2, M), U32),
            pltpu.VMEM((FF // 2, M), U32),
            pltpu.VMEM((S // 2, M), U32),
            pltpu.VMEM((2, S // 2, D), U32),
            pltpu.VMEM((2, S // 2, D), U32),
            pltpu.VMEM((2, S // 2, D), U32),
            pltpu.VMEM((2, (M + 2 * DC) // 2, D), U32),
            pltpu.VMEM((H, S // 2, D), U32),
            pltpu.VMEM((S, M), F32),
            pltpu.VMEM((S, M), BF16),
            pltpu.SemaphoreType.DMA((2 * len(XA),)),
            pltpu.SemaphoreType.DMA((3 * H // 2,)),
            pltpu.SemaphoreType.DMA((4,)),
            pltpu.SemaphoreType.DMA(()),
        ],
        compiler_params=pltpu.CompilerParams(vmem_limit_bytes=100 * 1024 * 1024),
    )(
        A_x.reshape(S, M),
        A_c_kv.reshape(S, DC),
        A_w_q,
        A_w_uk,
        A_w_uv,
        A_w_o.reshape(H * D, M),
        B_w_r,
        B_w_gate.T,
        B_w_up.T,
        B_w_down,
    )
    return out.reshape(1, S, M)
```

```python
import math

import numpy as np
import jax
import jax.numpy as jnp
from jax import lax
import jax.experimental.pallas as pl
import jax.experimental.pallas.tpu as pltpu

BF16 = jnp.bfloat16
F32 = jnp.float32
U32 = jnp.uint32
TOPC = 8
LN_EPS = float(np.float32(np.asarray(1e-5, dtype=jnp.bfloat16)))
NEG = -1e30
KEY0 = 0x10000000
T = 128
CK = 4

LAG = (10,8)
BIAS = (-1, 0)
GATE = (3,2)
GATE_ROW = (64,120)
Q_FIRST = (0, 1)
HOLD = (5,3,2)
CHUNKS = (0, 1, 3, 6, 10, 16)
AHEAD = 3
ANCHOR = 4
FFN_BLOCKS = 2
FLAT_BLOCKS = 4
OUT_ROWS = 256
OUT_UNROLL = 2

_reciprocal = getattr(pltpu, "reciprocal", None) or pl.reciprocal


def _rb(v):
    return v.astype(BF16).astype(F32)


def _dot(a, b):
    return jnp.dot(a, b, preferred_element_type=F32)


def _dot_nt(a, b):
    return lax.dot_general(a, b, (((1,), (1,)), ((), ())), preferred_element_type=F32)


def _recip(v):
    inv = _reciprocal(v, approx=True)
    return inv * (2.0 - v * inv)


def _ld(ref, r0, n, *lead):
    return pltpu.bitcast(ref[(*lead, pl.ds(r0 // 2, n // 2), slice(None))], BF16)


def _st(ref, r0, val, *lead):
    n = val.shape[0]
    ref[(*lead, pl.ds(r0 // 2, n // 2), slice(None))] = pltpu.bitcast(val.astype(BF16), U32)


def _tree(op, xs):
    while len(xs) > 1:
        xs = [op(xs[i], xs[i + 1]) if i + 1 < len(xs) else xs[i] for i in range(0, len(xs), 2)]
    return xs[0]


def _tiles(v):
    return [v[:, j * T:(j + 1) * T] for j in range(v.shape[1] // T)]


def _rowsum(v):
    return jnp.sum(_tree(jnp.add, _tiles(v)), axis=-1, keepdims=True)


def _merge(*lists):
    keyed = []
    for k, items in enumerate(lists):
        keyed += [((j + 0.5) / len(items), k, j) for j in range(len(items))]
    return [lists[k][j] for _, k, j in sorted(keyed)]


def _kernel(x_hbm, c_hbm, wq_hbm, wuk_hbm, wuv_hbm, wo_hbm, wr_ref, wg_hbm, wu_hbm, wd_hbm,
            out_hbm,
            x_v, c_v, wp_v, wo_v, wg_v, wu_v, wd_v,
            xn_v, q_v, k_v, v_v, wh_v, ctx_v, acc_v, o_v, xsems, wsems, lsems, osem):
    S, M, DC, FF = 2 * x_v.shape[0], x_v.shape[1], c_v.shape[1], 2 * wd_v.shape[0]
    H, D = ctx_v.shape[0], ctx_v.shape[2]
    NB, NPAIR, MT, CT = S // T, H // 2, M // T, DC // T

    def in_copies(j):
        rows = pl.ds(CHUNKS[j] * T // 2, (CHUNKS[j + 1] - CHUNKS[j]) * T // 2)
        return [pltpu.make_async_copy(src.bitcast(U32).at[rows], dst.at[rows], xsems.at[2 * j + i])
                for i, (src, dst) in enumerate(((c_hbm, c_v), (x_hbm, x_v)))]

    def pair_copies(g):
        return [pltpu.make_async_copy(src.bitcast(U32).at[:, g, :],
                                      wp_v.at[g, pl.ds(r0, n)], wsems.at[3 * g + i])
                for i, (src, r0, n) in enumerate(
                    ((wuk_hbm, M, DC), (wuv_hbm, M + DC, DC), (wq_hbm, 0, M)))]

    late = [pltpu.make_async_copy(s.bitcast(U32), d, lsems.at[i]) for i, (s, d) in enumerate(
        ((wg_hbm, wg_v), (wu_hbm, wu_v), (wd_hbm, wd_v), (wo_hbm, wo_v)))]

    def start(cps, priority=0):
        for cp in cps:
            cp.start(priority=priority)

    def wait(cps):
        for cp in cps:
            cp.wait()

    first_w = pair_copies(0)
    start(first_w + in_copies(0))
    for j in range(1, len(CHUNKS) - 1):
        start(in_copies(j), priority=1)
    for g in range(1, NPAIR):
        start(pair_copies(g), priority=1)

    lane = lax.broadcasted_iota(jnp.int32, (8, T), 1)
    sub = lax.broadcasted_iota(jnp.int32, (8, T), 0)
    qscale = (D ** -0.5) * math.log2(math.e)

    zero = jnp.min(lane)

    def after(tok, v):
        return jnp.where(zero > 0, tok, v)

    queue = []
    pending = []
    clock = [0]
    every = [0]

    def operand(ref, r0, n, *lead):
        w32 = ref[(*lead, pl.ds(r0 // 2, n // 2), slice(None))]
        clock[0] += 1
        due = [tok for t, tok in pending if t < clock[0]]
        pending[:] = [e for e in pending if e[0] >= clock[0]]
        if due:
            top = w32[0:8, 0:T]
            for tok in due:
                top = after(pltpu.bitcast(tok, U32), top)
            if w32.shape[1] > T:
                top = jnp.concatenate([top, w32[0:8, T:]], axis=1)
            w32 = jnp.concatenate([top, w32[8:]], axis=0)
        if queue and every[0] and clock[0] % every[0] == 0:
            queue.pop(0)()
        return pltpu.bitcast(w32, BF16)

    def anchor(tok):
        pending.append((clock[0] + ANCHOR, tok))

    def flush():
        while queue:
            queue.pop(0)()

    def layernorm(i):
        xf = _ld(x_v, i * T, T).astype(F32)
        mean = _rowsum(xf) * (1.0 / M)
        mean_b = _rb(mean)
        cen = xf - mean_b
        off = mean - mean_b
        var = jnp.maximum(_rowsum(cen * cen) * (1.0 / M) - off * off, 0.0)
        _st(xn_v, i * T, _rb(cen) * _recip(_rb(jnp.sqrt(_rb(_rb(var) + LN_EPS)))))

    def unpack_weights(g, buf, t):
        even = wp_v[g, pl.ds(t * T, T // 2, stride=2), :]
        odd = wp_v[g, pl.ds(t * T + 1, T // 2, stride=2), :]
        if buf:
            w = (even >> 16) | (odd & U32(0xFFFF0000))
        else:
            w = (even & U32(0xFFFF)) | (odd << 16)
        wh_v[buf, pl.ds(t * T // 2, T // 2), :] = w

    def unpacking(g, buf):
        return [(0, lambda t=t: unpack_weights(g, buf, t)) for t in range(MT + 2 * CT)]

    def project_q(i, buf):
        _st(q_v, i * T, _dot(operand(xn_v, i * T, T), _ld(wh_v, 0, M, buf)) * qscale, buf)

    def project_k(i, buf):
        _st(k_v, i * T, _dot(operand(c_v, i * T, T), _ld(wh_v, M, DC, buf)), buf)

    def project_v(i, buf, behind=None):
        c = operand(c_v, i * T, T)
        if behind is not None:
            c = pltpu.bitcast(c, U32)
            tok = jnp.concatenate([pltpu.bitcast(behind[T - 8:T], U32)] * CT, axis=1)
            c = pltpu.bitcast(jnp.concatenate([after(tok, c[0:8]), c[8:]], axis=0), BF16)
        _st(v_v, i * T, _dot(c, _ld(wh_v, M + DC, DC, buf)), buf)

    def projections(buf):
        qs = [(MT, lambda i=i: project_q(i, buf)) for i in range(NB)]
        ks = [(CT, lambda i=i: project_k(i, buf)) for i in range(NB)]
        vs = [(CT, lambda i=i, **kw: project_v(i, buf, **kw)) for i in range(NB)]
        return (qs + ks if Q_FIRST[buf] else ks + qs) + vs

    def scores(i, t, n, buf, st):
        tiles = _tiles(_dot_nt(operand(q_v, i * T, T, buf), _ld(k_v, t * T, n * T, buf)))
        if t + n == i + 1:
            row = lax.broadcasted_iota(jnp.int32, (T, T), 0)
            col = lax.broadcasted_iota(jnp.int32, (T, T), 1)
            tiles[-1] = jnp.where(col <= row, tiles[-1], NEG)
        st[t] = jnp.concatenate(tiles, axis=1) if n > 1 else tiles[0]
        st["m"] = _tree(jnp.maximum, tiles + ([st["m"]] if t else []))
        if t + n == i + 1:
            st["m"] = jnp.max(st["m"], axis=-1, keepdims=True)

    last_ctx = []

    def context(i, t, n, h, buf, st):
        if GATE[buf] and t // CK == GATE[buf]:
            tok = st["pv"][0][GATE_ROW[buf]:GATE_ROW[buf] + 8]
            st["m"] = after(jnp.concatenate([tok] * (T // 8), axis=0), st["m"])
        m = st["m"]
        if m.shape[1] == T and n > 1:
            m = jnp.concatenate([m] * n, axis=1)
        d = st[t] - m
        if t == 0 and last_ctx:
            d0 = after(last_ctx.pop(), d[:, 0:T])
            d = jnp.concatenate([d0, d[:, T:]], axis=1) if n > 1 else d0
        p = jnp.exp2(d)
        l = _tree(jnp.add, _tiles(p))
        o = _dot(p.astype(BF16), operand(v_v, t * T, n * T, buf))
        st.setdefault("pv", []).append(o)
        if t:
            l, o = st["l"] + l, st["o"] + o
        st["l"], st["o"] = l, o
        if t + n == i + 1:
            o = o * _recip(jnp.sum(l, axis=-1, keepdims=True))
            last_ctx.append(o)
            _st(ctx_v, i * T, o, h)

    def head(h, buf, fillers, hold=False, before=None):
        work = [(i, t, min(CK, i + 1 - t)) for i in range(NB) for t in range(0, i + 1, CK)]
        state = [{} for _ in range(NB)]
        held = []
        if hold:
            cut = len(fillers) - HOLD[0] - HOLD[1]
            fillers, held = fillers[:cut], fillers[cut:]
        att_total = 2 * sum(n for _, _, n in work)
        fill_total = sum(c for c, _ in fillers)
        a = b = f = att = fill = 0
        ready = {}
        scored = False
        while b < len(work) or f < len(fillers):
            b_ok = b < len(work) and ready.get(work[b][0], math.inf) <= att + fill
            if f < len(fillers) and ((fill - BIAS[buf]) * att_total < att * fill_total
                                     or (a == len(work) and not b_ok)):
                fillers[f][1]()
                fill += fillers[f][0]
                f += 1
            elif a < len(work) and not (b_ok and scored):
                i, t, n = work[a]
                if before is not None and t == 0:
                    fill += before(i)
                scores(i, t, n, buf, state[i])
                a, att, scored = a + 1, att + n, True
                if t + n == i + 1:
                    ready[i] = att + fill + LAG[buf]
                if a == len(work):
                    for _, fn in held[:HOLD[0]]:
                        fn(behind=state[i][t - CK][:, 0:T])
            else:
                i, t, n = work[b]
                context(i, t, n, h, buf, state[i])
                b, att, scored = b + 1, att + n, False
        for _, fn in held[HOLD[0]:]:
            fn(behind=state[-1]["pv"][-HOLD[2]])

    def first_weights(t0, n):
        for t in range(t0, t0 + n):
            unpack_weights(0, 0, t)
            unpack_weights(0, 1, t)

    def prepare(i):
        cost = 0
        if i in CHUNKS[:-1]:
            wait(in_copies(CHUNKS.index(i)))
        if i == 0:
            wait(first_w[:1])
            first_weights(MT, CT)
        if i == 1:
            wait(first_w[1:])
        if i < NB:
            project_k(i, 0)
            project_k(i, 1)
            cost += 2 * CT
        if i == 1:
            first_weights(MT + CT, CT)
            first_weights(0, MT)
        if 1 <= i <= NB:
            project_v(i - 1, 0)
            layernorm(i - 1)
            project_q(i - 1, 0)
            project_q(i - 1, 1)
            cost += CT + 2 * MT
        if i >= NB:
            for j in range((i - NB) * NB // AHEAD, (i - NB + 1) * NB // AHEAD):
                project_v(j, 1)
                cost += CT
        return cost

    for i in range(AHEAD):
        prepare(i)
    head(0, 0, [], before=lambda i: prepare(i + AHEAD))
    wait(pair_copies(1))
    start(late)
    for _, fn in unpacking(1, 0):
        fn()

    def pair_body(g, carry):
        last_ctx.clear()

        @pl.when(g + 1 < NPAIR)
        def _():
            wait(pair_copies(g + 1))

        head(2 * g - 1, 1, _merge(projections(0), unpacking(g, 1)))
        head(2 * g, 0, unpacking(jnp.minimum(g + 1, NPAIR - 1), 0) + projections(1), hold=True)
        return carry

    lax.fori_loop(1, NPAIR, pair_body, 0)
    last_ctx.clear()
    wait(late[3:])

    wr = wr_ref[...].astype(F32).reshape(1, M)
    routed = [jnp.zeros((8, T), F32) for _ in range(S // (8 * T))]
    keys, sel, sel_rows, ffn = [], [], [], {}

    def router(i):
        r = _rowsum(_ld(xn_v, i * T, T).astype(F32) * wr)
        for g in range(T // 8):
            k, ln = divmod(i * T // 8 + g, T)
            routed[k] = jnp.where(lane == ln, r[g * 8:(g + 1) * 8, :], routed[k])
        anchor(routed[k])

    def select_step():
        if not keys:
            for k, r in enumerate(routed):
                bits = pltpu.bitcast(_rb(r), jnp.int32) >> 16
                mag = bits & 0x7FFF
                rank = jnp.where(bits < 0, 0x8000 - mag, 0x8000 + mag)
                rank = jnp.where(mag > 0x7F80, 0, rank)
                row = k * 8 * T + lane * 8 + sub
                keys.append(pltpu.bitcast(rank * S + (S - 1 - row) + KEY0, F32))
        top = jnp.max(jnp.max(_tree(jnp.maximum, keys), axis=0, keepdims=True), axis=1, keepdims=True)
        top = jnp.broadcast_to(top, (8, T))
        sel.append(pltpu.bitcast(top, jnp.int32) - KEY0)
        keys[:] = [jnp.where(kk == top, 0.0, kk) for kk in keys]
        anchor(top)

    def gather():
        slot = lax.broadcasted_iota(jnp.int32, (TOPC, M), 0)
        xs = jnp.zeros((TOPC, M), F32)
        key = jnp.zeros((TOPC, T), jnp.int32)
        for j, top in enumerate(sel):
            row = S - 1 - (top[0, 0] & (S - 1))
            sel_rows.append(row)
            w32 = xn_v[pl.ds(row >> 1, 1), :] << (16 - 16 * (row & 1)).astype(U32)
            xs = jnp.where(slot == j, pltpu.bitcast(w32 & U32(0xFFFF0000), F32), xs)
            key = jnp.where(sub == j, top, key)
        rank = key >> (S.bit_length() - 1)
        bits = jnp.where(rank >= 0x8000, rank - 0x8000, (0x8000 - rank) | 0x8000)
        bits = jnp.where(rank == 0, 0x7FC0, bits)
        ffn["gain"] = jax.nn.sigmoid(pltpu.bitcast(bits << 16, F32))
        ffn["x"] = xs.astype(BF16)

    FG = 4 * T

    def ffn_in(name, w_v, f0, k):
        w = pltpu.bitcast(w_v[f0 // 2:min(f0 + FG, FF) // 2, k * T:(k + 1) * T], BF16)
        part = _dot_nt(ffn["x"][:, k * T:(k + 1) * T], w)
        ffn[name, f0] = ffn[name, f0] + part if k else part

    def ffn_down(f0, n0, n1):
        if n0 == 0:
            g, u = ffn["g", f0], ffn["u", f0]
            ffn["h", f0] = (g * jax.nn.sigmoid(g) * u).astype(BF16)
        w = pltpu.bitcast(wd_v[f0 // 2:min(f0 + FG, FF) // 2, n0 * T:n1 * T], BF16)
        for n, part in zip(range(n0, n1), _tiles(_dot(ffn["h", f0], w))):
            ffn["y", n] = ffn["y", n] + part if f0 else part

    ffn_steps = []
    for f0 in range(0, FF, FG):
        for k in range(MT):
            gate = lambda f0=f0, k=k: ffn_in("g", wg_v, f0, k)
            up = lambda f0=f0, k=k: ffn_in("u", wu_v, f0, k)
            ffn_steps += [gate, up] if f0 + FG <= FF else [lambda gate=gate, up=up: (gate(), up())]
    for f0 in range(0, FF, FG):
        step = 1 if f0 + FG <= FF else 2
        for n in range(0, MT, step):
            ffn_steps.append(lambda f0=f0, n=n, step=step: ffn_down(f0, n, min(n + step, MT)))

    def residual(r0, n):
        acc_v[r0:r0 + n, :] = _ld(x_v, r0, n).astype(F32) + _ld(xn_v, r0, n).astype(F32)
        anchor(acc_v[pl.ds(pl.multiple_of(zero * 8, 8), 8), 0:T])

    def out_project(rp, n, h0, h1):
        ctx = jnp.concatenate(
            [pltpu.bitcast(ctx_v[h, pl.ds(rp, n // 2), :], BF16) for h in range(h0, h1)], axis=1)
        return _dot(ctx, operand(wo_v, h0 * D, (h1 - h0) * D))

    attn = {}

    def out_step(i, h):
        part = out_project(i * T // 2, T, h, h + 1)
        attn[i] = attn[i] + part if h else part

    def finish(rp, val):
        rows = pl.ds(2 * rp, val.shape[0])
        o_v[rows, :] = (acc_v[rows, :] + val).astype(BF16)
        pltpu.make_async_copy(o_v.at[rows], out_hbm.at[rows], osem).start()

    queue.extend([lambda i=i: router(i) for i in range(NB)] + [select_step] * TOPC + [gather])
    every[0] = 4
    head(H - 1, 1, [(MT, lambda h=h: out_step(0, h)) for h in range(H - 1)])
    flush()
    wait(late[:3])
    out_step(0, H - 1)
    queue.extend([lambda r0=r0: residual(r0, 32) for r0 in range(0, S, 32)])
    every[0] = 1
    for fn in _merge([lambda i=i, h=h: out_step(i, h)
                      for i in range(1, FFN_BLOCKS + 1) for h in range(H)],
                     ffn_steps + [lambda: None] * 10):
        fn()
    flush()
    pending.clear()
    y = jnp.concatenate([ffn["y", n] * ffn["gain"] for n in range(MT)], axis=1)
    olds = [acc_v[pl.ds(row, 1), :] for row in sel_rows]
    for j, row in enumerate(sel_rows):
        acc_v[pl.ds(row, 1), :] = olds[j] + y[j:j + 1, :]

    for i in range(FFN_BLOCKS + 1, FLAT_BLOCKS):
        for h in range(H):
            out_step(i, h)
            if h % 8 == 3 and len(attn) > 1:
                j = min(attn)
                finish(j * T // 2, attn.pop(j))
    for j in sorted(attn):
        finish(j * T // 2, attn[j])

    def out_body(b, carry):
        for u in range(OUT_UNROLL):
            r0 = FLAT_BLOCKS * T + (b * OUT_UNROLL + u) * OUT_ROWS
            rp = pl.multiple_of(r0 // 2, T // 2)
            finish(rp, out_project(rp, OUT_ROWS, 0, H))
        return carry

    assert (S - FLAT_BLOCKS * T) % (OUT_UNROLL * OUT_ROWS) == 0
    lax.fori_loop(0, (S - FLAT_BLOCKS * T) // (OUT_UNROLL * OUT_ROWS), out_body, 0)
    pltpu.make_async_copy(o_v, out_hbm, osem).wait()


@jax.jit
def pallas_parallel_sum__compressed_kv_cla__moe_arch_mod__prompt_kernel(
    A_x: jax.Array,
    A_c_kv: jax.Array,
    A_w_q: jax.Array,
    A_w_uk: jax.Array,
    A_w_uv: jax.Array,
    A_w_o: jax.Array,
    B_x: jax.Array,
    B_w_r: jax.Array,
    B_w_gate: jax.Array,
    B_w_up: jax.Array,
    B_w_down: jax.Array,
):
    del B_x
    _, S, M = A_x.shape
    DC = A_c_kv.shape[2]
    H, D = A_w_q.shape[1], A_w_q.shape[2]
    FF = B_w_gate.shape[1]
    hbm = pl.BlockSpec(memory_space=pltpu.HBM)
    out = pl.pallas_call(
        _kernel,
        out_shape=jax.ShapeDtypeStruct((S, M), A_x.dtype),
        in_specs=[hbm] * 6 + [pl.BlockSpec(memory_space=pltpu.VMEM)] + [hbm] * 3,
        out_specs=hbm,
        scratch_shapes=[
            pltpu.VMEM((S // 2, M), U32),
            pltpu.VMEM((S // 2, DC), U32),
            pltpu.VMEM((H // 2, M + 2 * DC, D), U32),
            pltpu.VMEM((H * D // 2, M), U32),
            pltpu.VMEM((FF // 2, M), U32),
            pltpu.VMEM((FF // 2, M), U32),
            pltpu.VMEM((FF // 2, M), U32),
            pltpu.VMEM((S // 2, M), U32),
            pltpu.VMEM((2, S // 2, D), U32),
            pltpu.VMEM((2, S // 2, D), U32),
            pltpu.VMEM((2, S // 2, D), U32),
            pltpu.VMEM((2, (M + 2 * DC) // 2, D), U32),
            pltpu.VMEM((H, S // 2, D), U32),
            pltpu.VMEM((S, M), F32),
            pltpu.VMEM((S, M), BF16),
            pltpu.SemaphoreType.DMA((2 * (len(CHUNKS) - 1),)),
            pltpu.SemaphoreType.DMA((3 * H // 2,)),
            pltpu.SemaphoreType.DMA((4,)),
            pltpu.SemaphoreType.DMA(()),
        ],
        compiler_params=pltpu.CompilerParams(vmem_limit_bytes=100 * 1024 * 1024),
    )(
        A_x.reshape(S, M),
        A_c_kv.reshape(S, DC),
        A_w_q,
        A_w_uk,
        A_w_uv,
        A_w_o.reshape(H * D, M),
        B_w_r,
        B_w_gate.T,
        B_w_up.T,
        B_w_down,
    )
    return out.reshape(1, S, M)
```

```python
import math

import numpy as np
import jax
import jax.numpy as jnp
from jax import lax
import jax.experimental.pallas as pl
import jax.experimental.pallas.tpu as pltpu

BF16 = jnp.bfloat16
F32 = jnp.float32
U32 = jnp.uint32
TOPC = 8
LN_EPS = float(np.float32(np.asarray(1e-5, dtype=jnp.bfloat16)))
NEG = -1e30
KEY0 = 0x10000000
T = 128
CK = 4

LAG = (10,8)
BIAS = (-1,1)
GATE = (3,3)
GATE_ROW = (64,120)
Q_FIRST = (0,1)
HOLD = (5,3,2)
CHUNKS = (0, 1, 3, 6, 10, 16)
AHEAD = 3
ANCHOR = 4
FFN_BLOCKS = 2
FLAT_BLOCKS = 4
OUT_ROWS = 256
OUT_UNROLL = 2

_reciprocal = getattr(pltpu, "reciprocal", None) or pl.reciprocal


def _rb(v):
    return v.astype(BF16).astype(F32)


def _dot(a, b):
    return jnp.dot(a, b, preferred_element_type=F32)


def _dot_nt(a, b):
    return lax.dot_general(a, b, (((1,), (1,)), ((), ())), preferred_element_type=F32)


def _recip(v):
    inv = _reciprocal(v, approx=True)
    return inv * (2.0 - v * inv)


def _ld(ref, r0, n, *lead):
    return pltpu.bitcast(ref[(*lead, pl.ds(r0 // 2, n // 2), slice(None))], BF16)


def _st(ref, r0, val, *lead):
    n = val.shape[0]
    ref[(*lead, pl.ds(r0 // 2, n // 2), slice(None))] = pltpu.bitcast(val.astype(BF16), U32)


def _tree(op, xs):
    while len(xs) > 1:
        xs = [op(xs[i], xs[i + 1]) if i + 1 < len(xs) else xs[i] for i in range(0, len(xs), 2)]
    return xs[0]


def _tiles(v):
    return [v[:, j * T:(j + 1) * T] for j in range(v.shape[1] // T)]


def _rowsum(v):
    return jnp.sum(_tree(jnp.add, _tiles(v)), axis=-1, keepdims=True)


def _merge(*lists):
    keyed = []
    for k, items in enumerate(lists):
        keyed += [((j + 0.5) / len(items), k, j) for j in range(len(items))]
    return [lists[k][j] for _, k, j in sorted(keyed)]


def _kernel(x_hbm, c_hbm, wq_hbm, wuk_hbm, wuv_hbm, wo_hbm, wr_hbm, wg_hbm, wu_hbm, wd_hbm,
            out_hbm,
            x_v, c_v, wp_v, wo_v, wr_v, wg_v, wu_v, wd_v,
            xn_v, q_v, k_v, v_v, wh_v, ctx_v, acc_v, o_v, xsems, wsems, lsems, osem):
    S, M, DC, FF = 2 * x_v.shape[0], x_v.shape[1], c_v.shape[1], 2 * wd_v.shape[0]
    H, D = ctx_v.shape[0], ctx_v.shape[2]
    NB, NPAIR, MT, CT = S // T, H // 2, M // T, DC // T

    def in_copies(j):
        rows = pl.ds(CHUNKS[j] * T // 2, (CHUNKS[j + 1] - CHUNKS[j]) * T // 2)
        return [pltpu.make_async_copy(src.bitcast(U32).at[rows], dst.at[rows], xsems.at[2 * j + i])
                for i, (src, dst) in enumerate(((c_hbm, c_v), (x_hbm, x_v)))]

    def pair_copies(g):
        return [pltpu.make_async_copy(src.bitcast(U32).at[:, g, :],
                                      wp_v.at[g, pl.ds(r0, n)], wsems.at[3 * g + i])
                for i, (src, r0, n) in enumerate(
                    ((wuk_hbm, M, DC), (wuv_hbm, M + DC, DC), (wq_hbm, 0, M)))]

    late = [pltpu.make_async_copy(s.bitcast(U32), d, lsems.at[i]) for i, (s, d) in enumerate(
        ((wg_hbm, wg_v), (wu_hbm, wu_v), (wd_hbm, wd_v), (wo_hbm, wo_v)))]
    late.append(pltpu.make_async_copy(wr_hbm, wr_v, lsems.at[4]))

    def start(cps, priority=0):
        for cp in cps:
            cp.start(priority=priority)

    def wait(cps):
        for cp in cps:
            cp.wait()

    first_w = pair_copies(0)
    start(first_w + in_copies(0))
    for j in range(1, len(CHUNKS) - 1):
        start(in_copies(j), priority=1)
    for g in range(1, NPAIR):
        start(pair_copies(g), priority=1)

    lane = lax.broadcasted_iota(jnp.int32, (8, T), 1)
    sub = lax.broadcasted_iota(jnp.int32, (8, T), 0)
    qscale = (D ** -0.5) * math.log2(math.e)

    zero = jnp.min(lane)

    def after(tok, v):
        return jnp.where(zero > 0, tok, v)

    queue = []
    pending = []
    clock = [0]
    every = [0]

    def operand(ref, r0, n, *lead):
        w32 = ref[(*lead, pl.ds(r0 // 2, n // 2), slice(None))]
        clock[0] += 1
        due = [tok for t, tok in pending if t < clock[0]]
        pending[:] = [e for e in pending if e[0] >= clock[0]]
        if due:
            top = w32[0:8, 0:T]
            for tok in due:
                top = after(pltpu.bitcast(tok, U32), top)
            if w32.shape[1] > T:
                top = jnp.concatenate([top, w32[0:8, T:]], axis=1)
            w32 = jnp.concatenate([top, w32[8:]], axis=0)
        if queue and every[0] and clock[0] % every[0] == 0:
            queue.pop(0)()
        return pltpu.bitcast(w32, BF16)

    def anchor(tok):
        pending.append((clock[0] + ANCHOR, tok))

    def flush():
        while queue:
            queue.pop(0)()

    def layernorm(i):
        xf = _ld(x_v, i * T, T).astype(F32)
        mean = _rowsum(xf) * (1.0 / M)
        mean_b = _rb(mean)
        cen = xf - mean_b
        off = mean - mean_b
        var = jnp.maximum(_rowsum(cen * cen) * (1.0 / M) - off * off, 0.0)
        _st(xn_v, i * T, _rb(cen) * _recip(_rb(jnp.sqrt(_rb(_rb(var) + LN_EPS)))))

    def unpack_weights(g, buf, t):
        even = wp_v[g, pl.ds(t * T, T // 2, stride=2), :]
        odd = wp_v[g, pl.ds(t * T + 1, T // 2, stride=2), :]
        if buf:
            w = (even >> 16) | (odd & U32(0xFFFF0000))
        else:
            w = (even & U32(0xFFFF)) | (odd << 16)
        wh_v[buf, pl.ds(t * T // 2, T // 2), :] = w

    def unpacking(g, buf):
        return [(0, lambda t=t: unpack_weights(g, buf, t)) for t in range(MT + 2 * CT)]

    def project_q(i, buf):
        _st(q_v, i * T, _dot(operand(xn_v, i * T, T), _ld(wh_v, 0, M, buf)) * qscale, buf)

    def project_k(i, buf):
        _st(k_v, i * T, _dot(operand(c_v, i * T, T), _ld(wh_v, M, DC, buf)), buf)

    def project_v(i, buf, behind=None):
        c = operand(c_v, i * T, T)
        if behind is not None:
            c = pltpu.bitcast(c, U32)
            tok = jnp.concatenate([pltpu.bitcast(behind[T - 8:T], U32)] * CT, axis=1)
            c = pltpu.bitcast(jnp.concatenate([after(tok, c[0:8]), c[8:]], axis=0), BF16)
        _st(v_v, i * T, _dot(c, _ld(wh_v, M + DC, DC, buf)), buf)

    def projections(buf):
        qs = [(MT, lambda i=i: project_q(i, buf)) for i in range(NB)]
        ks = [(CT, lambda i=i: project_k(i, buf)) for i in range(NB)]
        vs = [(CT, lambda i=i, **kw: project_v(i, buf, **kw)) for i in range(NB)]
        return (qs + ks if Q_FIRST[buf] else ks + qs) + vs

    def scores(i, t, n, buf, st):
        tiles = _tiles(_dot_nt(operand(q_v, i * T, T, buf), _ld(k_v, t * T, n * T, buf)))
        if t + n == i + 1:
            row = lax.broadcasted_iota(jnp.int32, (T, T), 0)
            col = lax.broadcasted_iota(jnp.int32, (T, T), 1)
            tiles[-1] = jnp.where(col <= row, tiles[-1], NEG)
        st[t] = jnp.concatenate(tiles, axis=1) if n > 1 else tiles[0]
        st["m"] = _tree(jnp.maximum, tiles + ([st["m"]] if t else []))
        if t + n == i + 1:
            st["m"] = jnp.max(st["m"], axis=-1, keepdims=True)

    last_ctx = []

    def context(i, t, n, h, buf, st):
        if GATE[buf] and t // CK == GATE[buf]:
            tok = st["pv"][0][GATE_ROW[buf]:GATE_ROW[buf] + 8]
            st["m"] = after(jnp.concatenate([tok] * (T // 8), axis=0), st["m"])
        m = st["m"]
        if m.shape[1] == T and n > 1:
            m = jnp.concatenate([m] * n, axis=1)
        d = st[t] - m
        if t == 0 and last_ctx:
            d0 = after(last_ctx.pop(), d[:, 0:T])
            d = jnp.concatenate([d0, d[:, T:]], axis=1) if n > 1 else d0
        p = jnp.exp2(d)
        l = _tree(jnp.add, _tiles(p))
        o = _dot(p.astype(BF16), operand(v_v, t * T, n * T, buf))
        st.setdefault("pv", []).append(o)
        if t:
            l, o = st["l"] + l, st["o"] + o
        st["l"], st["o"] = l, o
        if t + n == i + 1:
            o = o * _recip(jnp.sum(l, axis=-1, keepdims=True))
            last_ctx.append(o)
            _st(ctx_v, i * T, o, h)

    def head(h, buf, fillers, hold=False, before=None):
        work = [(i, t, min(CK, i + 1 - t)) for i in range(NB) for t in range(0, i + 1, CK)]
        state = [{} for _ in range(NB)]
        held = []
        if hold:
            cut = len(fillers) - HOLD[0] - HOLD[1]
            fillers, held = fillers[:cut], fillers[cut:]
        att_total = 2 * sum(n for _, _, n in work)
        fill_total = sum(c for c, _ in fillers)
        a = b = f = att = fill = 0
        ready = {}
        scored = False
        while b < len(work) or f < len(fillers):
            b_ok = b < len(work) and ready.get(work[b][0], math.inf) <= att + fill
            if f < len(fillers) and ((fill - BIAS[buf]) * att_total < att * fill_total
                                     or (a == len(work) and not b_ok)):
                fillers[f][1]()
                fill += fillers[f][0]
                f += 1
            elif a < len(work) and not (b_ok and scored):
                i, t, n = work[a]
                if before is not None and t == 0:
                    fill += before(i)
                scores(i, t, n, buf, state[i])
                a, att, scored = a + 1, att + n, True
                if t + n == i + 1:
                    ready[i] = att + fill + LAG[buf]
                if a == len(work):
                    for _, fn in held[:HOLD[0]]:
                        fn(behind=state[i][t - CK][:, 0:T])
            else:
                i, t, n = work[b]
                context(i, t, n, h, buf, state[i])
                b, att, scored = b + 1, att + n, False
        for _, fn in held[HOLD[0]:]:
            fn(behind=state[-1]["pv"][-HOLD[2]])

    def first_weights(t0, n):
        for t in range(t0, t0 + n):
            unpack_weights(0, 0, t)
            unpack_weights(0, 1, t)

    def prepare(i):
        cost = 0
        if i in CHUNKS[:-1]:
            wait(in_copies(CHUNKS.index(i)))
        if i == 0:
            wait(first_w[:1])
            first_weights(MT, CT)
        if i == 1:
            wait(first_w[1:])
        if i < NB:
            project_k(i, 0)
            project_k(i, 1)
            cost += 2 * CT
        if i == 1:
            first_weights(MT + CT, CT)
            first_weights(0, MT)
        if 1 <= i <= NB:
            project_v(i - 1, 0)
            layernorm(i - 1)
            project_q(i - 1, 0)
            project_q(i - 1, 1)
            cost += CT + 2 * MT
        if i >= NB:
            for j in range((i - NB) * NB // AHEAD, (i - NB + 1) * NB // AHEAD):
                project_v(j, 1)
                cost += CT
        return cost

    for i in range(AHEAD):
        prepare(i)
    head(0, 0, [], before=lambda i: prepare(i + AHEAD))
    wait(pair_copies(1))
    start(late)
    for _, fn in unpacking(1, 0):
        fn()

    def pair_body(g, carry):
        last_ctx.clear()

        @pl.when(g + 1 < NPAIR)
        def _():
            wait(pair_copies(g + 1))

        head(2 * g - 1, 1, _merge(projections(0), unpacking(g, 1)))
        head(2 * g, 0, unpacking(jnp.minimum(g + 1, NPAIR - 1), 0) + projections(1), hold=True)
        return carry

    lax.fori_loop(1, NPAIR, pair_body, 0)
    last_ctx.clear()
    wait(late[3:])

    wr = wr_v[...].astype(F32).reshape(1, M)
    routed = [jnp.zeros((8, T), F32) for _ in range(S // (8 * T))]
    keys, sel, sel_rows, ffn = [], [], [], {}

    def router(i):
        r = _rowsum(_ld(xn_v, i * T, T).astype(F32) * wr)
        for g in range(T // 8):
            k, ln = divmod(i * T // 8 + g, T)
            routed[k] = jnp.where(lane == ln, r[g * 8:(g + 1) * 8, :], routed[k])
        anchor(routed[k])

    def select_step():
        if not keys:
            for k, r in enumerate(routed):
                bits = pltpu.bitcast(_rb(r), jnp.int32) >> 16
                mag = bits & 0x7FFF
                rank = jnp.where(bits < 0, 0x8000 - mag, 0x8000 + mag)
                rank = jnp.where(mag > 0x7F80, 0, rank)
                row = k * 8 * T + lane * 8 + sub
                keys.append(pltpu.bitcast(rank * S + (S - 1 - row) + KEY0, F32))
        top = jnp.max(jnp.max(_tree(jnp.maximum, keys), axis=0, keepdims=True), axis=1, keepdims=True)
        top = jnp.broadcast_to(top, (8, T))
        sel.append(pltpu.bitcast(top, jnp.int32) - KEY0)
        keys[:] = [jnp.where(kk == top, 0.0, kk) for kk in keys]
        anchor(top)

    def gather():
        slot = lax.broadcasted_iota(jnp.int32, (TOPC, M), 0)
        xs = jnp.zeros((TOPC, M), F32)
        key = jnp.zeros((TOPC, T), jnp.int32)
        for j, top in enumerate(sel):
            row = S - 1 - (top[0, 0] & (S - 1))
            sel_rows.append(row)
            w32 = xn_v[pl.ds(row >> 1, 1), :] << (16 - 16 * (row & 1)).astype(U32)
            xs = jnp.where(slot == j, pltpu.bitcast(w32 & U32(0xFFFF0000), F32), xs)
            key = jnp.where(sub == j, top, key)
        rank = key >> (S.bit_length() - 1)
        bits = jnp.where(rank >= 0x8000, rank - 0x8000, (0x8000 - rank) | 0x8000)
        bits = jnp.where(rank == 0, 0x7FC0, bits)
        ffn["gain"] = jax.nn.sigmoid(pltpu.bitcast(bits << 16, F32))
        ffn["x"] = xs.astype(BF16)

    FG = 4 * T

    def ffn_in(name, w_v, f0, k):
        w = pltpu.bitcast(w_v[f0 // 2:min(f0 + FG, FF) // 2, k * T:(k + 1) * T], BF16)
        part = _dot_nt(ffn["x"][:, k * T:(k + 1) * T], w)
        ffn[name, f0] = ffn[name, f0] + part if k else part

    def ffn_down(f0, n0, n1):
        if n0 == 0:
            g, u = ffn["g", f0], ffn["u", f0]
            ffn["h", f0] = (g * jax.nn.sigmoid(g) * u).astype(BF16)
        w = pltpu.bitcast(wd_v[f0 // 2:min(f0 + FG, FF) // 2, n0 * T:n1 * T], BF16)
        for n, part in zip(range(n0, n1), _tiles(_dot(ffn["h", f0], w))):
            ffn["y", n] = ffn["y", n] + part if f0 else part

    ffn_steps = []
    for f0 in range(0, FF, FG):
        for k in range(MT):
            gate = lambda f0=f0, k=k: ffn_in("g", wg_v, f0, k)
            up = lambda f0=f0, k=k: ffn_in("u", wu_v, f0, k)
            ffn_steps += [gate, up] if f0 + FG <= FF else [lambda gate=gate, up=up: (gate(), up())]
    for f0 in range(0, FF, FG):
        step = 1 if f0 + FG <= FF else 2
        for n in range(0, MT, step):
            ffn_steps.append(lambda f0=f0, n=n, step=step: ffn_down(f0, n, min(n + step, MT)))

    def residual(r0, n):
        acc_v[r0:r0 + n, :] = _ld(x_v, r0, n).astype(F32) + _ld(xn_v, r0, n).astype(F32)
        anchor(acc_v[pl.ds(pl.multiple_of(zero * 8, 8), 8), 0:T])

    def out_project(rp, n, h0, h1):
        ctx = jnp.concatenate(
            [pltpu.bitcast(ctx_v[h, pl.ds(rp, n // 2), :], BF16) for h in range(h0, h1)], axis=1)
        return _dot(ctx, operand(wo_v, h0 * D, (h1 - h0) * D))

    attn = {}

    def out_step(i, h):
        part = out_project(i * T // 2, T, h, h + 1)
        attn[i] = attn[i] + part if h else part

    def finish(rp, val):
        rows = pl.ds(2 * rp, val.shape[0])
        o_v[rows, :] = (acc_v[rows, :] + val).astype(BF16)
        pltpu.make_async_copy(o_v.at[rows], out_hbm.at[rows], osem).start()

    queue.extend([lambda i=i: router(i) for i in range(NB)] + [select_step] * TOPC + [gather])
    every[0] = 4
    head(H - 1, 1, [(MT, lambda h=h: out_step(0, h)) for h in range(H - 1)])
    flush()
    wait(late[:3])
    out_step(0, H - 1)
    queue.extend([lambda r0=r0: residual(r0, 32) for r0 in range(0, S, 32)])
    every[0] = 1
    for fn in _merge([lambda i=i, h=h: out_step(i, h)
                      for i in range(1, FFN_BLOCKS + 1) for h in range(H)],
                     ffn_steps + [lambda: None] * 10):
        fn()
    flush()
    pending.clear()
    y = jnp.concatenate([ffn["y", n] * ffn["gain"] for n in range(MT)], axis=1)
    olds = [acc_v[pl.ds(row, 1), :] for row in sel_rows]
    for j, row in enumerate(sel_rows):
        acc_v[pl.ds(row, 1), :] = olds[j] + y[j:j + 1, :]

    for i in range(FFN_BLOCKS + 1, FLAT_BLOCKS):
        for h in range(H):
            out_step(i, h)
            if h % 8 == 3 and len(attn) > 1:
                j = min(attn)
                finish(j * T // 2, attn.pop(j))
    for j in sorted(attn):
        finish(j * T // 2, attn[j])

    def out_body(b, carry):
        for u in range(OUT_UNROLL):
            r0 = FLAT_BLOCKS * T + (b * OUT_UNROLL + u) * OUT_ROWS
            rp = pl.multiple_of(r0 // 2, T // 2)
            finish(rp, out_project(rp, OUT_ROWS, 0, H))
        return carry

    assert (S - FLAT_BLOCKS * T) % (OUT_UNROLL * OUT_ROWS) == 0
    lax.fori_loop(0, (S - FLAT_BLOCKS * T) // (OUT_UNROLL * OUT_ROWS), out_body, 0)
    pltpu.make_async_copy(o_v, out_hbm, osem).wait()


@jax.jit
def pallas_parallel_sum__compressed_kv_cla__moe_arch_mod__prompt_kernel(
    A_x: jax.Array,
    A_c_kv: jax.Array,
    A_w_q: jax.Array,
    A_w_uk: jax.Array,
    A_w_uv: jax.Array,
    A_w_o: jax.Array,
    B_x: jax.Array,
    B_w_r: jax.Array,
    B_w_gate: jax.Array,
    B_w_up: jax.Array,
    B_w_down: jax.Array,
):
    del B_x
    _, S, M = A_x.shape
    DC = A_c_kv.shape[2]
    H, D = A_w_q.shape[1], A_w_q.shape[2]
    FF = B_w_gate.shape[1]
    hbm = pl.BlockSpec(memory_space=pltpu.HBM)
    out = pl.pallas_call(
        _kernel,
        out_shape=jax.ShapeDtypeStruct((S, M), A_x.dtype),
        in_specs=[hbm] * 10,
        out_specs=hbm,
        scratch_shapes=[
            pltpu.VMEM((S // 2, M), U32),
            pltpu.VMEM((S // 2, DC), U32),
            pltpu.VMEM((H // 2, M + 2 * DC, D), U32),
            pltpu.VMEM((H * D // 2, M), U32),
            pltpu.VMEM((M,), BF16),
            pltpu.VMEM((FF // 2, M), U32),
            pltpu.VMEM((FF // 2, M), U32),
            pltpu.VMEM((FF // 2, M), U32),
            pltpu.VMEM((S // 2, M), U32),
            pltpu.VMEM((2, S // 2, D), U32),
            pltpu.VMEM((2, S // 2, D), U32),
            pltpu.VMEM((2, S // 2, D), U32),
            pltpu.VMEM((2, (M + 2 * DC) // 2, D), U32),
            pltpu.VMEM((H, S // 2, D), U32),
            pltpu.VMEM((S, M), F32),
            pltpu.VMEM((S, M), BF16),
            pltpu.SemaphoreType.DMA((2 * (len(CHUNKS) - 1),)),
            pltpu.SemaphoreType.DMA((3 * H // 2,)),
            pltpu.SemaphoreType.DMA((5,)),
            pltpu.SemaphoreType.DMA(()),
        ],
        compiler_params=pltpu.CompilerParams(vmem_limit_bytes=100 * 1024 * 1024),
    )(
        A_x.reshape(S, M),
        A_c_kv.reshape(S, DC),
        A_w_q,
        A_w_uk,
        A_w_uv,
        A_w_o.reshape(H * D, M),
        B_w_r,
        B_w_gate.T,
        B_w_up.T,
        B_w_down,
    )
    return out.reshape(1, S, M)
```

```python
import math

import numpy as np
import jax
import jax.numpy as jnp
from jax import lax
import jax.experimental.pallas as pl
import jax.experimental.pallas.tpu as pltpu

BF16 = jnp.bfloat16
F32 = jnp.float32
U32 = jnp.uint32
TOPC = 8
LN_EPS = float(np.float32(np.asarray(1e-5, dtype=jnp.bfloat16)))
NEG = -1e30
KEY0 = 0x10000000
T = 128
CK = 4

LAG = (10, 8)
BIAS = (-1, 1)
GATE = (3, 3)
GATE_ROW = (64, 120)
Q_FIRST = (0, 1)
HOLD = (5, 3, 2)
CHUNKS = (0, 1, 3, 6, 10, 16)
AHEAD = 3
ANCHOR = 4
FFN_BLOCKS = 2
FLAT_BLOCKS = 4
OUT_ROWS = 256
OUT_UNROLL = 2

_reciprocal = getattr(pltpu, "reciprocal", None) or pl.reciprocal


def _rb(v):
    return v.astype(BF16).astype(F32)


def _dot(a, b):
    return jnp.dot(a, b, preferred_element_type=F32)


def _dot_nt(a, b):
    return lax.dot_general(a, b, (((1,), (1,)), ((), ())), preferred_element_type=F32)


def _recip(v):
    inv = _reciprocal(v, approx=True)
    return inv * (2.0 - v * inv)


def _ld(ref, r0, n, *lead):
    return pltpu.bitcast(ref[(*lead, pl.ds(r0 // 2, n // 2), slice(None))], BF16)


def _st(ref, r0, val, *lead):
    n = val.shape[0]
    ref[(*lead, pl.ds(r0 // 2, n // 2), slice(None))] = pltpu.bitcast(val.astype(BF16), U32)


def _tree(op, xs):
    while len(xs) > 1:
        xs = [op(xs[i], xs[i + 1]) if i + 1 < len(xs) else xs[i] for i in range(0, len(xs), 2)]
    return xs[0]


def _tiles(v):
    return [v[:, j * T:(j + 1) * T] for j in range(v.shape[1] // T)]


def _rowsum(v):
    return jnp.sum(_tree(jnp.add, _tiles(v)), axis=-1, keepdims=True)


def _merge(*lists):
    keyed = []
    for k, items in enumerate(lists):
        keyed += [((j + 0.5) / len(items), k, j) for j in range(len(items))]
    return [lists[k][j] for _, k, j in sorted(keyed)]


def _kernel(x_hbm, c_hbm, wq_hbm, wuk_hbm, wuv_hbm, wo_hbm, wr_hbm, wg_hbm, wu_hbm, wd_hbm,
            out_hbm,
            x_v, c_v, wp_v, wo_v, wr_v, wg_v, wu_v, wd_v,
            xn_v, q_v, k_v, v_v, wh_v, ctx_v, acc_v, o_v, xsems, wsems, lsems, osem):
    S, M, DC, FF = 2 * x_v.shape[0], x_v.shape[1], c_v.shape[1], 2 * wd_v.shape[0]
    H, D = ctx_v.shape[0], ctx_v.shape[2]
    NB, NPAIR, MT, CT = S // T, H // 2, M // T, DC // T

    def in_copies(j):
        rows = pl.ds(CHUNKS[j] * T // 2, (CHUNKS[j + 1] - CHUNKS[j]) * T // 2)
        return [pltpu.make_async_copy(src.bitcast(U32).at[rows], dst.at[rows], xsems.at[2 * j + i])
                for i, (src, dst) in enumerate(((c_hbm, c_v), (x_hbm, x_v)))]

    def pair_copies(g):
        return [pltpu.make_async_copy(src.bitcast(U32).at[:, g, :],
                                      wp_v.at[g, pl.ds(r0, n)], wsems.at[3 * g + i])
                for i, (src, r0, n) in enumerate(
                    ((wuk_hbm, M, DC), (wuv_hbm, M + DC, DC), (wq_hbm, 0, M)))]

    late = [pltpu.make_async_copy(s.bitcast(U32), d, lsems.at[i]) for i, (s, d) in enumerate(
        ((wg_hbm, wg_v), (wu_hbm, wu_v), (wd_hbm, wd_v), (wo_hbm, wo_v)))]
    late.append(pltpu.make_async_copy(wr_hbm, wr_v, lsems.at[4]))

    def start(cps, priority=0):
        for cp in cps:
            cp.start(priority=priority)

    def wait(cps):
        for cp in cps:
            cp.wait()

    first_w = pair_copies(0)
    start(first_w + in_copies(0))
    for j in range(1, len(CHUNKS) - 1):
        start(in_copies(j), priority=1)
    for g in range(1, NPAIR):
        start(pair_copies(g), priority=1)

    lane = lax.broadcasted_iota(jnp.int32, (8, T), 1)
    sub = lax.broadcasted_iota(jnp.int32, (8, T), 0)
    qscale = (D ** -0.5) * math.log2(math.e)

    zero = jnp.min(lane)

    def after(tok, v):
        return jnp.where(zero > 0, tok, v)

    queue = []
    pending = []
    clock = [0]
    every = [0]

    def operand(ref, r0, n, *lead):
        w32 = ref[(*lead, pl.ds(r0 // 2, n // 2), slice(None))]
        clock[0] += 1
        due = [tok for t, tok in pending if t < clock[0]]
        pending[:] = [e for e in pending if e[0] >= clock[0]]
        if due:
            top = w32[0:8, 0:T]
            for tok in due:
                top = after(pltpu.bitcast(tok, U32), top)
            if w32.shape[1] > T:
                top = jnp.concatenate([top, w32[0:8, T:]], axis=1)
            w32 = jnp.concatenate([top, w32[8:]], axis=0)
        if queue and every[0] and clock[0] % every[0] == 0:
            queue.pop(0)()
        return pltpu.bitcast(w32, BF16)

    def anchor(tok):
        pending.append((clock[0] + ANCHOR, tok))

    def flush():
        while queue:
            queue.pop(0)()

    def layernorm(i):
        xf = _ld(x_v, i * T, T).astype(F32)
        mean = _rowsum(xf) * (1.0 / M)
        mean_b = _rb(mean)
        cen = xf - mean_b
        off = mean - mean_b
        var = jnp.maximum(_rowsum(cen * cen) * (1.0 / M) - off * off, 0.0)
        _st(xn_v, i * T, _rb(cen) * _recip(_rb(jnp.sqrt(_rb(_rb(var) + LN_EPS)))))

    def unpack_weights(g, buf, t):
        even = wp_v[g, pl.ds(t * T, T // 2, stride=2), :]
        odd = wp_v[g, pl.ds(t * T + 1, T // 2, stride=2), :]
        if buf:
            w = (even >> 16) | (odd & U32(0xFFFF0000))
        else:
            w = (even & U32(0xFFFF)) | (odd << 16)
        wh_v[buf, pl.ds(t * T // 2, T // 2), :] = w

    def unpacking(g, buf):
        return [(0, lambda t=t: unpack_weights(g, buf, t)) for t in range(MT + 2 * CT)]

    def project_q(i, buf):
        _st(q_v, i * T, _dot(operand(xn_v, i * T, T), _ld(wh_v, 0, M, buf)) * qscale, buf)

    def project_k(i, buf):
        _st(k_v, i * T, _dot(operand(c_v, i * T, T), _ld(wh_v, M, DC, buf)), buf)

    def project_v(i, buf, behind=None):
        c = operand(c_v, i * T, T)
        if behind is not None:
            c = pltpu.bitcast(c, U32)
            tok = jnp.concatenate([pltpu.bitcast(behind[T - 8:T], U32)] * CT, axis=1)
            c = pltpu.bitcast(jnp.concatenate([after(tok, c[0:8]), c[8:]], axis=0), BF16)
        _st(v_v, i * T, _dot(c, _ld(wh_v, M + DC, DC, buf)), buf)

    def projections(buf):
        qs = [(MT, lambda i=i: project_q(i, buf)) for i in range(NB)]
        ks = [(CT, lambda i=i: project_k(i, buf)) for i in range(NB)]
        vs = [(CT, lambda i=i, **kw: project_v(i, buf, **kw)) for i in range(NB)]
        return (qs + ks if Q_FIRST[buf] else ks + qs) + vs

    def scores(i, t, n, buf, st):
        tiles = _tiles(_dot_nt(operand(q_v, i * T, T, buf), _ld(k_v, t * T, n * T, buf)))
        if t + n == i + 1:
            row = lax.broadcasted_iota(jnp.int32, (T, T), 0)
            col = lax.broadcasted_iota(jnp.int32, (T, T), 1)
            tiles[-1] = jnp.where(col <= row, tiles[-1], NEG)
        st[t] = jnp.concatenate(tiles, axis=1) if n > 1 else tiles[0]
        st["m"] = _tree(jnp.maximum, tiles + ([st["m"]] if t else []))
        if t + n == i + 1:
            st["m"] = jnp.max(st["m"], axis=-1, keepdims=True)

    last_ctx = []

    def context(i, t, n, h, buf, st):
        if GATE[buf] and t // CK == GATE[buf]:
            tok = st["pv"][0][GATE_ROW[buf]:GATE_ROW[buf] + 8]
            st["m"] = after(jnp.concatenate([tok] * (T // 8), axis=0), st["m"])
        m = st["m"]
        if m.shape[1] == T and n > 1:
            m = jnp.concatenate([m] * n, axis=1)
        d = st[t] - m
        if t == 0 and last_ctx:
            d0 = after(last_ctx.pop(), d[:, 0:T])
            d = jnp.concatenate([d0, d[:, T:]], axis=1) if n > 1 else d0
        p = jnp.exp2(d)
        l = _tree(jnp.add, _tiles(p))
        o = _dot(p.astype(BF16), operand(v_v, t * T, n * T, buf))
        st.setdefault("pv", []).append(o)
        if t:
            l, o = st["l"] + l, st["o"] + o
        st["l"], st["o"] = l, o
        if t + n == i + 1:
            o = o * _recip(jnp.sum(l, axis=-1, keepdims=True))
            last_ctx.append(o)
            _st(ctx_v, i * T, o, h)

    def head(h, buf, fillers, hold=False, before=None):
        work = [(i, t, min(CK, i + 1 - t)) for i in range(NB) for t in range(0, i + 1, CK)]
        state = [{} for _ in range(NB)]
        held = []
        if hold:
            cut = len(fillers) - HOLD[0] - HOLD[1]
            fillers, held = fillers[:cut], fillers[cut:]
        att_total = 2 * sum(n for _, _, n in work)
        fill_total = sum(c for c, _ in fillers)
        a = b = f = att = fill = 0
        ready = {}
        scored = False
        while b < len(work) or f < len(fillers):
            b_ok = b < len(work) and ready.get(work[b][0], math.inf) <= att + fill
            if f < len(fillers) and ((fill - BIAS[buf]) * att_total < att * fill_total
                                     or (a == len(work) and not b_ok)):
                fillers[f][1]()
                fill += fillers[f][0]
                f += 1
            elif a < len(work) and not (b_ok and scored):
                i, t, n = work[a]
                if before is not None and t == 0:
                    fill += before(i)
                scores(i, t, n, buf, state[i])
                a, att, scored = a + 1, att + n, True
                if t + n == i + 1:
                    ready[i] = att + fill + LAG[buf]
                if a == len(work):
                    for _, fn in held[:HOLD[0]]:
                        fn(behind=state[i][t - CK][:, 0:T])
            else:
                i, t, n = work[b]
                context(i, t, n, h, buf, state[i])
                b, att, scored = b + 1, att + n, False
        for _, fn in held[HOLD[0]:]:
            fn(behind=state[-1]["pv"][-HOLD[2]])

    def first_weights(t0, n):
        for t in range(t0, t0 + n):
            unpack_weights(0, 0, t)
            unpack_weights(0, 1, t)

    def prepare(i):
        cost = 0
        if i in CHUNKS[:-1]:
            wait(in_copies(CHUNKS.index(i)))
        if i == 0:
            wait(first_w[:1])
            first_weights(MT, CT)
        if i == 1:
            wait(first_w[1:])
        if i < NB:
            project_k(i, 0)
            project_k(i, 1)
            cost += 2 * CT
        if i == 1:
            first_weights(MT + CT, CT)
            first_weights(0, MT)
        if 1 <= i <= NB:
            project_v(i - 1, 0)
            layernorm(i - 1)
            project_q(i - 1, 0)
            project_q(i - 1, 1)
            cost += CT + 2 * MT
        if i >= NB:
            for j in range((i - NB) * NB // AHEAD, (i - NB + 1) * NB // AHEAD):
                project_v(j, 1)
                cost += CT
        return cost

    for i in range(AHEAD):
        prepare(i)
    head(0, 0, [], before=lambda i: prepare(i + AHEAD))
    wait(pair_copies(1))
    start(late)
    for _, fn in unpacking(1, 0):
        fn()

    def pair_body(g, carry):
        last_ctx.clear()

        @pl.when(g + 1 < NPAIR)
        def _():
            wait(pair_copies(g + 1))

        head(2 * g - 1, 1, _merge(projections(0), unpacking(g, 1)))
        head(2 * g, 0, unpacking(jnp.minimum(g + 1, NPAIR - 1), 0) + projections(1), hold=True)
        return carry

    lax.fori_loop(1, NPAIR, pair_body, 0)
    last_ctx.clear()
    wait(late[3:])

    wr = wr_v[...].astype(F32).reshape(1, M)
    routed = [jnp.zeros((8, T), F32) for _ in range(S // (8 * T))]
    keys, sel, sel_rows, ffn = [], [], [], {}

    def router(i):
        r = _rowsum(_ld(xn_v, i * T, T).astype(F32) * wr)
        for g in range(T // 8):
            k, ln = divmod(i * T // 8 + g, T)
            routed[k] = jnp.where(lane == ln, r[g * 8:(g + 1) * 8, :], routed[k])
        anchor(routed[k])

    def select_step():
        if not keys:
            for k, r in enumerate(routed):
                bits = pltpu.bitcast(_rb(r), jnp.int32) >> 16
                mag = bits & 0x7FFF
                rank = jnp.where(bits < 0, 0x8000 - mag, 0x8000 + mag)
                rank = jnp.where(mag > 0x7F80, 0, rank)
                row = k * 8 * T + lane * 8 + sub
                keys.append(pltpu.bitcast(rank * S + (S - 1 - row) + KEY0, F32))
        top = jnp.max(jnp.max(_tree(jnp.maximum, keys), axis=0, keepdims=True), axis=1, keepdims=True)
        top = jnp.broadcast_to(top, (8, T))
        sel.append(pltpu.bitcast(top, jnp.int32) - KEY0)
        keys[:] = [jnp.where(kk == top, 0.0, kk) for kk in keys]
        anchor(top)

    def gather():
        slot = lax.broadcasted_iota(jnp.int32, (TOPC, M), 0)
        xs = jnp.zeros((TOPC, M), F32)
        key = jnp.zeros((TOPC, T), jnp.int32)
        for j, top in enumerate(sel):
            row = S - 1 - (top[0, 0] & (S - 1))
            sel_rows.append(row)
            w32 = xn_v[pl.ds(row >> 1, 1), :] << (16 - 16 * (row & 1)).astype(U32)
            xs = jnp.where(slot == j, pltpu.bitcast(w32 & U32(0xFFFF0000), F32), xs)
            key = jnp.where(sub == j, top, key)
        rank = key >> (S.bit_length() - 1)
        bits = jnp.where(rank >= 0x8000, rank - 0x8000, (0x8000 - rank) | 0x8000)
        bits = jnp.where(rank == 0, 0x7FC0, bits)
        ffn["gain"] = jax.nn.sigmoid(pltpu.bitcast(bits << 16, F32))
        ffn["x"] = xs.astype(BF16)

    FG = 4 * T

    def ffn_in(name, w_v, f0, k):
        w = pltpu.bitcast(w_v[f0 // 2:min(f0 + FG, FF) // 2, k * T:(k + 1) * T], BF16)
        part = _dot_nt(ffn["x"][:, k * T:(k + 1) * T], w)
        ffn[name, f0] = ffn[name, f0] + part if k else part

    def ffn_down(f0, n0, n1):
        if n0 == 0:
            g, u = ffn["g", f0], ffn["u", f0]
            ffn["h", f0] = (g * jax.nn.sigmoid(g) * u).astype(BF16)
        w = pltpu.bitcast(wd_v[f0 // 2:min(f0 + FG, FF) // 2, n0 * T:n1 * T], BF16)
        for n, part in zip(range(n0, n1), _tiles(_dot(ffn["h", f0], w))):
            ffn["y", n] = ffn["y", n] + part if f0 else part

    ffn_steps = []
    for f0 in range(0, FF, FG):
        for k in range(MT):
            gate = lambda f0=f0, k=k: ffn_in("g", wg_v, f0, k)
            up = lambda f0=f0, k=k: ffn_in("u", wu_v, f0, k)
            ffn_steps += [gate, up] if f0 + FG <= FF else [lambda gate=gate, up=up: (gate(), up())]
    for f0 in range(0, FF, FG):
        step = 1 if f0 + FG <= FF else 2
        for n in range(0, MT, step):
            ffn_steps.append(lambda f0=f0, n=n, step=step: ffn_down(f0, n, min(n + step, MT)))

    def residual(r0, n):
        acc_v[r0:r0 + n, :] = _ld(x_v, r0, n).astype(F32) + _ld(xn_v, r0, n).astype(F32)
        anchor(acc_v[pl.ds(pl.multiple_of(zero * 8, 8), 8), 0:T])

    def out_project(rp, n, h0, h1):
        ctx = jnp.concatenate(
            [pltpu.bitcast(ctx_v[h, pl.ds(rp, n // 2), :], BF16) for h in range(h0, h1)], axis=1)
        return _dot(ctx, operand(wo_v, h0 * D, (h1 - h0) * D))

    attn = {}

    def out_step(i, h):
        part = out_project(i * T // 2, T, h, h + 1)
        attn[i] = attn[i] + part if h else part

    def finish(rp, val):
        rows = pl.ds(2 * rp, val.shape[0])
        o_v[rows, :] = (acc_v[rows, :] + val).astype(BF16)
        pltpu.make_async_copy(o_v.at[rows], out_hbm.at[rows], osem).start()

    queue.extend([lambda i=i: router(i) for i in range(NB)] + [select_step] * TOPC + [gather])
    every[0] = 4
    head(H - 1, 1, [(MT, lambda h=h: out_step(0, h)) for h in range(H - 1)])
    flush()
    wait(late[:3])
    out_step(0, H - 1)
    queue.extend([lambda r0=r0: residual(r0, 32) for r0 in range(0, S, 32)])
    every[0] = 1
    for fn in _merge([lambda i=i, h=h: out_step(i, h)
                      for i in range(1, FFN_BLOCKS + 1) for h in range(H)],
                     ffn_steps + [lambda: None] * 10):
        fn()
    flush()
    pending.clear()
    y = jnp.concatenate([ffn["y", n] * ffn["gain"] for n in range(MT)], axis=1)
    olds = [acc_v[pl.ds(row, 1), :] for row in sel_rows]
    for j, row in enumerate(sel_rows):
        acc_v[pl.ds(row, 1), :] = olds[j] + y[j:j + 1, :]

    for i in range(FFN_BLOCKS + 1, FLAT_BLOCKS):
        for h in range(H):
            out_step(i, h)
            if h % 8 == 3 and len(attn) > 1:
                j = min(attn)
                finish(j * T // 2, attn.pop(j))
    for j in sorted(attn):
        finish(j * T // 2, attn[j])

    def out_body(b, carry):
        for u in range(OUT_UNROLL):
            r0 = FLAT_BLOCKS * T + (b * OUT_UNROLL + u) * OUT_ROWS
            rp = pl.multiple_of(r0 // 2, T // 2)
            finish(rp, out_project(rp, OUT_ROWS, 0, H))
        return carry

    assert (S - FLAT_BLOCKS * T) % (OUT_UNROLL * OUT_ROWS) == 0
    lax.fori_loop(0, (S - FLAT_BLOCKS * T) // (OUT_UNROLL * OUT_ROWS), out_body, 0)
    pltpu.make_async_copy(o_v, out_hbm, osem).wait()


@jax.jit
def pallas_parallel_sum__compressed_kv_cla__moe_arch_mod__prompt_kernel(
    A_x: jax.Array,
    A_c_kv: jax.Array,
    A_w_q: jax.Array,
    A_w_uk: jax.Array,
    A_w_uv: jax.Array,
    A_w_o: jax.Array,
    B_x: jax.Array,
    B_w_r: jax.Array,
    B_w_gate: jax.Array,
    B_w_up: jax.Array,
    B_w_down: jax.Array,
):
    del B_x
    _, S, M = A_x.shape
    DC = A_c_kv.shape[2]
    H, D = A_w_q.shape[1], A_w_q.shape[2]
    FF = B_w_gate.shape[1]
    hbm = pl.BlockSpec(memory_space=pltpu.HBM)
    out = pl.pallas_call(
        _kernel,
        out_shape=jax.ShapeDtypeStruct((S, M), A_x.dtype),
        in_specs=[hbm] * 10,
        out_specs=hbm,
        scratch_shapes=[
            pltpu.VMEM((S // 2, M), U32),
            pltpu.VMEM((S // 2, DC), U32),
            pltpu.VMEM((H // 2, M + 2 * DC + 8, D), U32),
            pltpu.VMEM((H * D // 2, M), U32),
            pltpu.VMEM((M,), BF16),
            pltpu.VMEM((FF // 2, M), U32),
            pltpu.VMEM((FF // 2, M), U32),
            pltpu.VMEM((FF // 2, M), U32),
            pltpu.VMEM((S // 2, M), U32),
            pltpu.VMEM((2, S // 2, D), U32),
            pltpu.VMEM((2, S // 2, D), U32),
            pltpu.VMEM((2, S // 2, D), U32),
            pltpu.VMEM((2, (M + 2 * DC) // 2, D), U32),
            pltpu.VMEM((H, S // 2, D), U32),
            pltpu.VMEM((S, M), F32),
            pltpu.VMEM((S, M), BF16),
            pltpu.SemaphoreType.DMA((2 * (len(CHUNKS) - 1),)),
            pltpu.SemaphoreType.DMA((3 * H // 2,)),
            pltpu.SemaphoreType.DMA((5,)),
            pltpu.SemaphoreType.DMA(()),
        ],
        compiler_params=pltpu.CompilerParams(vmem_limit_bytes=100 * 1024 * 1024),
    )(
        A_x.reshape(S, M),
        A_c_kv.reshape(S, DC),
        A_w_q,
        A_w_uk,
        A_w_uv,
        A_w_o.reshape(H * D, M),
        B_w_r,
        B_w_gate.T,
        B_w_up.T,
        B_w_down,
    )
    return out.reshape(1, S, M)
```
